```python
import os as _os
_os.environ.setdefault("JAX_PLATFORMS", "cpu")
import jax
import jax.numpy as jnp

def _softmax(x, axis=-1):
    return jax.nn.softmax(x, axis=axis)
def _gelu(x):
    return jax.nn.gelu(x, approximate=True)
def _silu(x):
    return jax.nn.silu(x)
def _sigmoid(x):
    return jax.nn.sigmoid(x)
def _layernorm(x, axis=-1, eps=1e-5):
    m = jnp.mean(x, axis=axis, keepdims=True)
    v = jnp.var(x, axis=axis, keepdims=True)
    return (x - m) / jnp.sqrt(v + eps)
def _scatter_add(tgt, idx, src, axis=0):
    return tgt.at[idx].add(src)
def _segment_sum(src, seg, n):
    return jax.ops.segment_sum(src, seg, n)
class _Rng:
    def __init__(self, key):
        self._k = key
    def _next(self):
        self._k, sub = jax.random.split(self._k)
        return sub
    def normal(self, shape):
        return jax.random.normal(self._next(), shape, dtype=jnp.bfloat16)
    def randint(self, lo, hi, shape):
        return jax.random.randint(self._next(), shape, lo, hi, dtype=jnp.int32)
    def uniform(self, shape, lo=0.0, hi=1.0):
        return jax.random.uniform(self._next(), shape, jnp.bfloat16, lo, hi)
    def permutation(self, n):
        return jax.random.permutation(self._next(), n)


kernel_name = 'gated_mix__ssm_conv_h3__ssm_conv_h3__prompt'

def setup_inputs():
    _rng = _Rng(jax.random.key(int.from_bytes(__import__("os").urandom(4), "little")))
    _w = (lambda a: (lambda t: t.astype(jnp.bfloat16) if jnp.issubdtype(t.dtype, jnp.floating) else t)(jnp.asarray(a)))
    def _A_setup():
        B, S, D = 1, 2048, 640
        ks = 4
        return {
            "q": _w((lambda *s: _rng.normal(s) * 0.05)(B, S, D)),
            "k": _w((lambda *s: _rng.normal(s) * 0.05)(B, S, D)),
            "v": _w((lambda *s: _rng.normal(s) * 0.05)(B, S, D)),
            "shift_k": _w((lambda *s: _rng.normal(s) * 0.05)(D, ks) * 0.5),
            "ssm_k": _w((lambda *s: _rng.normal(s) * 0.05)(D, S) * (1.0 / S ** 0.5)),
            "ssm_D": _w((lambda *s: _rng.normal(s) * 0.05)(D)),
        }
    _A_in = _A_setup()

    def _B_setup():
        B, S, D = 1, 2048, 640
        ks = 4
        return {
            "q": _w((lambda *s: _rng.normal(s) * 0.05)(B, S, D)),
            "k": _w((lambda *s: _rng.normal(s) * 0.05)(B, S, D)),
            "v": _w((lambda *s: _rng.normal(s) * 0.05)(B, S, D)),
            "shift_k": _w((lambda *s: _rng.normal(s) * 0.05)(D, ks) * 0.5),
            "ssm_k": _w((lambda *s: _rng.normal(s) * 0.05)(D, S) * (1.0 / S ** 0.5)),
            "ssm_D": _w((lambda *s: _rng.normal(s) * 0.05)(D)),
        }
    _B_in = _B_setup()

    return {
        "A_q": _A_in["q"],
        "A_k": _A_in["k"],
        "A_v": _A_in["v"],
        "A_shift_k": _A_in["shift_k"],
        "A_ssm_k": _A_in["ssm_k"],
        "A_ssm_D": _A_in["ssm_D"],
        "B_q": _B_in["q"],
        "B_k": _B_in["k"],
        "B_v": _B_in["v"],
        "B_shift_k": _B_in["shift_k"],
        "B_ssm_k": _B_in["ssm_k"],
        "B_ssm_D": _B_in["ssm_D"],
        "gate_w": _w((lambda *s: _rng.normal(s) * 0.05)(640) * 16.0),
    }

def reference(A_q, A_k, A_v, A_shift_k, A_ssm_k, A_ssm_D, B_q, B_k, B_v, B_shift_k, B_ssm_k, B_ssm_D, gate_w):
    def _A_ref(q, k, v, shift_k, ssm_k, ssm_D):
        B, S, D = q.shape
        ks = shift_k.shape[-1]
        k_pad = jnp.pad(k, ((0, 0), (ks - 1, 0), (0, 0)))
        k_shift = jnp.zeros_like(k)
        for t in range(ks):
            k_shift = k_shift + k_pad[:, t:t + S, :] * shift_k[:, ks - 1 - t][None, None, :]
        kv = k_shift * v
        L = 2 * S
        kv_pad = jnp.pad(kv, ((0, 0), (0, S), (0, 0)))
        kf_pad = jnp.pad(ssm_k, ((0, 0), (0, S)))
        kv_f = (lambda x, axes=(-2,-1): jnp.fft.rfft2(x.astype(jnp.float32), axes=axes))(kv_pad[:, None, :, :], axes=(1, 2))
        kf_f = (lambda x, axes=(-2,-1): jnp.fft.rfft2(x.astype(jnp.float32), axes=axes))(kf_pad[:, None, :], axes=(1, 2))
        kf_f = (lambda x, *d: x.transpose(*d))(kf_f, 1, 2, 0)
        y_f = kv_f * kf_f[None, :, :, :]
        y = (lambda x, s, axes=(-2,-1): jnp.fft.irfft2(x, s=s, axes=axes).astype(jnp.bfloat16))(y_f, (1, L), axes=(1, 2))[:, 0, :S, :]
        y = y + kv * ssm_D[None, None, :]
        return q * y

    def _B_ref(q, k, v, shift_k, ssm_k, ssm_D):
        B, S, D = q.shape
        ks = shift_k.shape[-1]
        k_pad = jnp.pad(k, ((0, 0), (ks - 1, 0), (0, 0)))
        k_shift = jnp.zeros_like(k)
        for t in range(ks):
            k_shift = k_shift + k_pad[:, t:t + S, :] * shift_k[:, ks - 1 - t][None, None, :]
        kv = k_shift * v
        L = 2 * S
        kv_pad = jnp.pad(kv, ((0, 0), (0, S), (0, 0)))
        kf_pad = jnp.pad(ssm_k, ((0, 0), (0, S)))
        kv_f = (lambda x, axes=(-2,-1): jnp.fft.rfft2(x.astype(jnp.float32), axes=axes))(kv_pad[:, None, :, :], axes=(1, 2))
        kf_f = (lambda x, axes=(-2,-1): jnp.fft.rfft2(x.astype(jnp.float32), axes=axes))(kf_pad[:, None, :], axes=(1, 2))
        kf_f = (lambda x, *d: x.transpose(*d))(kf_f, 1, 2, 0)
        y_f = kv_f * kf_f[None, :, :, :]
        y = (lambda x, s, axes=(-2,-1): jnp.fft.irfft2(x, s=s, axes=axes).astype(jnp.bfloat16))(y_f, (1, L), axes=(1, 2))[:, 0, :S, :]
        y = y + kv * ssm_D[None, None, :]
        return q * y

    x = A_q
    g = _sigmoid((x * gate_w).sum(-1, keepdims=True))
    a = _A_ref(x, A_k, A_v, A_shift_k, A_ssm_k, A_ssm_D)
    b = _B_ref(x, B_k, B_v, B_shift_k, B_ssm_k, B_ssm_D)
    return g * a + (1 - g) * b
```

```python
import functools
import numpy as np
import jax
import jax.numpy as jnp
from jax.experimental import pallas as pl
from jax.experimental.pallas import tpu as pltpu

S, D, N1, N2 = 2048, 640, 128, 16
F32, BF16, U32 = jnp.float32, jnp.bfloat16, jnp.uint32


def _consts():
    n1 = np.arange(N1)[None, None, :]
    k1 = np.arange(N1)[None, :, None]
    n2 = np.arange(N2)[:, None, None]
    ph = -2 * np.pi * (n1 * k1 / 128.0 + n2 * k1 / 2048.0) + np.pi * (16 * n1 + n2) / 4096.0
    Gr, Gi = np.cos(ph), np.sin(ph)
    G = np.stack([Gr.reshape(N2, 16, 8, N1), Gi.reshape(N2, 16, 8, N1)], axis=2).reshape(N2, 256, N1)
    Ginv = np.transpose(G, (0, 2, 1)) / 2048.0
    Pm = np.zeros((128, 128), np.float32)
    for n2_ in range(16):
        for a in range(8):
            Pm[n2_ * 8 + a, 16 * a + n2_] = 1.0
    return G.astype(np.float32), Ginv.astype(np.float32), Pm

_C1, _S1, _R = float(np.cos(np.pi / 8)), float(np.sin(np.pi / 8)), float(np.sqrt(0.5))


def _bfly4(x, sgn):
    (ar, ai), (br, bi), (cr, ci), (dr, di) = x
    t0r, t0i = ar + cr, ai + ci
    t1r, t1i = ar - cr, ai - ci
    t2r, t2i = br + dr, bi + di
    t3r, t3i = br - dr, bi - di
    x0 = (t0r + t2r, t0i + t2i)
    x2 = (t0r - t2r, t0i - t2i)
    if sgn < 0:
        x1 = (t1r + t3i, t1i - t3r)
        x3 = (t1r - t3i, t1i + t3r)
    else:
        x1 = (t1r - t3i, t1i + t3r)
        x3 = (t1r + t3i, t1i - t3r)
    return [x0, x1, x2, x3]


def _tw(z, e, sgn):
    a, b = z
    if e == 0:
        return z
    if sgn < 0:
        if e == 4: return (b, -a)
        if e == 2: return ((a + b) * _R, (b - a) * _R)
        if e == 6: return ((b - a) * _R, (a + b) * (-_R))
        if e == 1: return (a * _C1 + b * _S1, b * _C1 - a * _S1)
        if e == 3: return (a * _S1 + b * _C1, b * _S1 - a * _C1)
        if e == 9: return (a * (-_C1) - b * _S1, a * _S1 - b * _C1)
    else:
        if e == 4: return (-b, a)
        if e == 2: return ((a - b) * _R, (a + b) * _R)
        if e == 6: return ((a + b) * (-_R), (a - b) * _R)
        if e == 1: return (a * _C1 - b * _S1, b * _C1 + a * _S1)
        if e == 3: return (a * _S1 - b * _C1, b * _S1 + a * _C1)
        if e == 9: return (b * _S1 - a * _C1, a * (-_S1) - b * _C1)
    raise ValueError(e)


def fft16(x, sgn):
    A = [_bfly4([x[nb], x[nb + 4], x[nb + 8], x[nb + 12]], sgn) for nb in range(4)]
    B = [[_tw(A[nb][ka], nb * ka, sgn) for ka in range(4)] for nb in range(4)]
    X = [None] * 16
    for ka in range(4):
        o = _bfly4([B[0][ka], B[1][ka], B[2][ka], B[3][ka]], sgn)
        for kb in range(4):
            X[ka + 4 * kb] = o[kb]
    return X


def _row_bcast(v, rows=8):
    return jnp.broadcast_to(v, (rows, v.shape[-1]))


def kernel(q_ref, qf_ref, ka_ref, va_ref, kb_ref, vb_ref, ha_ref, hb_ref, ska_ref, skb_ref,
           da_ref, db_ref, gw_ref, g_ref, gi_ref, pm_ref, o_ref,
           hp, kvp, zh, zu, yp, gnat, par):
    j = pl.program_id(0)

    @pl.when(j == 0)
    def _gate():
        gw = gw_ref[...].reshape(1, D)
        for bb, d_ref in enumerate((da_ref, db_ref)):
            dd = _row_bcast(d_ref[...].astype(F32).reshape(1, D))
            for t in range(5):
                par[t, pl.ds(8 * bb, 8), :] = dd[:, 128 * t:128 * (t + 1)]
        gwb = jnp.broadcast_to(gw, (128, D))
        for r in range(S // 256):
            xs = qf_ref[0, pl.ds(r * 256, 256), :]
            lg = jax.lax.dot_general(xs, gwb, (((1,), (1,)), ((), ())), preferred_element_type=F32)
            gnat[pl.ds(r * 256, 256), :] = jax.nn.sigmoid(lg)

    pm = pm_ref[...]
    for b, h_ref in enumerate((ha_ref, hb_ref)):
        for jj in range(8):
            R = []
            for jt in (2 * jj, 2 * jj + 1):
                R.append(jax.lax.dot_general(pm, h_ref[:, pl.ds(128 * jt, 128)], (((1,), (1,)), ((), ())),
                                             preferred_element_type=F32))
            for n2 in range(16):
                blk = jnp.concatenate([R[0][8 * n2:8 * n2 + 8], R[1][8 * n2:8 * n2 + 8]], axis=0)
                hp[b, n2, pl.ds(16 * jj, 16), :] = blk.astype(BF16)

    lane0 = pl.multiple_of(j * 128, 128)
    for b, (k_ref, v_ref, sk_ref) in enumerate(((ka_ref, va_ref, ska_ref), (kb_ref, vb_ref, skb_ref))):
        skT = jnp.transpose(sk_ref[...].astype(F32))
        s = [_row_bcast(skT[t:t + 1, :], 16) for t in range(4)]
        kw = k_ref.bitcast(U32)
        vw = v_ref.bitcast(U32)

        def unpack(w):
            lo = jax.lax.bitcast_convert_type(w << 16, F32)
            hi = jax.lax.bitcast_convert_type(w & jnp.uint32(0xFFFF0000), F32)
            return lo, hi

        def p_body(a2, carry, first=False):
            base = pl.multiple_of(a2 * 128, 128)
            ksub = kw.at[0, pl.ds(base, 128), :]
            vsub = vw.at[0, pl.ds(base, 128), :]
            kk = {}
            for m in range(8):
                lo, hi = unpack(ksub[pl.ds(m, 16, stride=8), :])
                kk[2 * m], kk[2 * m + 1] = lo, hi
            for m in (6, 7):
                if first:
                    w = ksub[pl.ds(m, 16, stride=8), :]
                    w = pltpu.roll(w, 1, axis=0)
                    rid = jax.lax.broadcasted_iota(jnp.int32, (16, 128), 0)
                    w = jnp.where(rid == 0, jnp.uint32(0), w)
                else:
                    kprev = kw.at[0, pl.ds(pl.multiple_of(base - 8, 8), 128), :]
                    w = kprev[pl.ds(m, 16, stride=8), :]
                lo, hi = unpack(w)
                kk[2 * m - 16], kk[2 * m + 1 - 16] = lo, hi
            for m in range(8):
                vlo, vhi = unpack(vsub[pl.ds(m, 16, stride=8), :])
                for n2, vv in ((2 * m, vlo), (2 * m + 1, vhi)):
                    acc = kk[n2] * s[0] + kk[n2 - 1] * s[1] + kk[n2 - 2] * s[2] + kk[n2 - 3] * s[3]
                    kvp[b, n2, pl.ds(pl.multiple_of(a2 * 16, 16), 16), :] = (acc * vv).astype(BF16)
            return carry

        p_body(0, 0, first=True)
        jax.lax.fori_loop(1, 8, p_body, 0)

    def f_body(n2, carry):
        g = g_ref[n2]
        rh = jnp.concatenate([hp[0, n2], hp[1, n2]], axis=1)
        ru = jnp.concatenate([kvp[0, n2], kvp[1, n2]], axis=1)
        zhh = jnp.dot(g, rh, preferred_element_type=F32)
        zuu = jnp.dot(g, ru, preferred_element_type=F32)
        zh[0, n2] = zhh[:, :128]
        zh[1, n2] = zhh[:, 128:]
        zu[0, n2] = zuu[:, :128]
        zu[1, n2] = zuu[:, 128:]
        return carry
    jax.lax.fori_loop(0, 16, f_body, 0)

    dvec = [par[j, pl.ds(0, 8), :], par[j, pl.ds(8, 8), :]]

    def v_body(g, carry):
        r0 = pl.multiple_of(g * 16, 16)
        for b in range(2):
            x = [(zh[b, n2, pl.ds(r0, 8), :], zh[b, n2, pl.ds(r0 + 8, 8), :]) for n2 in range(16)]
            x[0] = (x[0][0] + dvec[b], x[0][1])
            H = fft16(x, -1)
            for k2 in range(16):
                zh[b, k2, pl.ds(r0, 8), :] = H[k2][0]
                zh[b, k2, pl.ds(r0 + 8, 8), :] = H[k2][1]
        for b in range(2):
            x = [(zu[b, n2, pl.ds(r0, 8), :], zu[b, n2, pl.ds(r0 + 8, 8), :]) for n2 in range(16)]
            U = fft16(x, -1)
            Y = []
            for k2 in range(16):
                hr, hi = zh[b, k2, pl.ds(r0, 8), :], zh[b, k2, pl.ds(r0 + 8, 8), :]
                ur, ui = U[k2]
                Y.append((ur * hr - ui * hi, ur * hi + ui * hr))
            T = fft16(Y, +1)
            for n2 in range(16):
                yp[b, n2, pl.ds(r0, 16), :] = jnp.concatenate([T[n2][0], T[n2][1]], axis=0).astype(BF16)
        return carry
    jax.lax.fori_loop(0, 16, v_body, 0)

    qw = q_ref.bitcast(U32)
    ow = o_ref.bitcast(U32)

    def i_body(m, carry):
        qword = qw[0, pl.ds(m, 128, stride=8), :]
        qlo = jax.lax.bitcast_convert_type(qword << 16, F32)
        qhi = jax.lax.bitcast_convert_type(qword & jnp.uint32(0xFFFF0000), F32)
        res = []
        for t, qq in ((0, qlo), (1, qhi)):
            n2 = 2 * m + t
            ry = jnp.concatenate([yp[0, n2], yp[1, n2]], axis=1)
            y = jnp.dot(gi_ref[n2], ry, preferred_element_type=F32)
            ya, yb = y[:, :128], y[:, 128:]
            gg = gnat[pl.ds(n2, 128, stride=16), :]
            res.append(qq * (yb + gg * (ya - yb)))
        word = pltpu.pack_elementwise((res[0], res[1]), packed_dtype=BF16)
        ow[0, pl.ds(m, 128, stride=8), :] = word
        return carry
    for m in range(8):
        i_body(m, 0)


def run(A_q, A_k, A_v, A_shift_k, A_ssm_k, A_ssm_D, B_q, B_k, B_v, B_shift_k, B_ssm_k, B_ssm_D, gate_w):
    G, Ginv, Pm = _consts()
    tile = lambda: pl.BlockSpec((1, S, 128), lambda j: (0, 0, j))
    full = lambda shp: pl.BlockSpec(shp, lambda j: (0,) * len(shp))
    return pl.pallas_call(
        kernel,
        grid=(D // 128,),
        in_specs=[tile(), full((1, S, D)), tile(), tile(), tile(), tile(),
                  pl.BlockSpec((128, S), lambda j: (j, 0)), pl.BlockSpec((128, S), lambda j: (j, 0)),
                  pl.BlockSpec((128, 4), lambda j: (j, 0)), pl.BlockSpec((128, 4), lambda j: (j, 0)),
                  full((D,)), full((D,)), full((D,)),
                  full((16, 256, 128)), full((16, 128, 256)), full((128, 128))],
        out_specs=tile(),
        out_shape=jax.ShapeDtypeStruct((1, S, D), BF16),
        scratch_shapes=[pltpu.VMEM((2, 16, 128, 128), BF16), pltpu.VMEM((2, 16, 128, 128), BF16),
                        pltpu.VMEM((2, 16, 256, 128), F32), pltpu.VMEM((2, 16, 256, 128), F32),
                        pltpu.VMEM((2, 16, 256, 128), BF16), pltpu.VMEM((S, 128), F32), pltpu.VMEM((5, 16, 128), F32)],
        compiler_params=pltpu.CompilerParams(dimension_semantics=("arbitrary",), vmem_limit_bytes=100 * 1024 * 1024),
    )(A_q, A_q, A_k, A_v, B_k, B_v, A_ssm_k, B_ssm_k, A_shift_k, B_shift_k, A_ssm_D, B_ssm_D, gate_w,
      jnp.asarray(G, BF16), jnp.asarray(Ginv, BF16), jnp.asarray(Pm, BF16))


@jax.jit
def pallas_gated_mix__ssm_conv_h3__ssm_conv_h3__prompt_kernel(
    A_q, A_k, A_v, A_shift_k, A_ssm_k, A_ssm_D, B_q, B_k, B_v, B_shift_k, B_ssm_k, B_ssm_D, gate_w,
):
    return run(A_q, A_k, A_v, A_shift_k, A_ssm_k, A_ssm_D, B_q, B_k, B_v, B_shift_k, B_ssm_k, B_ssm_D, gate_w)
```

```python
import functools
import numpy as np
import jax
import jax.numpy as jnp
from jax.experimental import pallas as pl
from jax.experimental.pallas import tpu as pltpu

S, D, N1, N2 = 2048, 640, 128, 16
NT = D // 128
NP = 2 * NT
F32, BF16, U32 = jnp.float32, jnp.bfloat16, jnp.uint32


def _consts():
    n1 = np.arange(N1)[None, None, :]
    k1 = np.arange(N1)[None, :, None]
    n2 = np.arange(N2)[:, None, None]
    ph = -2 * np.pi * (n1 * k1 / 128.0 + n2 * k1 / 2048.0) + np.pi * (16 * n1 + n2) / 4096.0
    Gr, Gi = np.cos(ph), np.sin(ph)
    G = np.stack([Gr.reshape(N2, 16, 8, N1), Gi.reshape(N2, 16, 8, N1)], axis=2).reshape(N2, 256, N1)
    Ginv = np.transpose(G, (0, 2, 1)) / 2048.0
    Pm = np.zeros((128, 128), np.float32)
    for n2_ in range(16):
        for a in range(8):
            Pm[n2_ * 8 + a, 16 * a + n2_] = 1.0
    return G.astype(np.float32), Ginv.astype(np.float32), Pm

_C1, _S1, _R = float(np.cos(np.pi / 8)), float(np.sin(np.pi / 8)), float(np.sqrt(0.5))


def _bfly4(x, sgn):
    (ar, ai), (br, bi), (cr, ci), (dr, di) = x
    t0r, t0i = ar + cr, ai + ci
    t1r, t1i = ar - cr, ai - ci
    t2r, t2i = br + dr, bi + di
    t3r, t3i = br - dr, bi - di
    x0 = (t0r + t2r, t0i + t2i)
    x2 = (t0r - t2r, t0i - t2i)
    if sgn < 0:
        x1 = (t1r + t3i, t1i - t3r)
        x3 = (t1r - t3i, t1i + t3r)
    else:
        x1 = (t1r - t3i, t1i + t3r)
        x3 = (t1r + t3i, t1i - t3r)
    return [x0, x1, x2, x3]


def _tw(z, e, sgn):
    a, b = z
    if e == 0:
        return z
    if sgn < 0:
        if e == 4: return (b, -a)
        if e == 2: return ((a + b) * _R, (b - a) * _R)
        if e == 6: return ((b - a) * _R, (a + b) * (-_R))
        if e == 1: return (a * _C1 + b * _S1, b * _C1 - a * _S1)
        if e == 3: return (a * _S1 + b * _C1, b * _S1 - a * _C1)
        if e == 9: return (a * (-_C1) - b * _S1, a * _S1 - b * _C1)
    else:
        if e == 4: return (-b, a)
        if e == 2: return ((a - b) * _R, (a + b) * _R)
        if e == 6: return ((a + b) * (-_R), (a - b) * _R)
        if e == 1: return (a * _C1 - b * _S1, b * _C1 + a * _S1)
        if e == 3: return (a * _S1 - b * _C1, b * _S1 + a * _C1)
        if e == 9: return (b * _S1 - a * _C1, a * (-_S1) - b * _C1)
    raise ValueError(e)


def fft16(x, sgn):
    A = [_bfly4([x[nb], x[nb + 4], x[nb + 8], x[nb + 12]], sgn) for nb in range(4)]
    B = [[_tw(A[nb][ka], nb * ka, sgn) for ka in range(4)] for nb in range(4)]
    X = [None] * 16
    for ka in range(4):
        o = _bfly4([B[0][ka], B[1][ka], B[2][ka], B[3][ka]], sgn)
        for kb in range(4):
            X[ka + 4 * kb] = o[kb]
    return X


def _unpack(w):
    lo = jax.lax.bitcast_convert_type(w << 16, F32)
    hi = jax.lax.bitcast_convert_type(w & jnp.uint32(0xFFFF0000), F32)
    return lo, hi


import os as _os2
_FLAGS = {k: True for k in _os2.environ.get('KFLAGS', '').split(',') if k} or None
NT_DIMS = (((1,), (1,)), ((), ()))


def kernel(q_hbm, ka_hbm, va_hbm, kb_hbm, vb_hbm, ha_hbm, hb_hbm, ska_ref, skb_ref,
           da_ref, db_ref, gw_ref, g_hbm, gi_hbm, pm_ref, o_hbm,
           qb, kb, vb, hb, gmat, gimat, ob, hp0, hp1, kvp0, kvp1, zh0, zh1, zu0, zu1, yp0, yp1, yb0, yb1, yb2, yb3, gnat, par, sems, osems):
    hp, kvp, zh, zu, yp, yb = (hp0, hp1), (kvp0, kvp1), (zh0, zh1), (zu0, zu1), (yp0, yp1), (yb0, yb1, yb2, yb3)
    k_hbm, v_hbm, h_hbm = (ka_hbm, kb_hbm), (va_hbm, vb_hbm), (ha_hbm, hb_hbm)

    def cp_k(p):
        return pltpu.make_async_copy(k_hbm[p % 2].at[0, :, pl.ds(128 * (p // 2), 128)], kb.at[p, pl.ds(16, S), :], sems.at[p])
    def cp_v(p):
        return pltpu.make_async_copy(v_hbm[p % 2].at[0, :, pl.ds(128 * (p // 2), 128)], vb.at[p], sems.at[NP + p])
    def cp_h(p):
        return pltpu.make_async_copy(h_hbm[p % 2].at[pl.ds(128 * (p // 2), 128), :], hb.at[p], sems.at[2 * NP + p])
    def cp_q(t):
        return pltpu.make_async_copy(q_hbm.at[0, :, pl.ds(128 * t, 128)], qb.at[t], sems.at[3 * NP + t])
    cp_g = pltpu.make_async_copy(g_hbm, gmat, sems.at[3 * NP + NT])
    cp_gi = pltpu.make_async_copy(gi_hbm, gimat, sems.at[3 * NP + NT + 1])
    def cp_o(t):
        return pltpu.make_async_copy(ob.at[t], o_hbm.at[0, :, pl.ds(128 * t, 128)], osems.at[t])

    cp_h(0).start(); cp_k(0).start(); cp_v(0).start(); cp_g.start()
    cp_h(1).start(); cp_k(1).start(); cp_v(1).start()

    for p in range(NP):
        kb[p, pl.ds(0, 16), :] = jnp.zeros((16, 128), BF16)
    sk = (jnp.transpose(ska_ref[...].astype(F32)), jnp.transpose(skb_ref[...].astype(F32)))
    dd = (da_ref[...].astype(F32).reshape(1, D), db_ref[...].astype(F32).reshape(1, D))
    for p in range(NP):
        b, t = p % 2, p // 2
        for tap in range(4):
            par[p, pl.ds(8 * tap, 8), :] = jnp.broadcast_to(sk[b][tap:tap + 1, 128 * t:128 * (t + 1)], (8, 128))
        par[p, pl.ds(32, 8), :] = jnp.broadcast_to(dd[b][:, 128 * t:128 * (t + 1)], (8, 128))

    kw, vw, qw, ow = kb.bitcast(U32), vb.bitcast(U32), qb.bitcast(U32), ob.bitcast(U32)

    def stage_T(p, jj):
        c0 = pl.multiple_of(jj * 256, 256)
        pm = pm_ref[...]
        R = [jax.lax.dot_general(pm, hb[p, :, pl.ds(c0 + 128 * u, 128)], NT_DIMS, preferred_element_type=F32)
             for u in range(2)]
        r0 = pl.multiple_of(jj * 16, 16)
        for n2 in range(16):
            blk = jnp.concatenate([R[0][8 * n2:8 * n2 + 8], R[1][8 * n2:8 * n2 + 8]], axis=0)
            hp[p % 2][n2, pl.ds(r0, 16), :] = blk.astype(BF16)

    def stage_P(p, a2):
        s = [jnp.concatenate([par[p, pl.ds(8 * tap, 8), :]] * 2, axis=0) for tap in range(4)]
        base = pl.multiple_of(a2 * 128, 128)
        ksub = kw.at[p, pl.ds(pl.multiple_of(base + 8, 8), 128), :]
        kprev = kw.at[p, pl.ds(base, 128), :]
        vsub = vw.at[p, pl.ds(base, 128), :]
        kk = {}
        for m in range(8):
            kk[2 * m], kk[2 * m + 1] = _unpack(ksub[pl.ds(m, 16, stride=8), :])
        for m in (6, 7):
            kk[2 * m - 16], kk[2 * m + 1 - 16] = _unpack(kprev[pl.ds(m, 16, stride=8), :])
        r0 = pl.multiple_of(a2 * 16, 16)
        for m in range(8):
            vlo, vhi = _unpack(vsub[pl.ds(m, 16, stride=8), :])
            for n2, vv in ((2 * m, vlo), (2 * m + 1, vhi)):
                acc = kk[n2] * s[0] + kk[n2 - 1] * s[1] + kk[n2 - 2] * s[2] + kk[n2 - 3] * s[3]
                kvp[p % 2][n2, pl.ds(r0, 16), :] = (acc * vv).astype(BF16)

    def stage_F(p, n2):
        g = gmat[n2]
        zh[p % 2][n2] = jnp.dot(g, hp[p % 2][n2], preferred_element_type=F32)
        zu[p % 2][n2] = jnp.dot(g, kvp[p % 2][n2], preferred_element_type=F32)

    def stage_V(p, g):
        r0 = pl.multiple_of(g * 16, 16)
        zhp, zup = zh[p % 2], zu[p % 2]
        x = [(zhp[n2, pl.ds(r0, 8), :], zhp[n2, pl.ds(r0 + 8, 8), :]) for n2 in range(16)]
        x[0] = (x[0][0] + par[p, pl.ds(32, 8), :], x[0][1])
        H = fft16(x, -1)
        for k2 in range(16):
            zhp[k2, pl.ds(r0, 8), :] = H[k2][0]
            zhp[k2, pl.ds(r0 + 8, 8), :] = H[k2][1]
        x = [(zup[n2, pl.ds(r0, 8), :], zup[n2, pl.ds(r0 + 8, 8), :]) for n2 in range(16)]
        U = fft16(x, -1)
        Y = []
        for k2 in range(16):
            hr, hi = zhp[k2, pl.ds(r0, 8), :], zhp[k2, pl.ds(r0 + 8, 8), :]
            ur, ui = U[k2]
            Y.append((ur * hr - ui * hi, ur * hi + ui * hr))
        T = fft16(Y, +1)
        for n2 in range(16):
            yp[p % 2][n2, pl.ds(r0, 16), :] = jnp.concatenate([T[n2][0], T[n2][1]], axis=0).astype(BF16)

    def stage_I(p, n2):
        yb[p % 4][n2] = jnp.dot(gimat[n2], yp[p % 2][n2], preferred_element_type=F32)

    def stage_B(t, a):
        pa, pb = (2 * t) % 4, (2 * t + 1) % 4
        r0 = pl.multiple_of(a * 8, 8)
        w0 = pl.multiple_of(a * 64, 64)
        qsub = qw.at[t, pl.ds(w0, 64), :]
        osub = ow.at[t, pl.ds(w0, 64), :]
        gsub = gnat.at[pl.ds(pl.multiple_of(a * 128, 128), 128), :]
        for m in range(8):
            qs = _unpack(qsub[pl.ds(m, 8, stride=8), :])
            res = []
            for u in range(2):
                n2 = 2 * m + u
                ya, yv = yb[pa][n2, pl.ds(r0, 8), :], yb[pb][n2, pl.ds(r0, 8), :]
                gg = gsub[pl.ds(n2, 8, stride=16), :]
                res.append(qs[u] * (yv + gg * (ya - yv)))
            osub[pl.ds(m, 8, stride=8), :] = pltpu.pack_elementwise((res[0], res[1]), packed_dtype=BF16)

    def gate():
        gw = gw_ref[...].reshape(1, D)
        gw8 = jnp.broadcast_to(gw, (8, D))
        for jt in range(S // 128):
            acc = None
            for t in range(NT):
                part = jax.lax.dot_general(gw8[:, 128 * t:128 * (t + 1)], qb[t, pl.ds(128 * jt, 128), :], NT_DIMS,
                                           preferred_element_type=F32)
                acc = part if acc is None else acc + part
            gs = jax.nn.sigmoid(acc)
            gnat[pl.ds(128 * jt, 128), :] = jnp.transpose(jnp.broadcast_to(gs[0:1, :], (128, 128)))

    GATE_SLOT = 5
    b_next = 0
    n_slots = NP + 5
    for s in range(n_slots):
        pT, pF, pV, pI = s, s - 1, s - 2, s - 3
        doT, doF, doV, doI = (0 <= pT < NP), (0 <= pF < NP), (0 <= pV < NP), (0 <= pI < NP)
        tB = None
        if b_next < NT and s >= 2 * b_next + 5 and s > GATE_SLOT:
            tB = b_next
            b_next += 1
        if s + 2 < NP:
            cp_h(s + 2).start(); cp_k(s + 2).start(); cp_v(s + 2).start()
        if s == 1:
            cp_gi.start()
        if s < NT:
            cp_q(s).start()
        if doT:
            cp_h(pT).wait(); cp_k(pT).wait(); cp_v(pT).wait()
        if s == 1:
            cp_g.wait()
        if s == 3:
            cp_gi.wait()
        if s == GATE_SLOT:
            for t in range(NT):
                cp_q(t).wait()
            gate()

        def body(i2, carry, pT=pT, pF=pF, pV=pV, pI=pI, doT=doT, doF=doF, doV=doV, doI=doI, tB=tB):
            import os as _o
            order = _o.environ.get("ORDER", "0")
            def F_(u):
                if doF: stage_F(pF, 2 * i2 + u)
            def I_(u):
                if doI: stage_I(pI, 2 * i2 + u)
            def V_(u):
                if doV: stage_V(pV, 2 * i2 + u)
            def B_(u):
                if tB is not None: stage_B(tB, 2 * i2 + u)
            def T_():
                if doT: stage_T(pT, i2)
            def P_():
                if doT: stage_P(pT, i2)
            if order == "0":
                F_(0); I_(0); V_(0); B_(0); F_(1); I_(1); V_(1); B_(1); T_(); P_()
            elif order == "1":
                V_(0); F_(0); I_(0); B_(0); V_(1); F_(1); I_(1); B_(1); T_(); P_()
            elif order == "2":
                P_(); V_(0); V_(1); B_(0); B_(1); F_(0); I_(0); F_(1); I_(1); T_()
            elif order == "3":
                F_(0); I_(0); T_(); V_(0); P_(); B_(0); F_(1); I_(1); V_(1); B_(1)
            return carry
        if doT or doF or doV or doI or tB is not None:
            jax.lax.fori_loop(0, 8, body, 0)
        if tB is not None:
            cp_o(tB).start()
    assert b_next == NT
    for t in range(NT):
        cp_o(t).wait()


def run(A_q, A_k, A_v, A_shift_k, A_ssm_k, A_ssm_D, B_q, B_k, B_v, B_shift_k, B_ssm_k, B_ssm_D, gate_w):
    G, Ginv, Pm = _consts()
    any_spec = pl.BlockSpec(memory_space=pl.ANY)
    vm = pl.BlockSpec(memory_space=pltpu.VMEM)
    return pl.pallas_call(
        kernel,
        in_specs=[any_spec] * 7 + [vm] * 5 + [any_spec, any_spec, vm],
        out_specs=any_spec,
        out_shape=jax.ShapeDtypeStruct((1, S, D), BF16),
        scratch_shapes=[
            pltpu.VMEM((NT, S, 128), BF16),
            pltpu.VMEM((NP, S + 16, 128), BF16),
            pltpu.VMEM((NP, S, 128), BF16),
            pltpu.VMEM((NP, 128, S), BF16),
            pltpu.VMEM((16, 256, 128), BF16),
            pltpu.VMEM((16, 128, 256), BF16),
            pltpu.VMEM((NT, S, 128), BF16),
            *[pltpu.VMEM((16, 128, 128), BF16)] * 4,
            *[pltpu.VMEM((16, 256, 128), F32)] * 4,
            *[pltpu.VMEM((16, 256, 128), BF16)] * 2,
            *[pltpu.VMEM((16, 128, 128), F32)] * 4,
            pltpu.VMEM((S, 128), F32),
            pltpu.VMEM((NP, 40, 128), F32),
            pltpu.SemaphoreType.DMA((3 * NP + NT + 2,)),
            pltpu.SemaphoreType.DMA((NT,)),
        ],
        compiler_params=pltpu.CompilerParams(vmem_limit_bytes=110 * 1024 * 1024, flags=_FLAGS),
    )(A_q, A_k, A_v, B_k, B_v, A_ssm_k, B_ssm_k, A_shift_k, B_shift_k, A_ssm_D, B_ssm_D, gate_w,
      jnp.asarray(G, BF16), jnp.asarray(Ginv, BF16), jnp.asarray(Pm, BF16))


@jax.jit
def pallas_gated_mix__ssm_conv_h3__ssm_conv_h3__prompt_kernel(
    A_q, A_k, A_v, A_shift_k, A_ssm_k, A_ssm_D, B_q, B_k, B_v, B_shift_k, B_ssm_k, B_ssm_D, gate_w,
):
    return run(A_q, A_k, A_v, A_shift_k, A_ssm_k, A_ssm_D, B_q, B_k, B_v, B_shift_k, B_ssm_k, B_ssm_D, gate_w)
```

```python
import functools
import numpy as np
import jax
import jax.numpy as jnp
from jax.experimental import pallas as pl
from jax.experimental.pallas import tpu as pltpu

S, D, N1, N2 = 2048, 640, 128, 16
NT = D // 128
NP = 2 * NT
F32, BF16, U32 = jnp.float32, jnp.bfloat16, jnp.uint32


def _pack_rows(m):
    u = np.ascontiguousarray(m, dtype=np.float32).view(np.uint32).astype(np.uint64)
    h = ((u + 0x7FFF + ((u >> 16) & 1)) >> 16).astype(np.uint32)
    return (h[0::2] | (h[1::2] << np.uint32(16))).astype(np.uint32)


def _consts():
    n1 = np.arange(N1)[None, None, :]
    k1 = np.arange(N1)[None, :, None]
    n2 = np.arange(N2)[:, None, None]
    ph = -2 * np.pi * (n1 * k1 / 128.0 + n2 * k1 / 2048.0) + np.pi * (16 * n1 + n2) / 4096.0
    Gr, Gi = np.cos(ph), np.sin(ph)
    G = np.stack([Gr.reshape(N2, 16, 8, N1), Gi.reshape(N2, 16, 8, N1)], axis=2).reshape(N2, 256, N1)
    Ginv = np.transpose(G, (0, 2, 1)) / 2048.0
    Pm = np.zeros((128, 128), np.float32)
    for n2_ in range(16):
        for a in range(8):
            Pm[n2_ * 8 + a, 16 * a + n2_] = 1.0
    Ginv = Ginv.reshape(N2, 128, 2, 128).transpose(0, 2, 1, 3)
    return _pack_rows(G.reshape(4096, 128)), _pack_rows(Ginv.reshape(4096, 128)), _pack_rows(Pm)

_C1, _S1, _R = float(np.cos(np.pi / 8)), float(np.sin(np.pi / 8)), float(np.sqrt(0.5))


def _bfly4(x, sgn):
    (ar, ai), (br, bi), (cr, ci), (dr, di) = x
    t0r, t0i = ar + cr, ai + ci
    t1r, t1i = ar - cr, ai - ci
    t2r, t2i = br + dr, bi + di
    t3r, t3i = br - dr, bi - di
    x0 = (t0r + t2r, t0i + t2i)
    x2 = (t0r - t2r, t0i - t2i)
    if sgn < 0:
        x1 = (t1r + t3i, t1i - t3r)
        x3 = (t1r - t3i, t1i + t3r)
    else:
        x1 = (t1r - t3i, t1i + t3r)
        x3 = (t1r + t3i, t1i - t3r)
    return [x0, x1, x2, x3]


def _tw(z, e, sgn):
    a, b = z
    if e == 0:
        return z
    if sgn < 0:
        if e == 4: return (b, -a)
        if e == 2: return ((a + b) * _R, (b - a) * _R)
        if e == 6: return ((b - a) * _R, (a + b) * (-_R))
        if e == 1: return (a * _C1 + b * _S1, b * _C1 - a * _S1)
        if e == 3: return (a * _S1 + b * _C1, b * _S1 - a * _C1)
        if e == 9: return (a * (-_C1) - b * _S1, a * _S1 - b * _C1)
    else:
        if e == 4: return (-b, a)
        if e == 2: return ((a - b) * _R, (a + b) * _R)
        if e == 6: return ((a + b) * (-_R), (a - b) * _R)
        if e == 1: return (a * _C1 - b * _S1, b * _C1 + a * _S1)
        if e == 3: return (a * _S1 - b * _C1, b * _S1 + a * _C1)
        if e == 9: return (b * _S1 - a * _C1, a * (-_S1) - b * _C1)
    raise ValueError(e)


def fft16(x, sgn):
    A = [_bfly4([x[nb], x[nb + 4], x[nb + 8], x[nb + 12]], sgn) for nb in range(4)]
    B = [[_tw(A[nb][ka], nb * ka, sgn) for ka in range(4)] for nb in range(4)]
    X = [None] * 16
    for ka in range(4):
        o = _bfly4([B[0][ka], B[1][ka], B[2][ka], B[3][ka]], sgn)
        for kb in range(4):
            X[ka + 4 * kb] = o[kb]
    return X


def _unpack(w):
    lo = jax.lax.bitcast_convert_type(w << 16, F32)
    hi = jax.lax.bitcast_convert_type(w & jnp.uint32(0xFFFF0000), F32)
    return lo, hi


import os as _os2
_FLAGS = {k: True for k in _os2.environ.get('KFLAGS', '').split(',') if k} or None
NT_DIMS = (((1,), (1,)), ((), ()))


import os as _os3
U = int(_os3.environ.get("U", "4"))
XZH, XZU, XHP, XKV, XYP, XYB, XROWS = 0, 4096, 8192, 9216, 10240, 12288, 16384


def kernel(off_ref, q_hbm, ka_hbm, va_hbm, kb_hbm, vb_hbm, ha_hbm, hb_hbm, ska_ref, skb_ref,
           da_ref, db_ref, gw_ref, g_hbm, gi_hbm, pmat, o_hbm,
           qb, kb, vb, hb, gmat, gimat, ob, zh0, zh1, zu0, zu1, hp0, hp1, kv0, kv1, yp0, yp1, yb0, yb1, yb2, yb3, ht, gnat, par, sems, osems):
    ZH, ZU, HP, KV, YP, YB = (zh0, zh1), (zu0, zu1), (hp0, hp1), (kv0, kv1), (yp0, yp1), (yb0, yb1, yb2, yb3)
    k_hbm, v_hbm, h_hbm = (ka_hbm, kb_hbm), (va_hbm, vb_hbm), (ha_hbm, hb_hbm)

    def cp_k(p):
        return pltpu.make_async_copy(k_hbm[p % 2].at[0, :, pl.ds(128 * (p // 2), 128)], kb.at[p, pl.ds(16, S), :], sems.at[p])
    def cp_v(p):
        return pltpu.make_async_copy(v_hbm[p % 2].at[0, :, pl.ds(128 * (p // 2), 128)], vb.at[p], sems.at[NP + p])
    def cp_h(p):
        return pltpu.make_async_copy(h_hbm[p % 2].at[pl.ds(128 * (p // 2), 128), :], hb.at[p], sems.at[2 * NP + p])
    def cp_q(t):
        return pltpu.make_async_copy(q_hbm.at[0, :, pl.ds(128 * t, 128)], qb.at[t], sems.at[3 * NP + t])
    cp_g = pltpu.make_async_copy(g_hbm, gmat, sems.at[3 * NP + NT])
    cp_gi = pltpu.make_async_copy(gi_hbm, gimat, sems.at[3 * NP + NT + 1])
    def cp_o(t):
        return pltpu.make_async_copy(ob.at[t], o_hbm.at[0, :, pl.ds(128 * t, 128)], osems.at[t])

    cp_h(0).start(); cp_k(0).start(); cp_v(0).start(); cp_g.start()
    cp_h(1).start(); cp_k(1).start(); cp_v(1).start()

    for p in range(NP):
        kb[p, pl.ds(0, 16), :] = jnp.zeros((16, 128), BF16)
    sk = (ska_ref[...].astype(F32), skb_ref[...].astype(F32))
    dd = (da_ref[...].astype(F32).reshape(1, D), db_ref[...].astype(F32).reshape(1, D))
    for p in range(NP):
        b, t = p % 2, p // 2
        for tap in range(4):
            par[p, pl.ds(8 * tap, 8), :] = jnp.broadcast_to(sk[b][tap:tap + 1, 128 * t:128 * (t + 1)], (8, 128))
        par[p, pl.ds(32, 8), :] = jnp.broadcast_to(dd[b][:, 128 * t:128 * (t + 1)], (8, 128))

    kw, vw, qw, ow = kb.bitcast(U32), vb.bitcast(U32), qb.bitcast(U32), ob.bitcast(U32)
    always = off_ref[0] == 0

    def ds(start, n, mult=None):
        if isinstance(start, int):
            return pl.ds(start, n)
        return pl.ds(pl.multiple_of(start, mult or n), n)

    def ldb(ref, w0, nrows):
        return pltpu.bitcast(ref[ds(w0, nrows // 2, 8), :], BF16)

    def pk(v):
        return pltpu.bitcast(v.astype(BF16), F32)

    def stage_TM(p, jj):
        r = jax.lax.broadcasted_iota(jnp.int32, (128, 128), 0)
        c = jax.lax.broadcasted_iota(jnp.int32, (128, 128), 1)
        pm = pmat[...]
        R = [jax.lax.dot_general(pltpu.bitcast(pm, BF16), hb[p, :, ds(jj * 256 + 128 * u, 128)], NT_DIMS, preferred_element_type=F32)
             for u in range(2)]
        hps = HP[p % 2].at[ds(jj * 8, 1024 - 56, 8), :]
        for n2 in range(16):
            hps[pl.ds(n2 * 64, 8), :] = pk(jnp.concatenate([R[0][8 * n2:8 * n2 + 8], R[1][8 * n2:8 * n2 + 8]], axis=0))

    def stage_T1(p, jj):
        for u in range(2):
            blk = hb[p, :, ds(jj * 256 + 128 * u, 128)].astype(F32)
            ht[pl.ds(128 * u, 128), :] = jnp.transpose(blk)

    def stage_T2(p, jj):
        hps = HP[p % 2].at[ds(jj * 8, 1024 - 56, 8), :]
        for n2 in range(16):
            hps[pl.ds(n2 * 64, 8), :] = pk(ht[pl.ds(n2, 16, stride=16), :])

    def stage_P(p, a2):
        s = [jnp.concatenate([par[p, pl.ds(8 * tap, 8), :]] * 2, axis=0) for tap in range(4)]
        base = a2 * 128
        ksub = kw.at[p, ds(base + 8, 128, 8), :]
        kprev = kw.at[p, ds(base, 128), :]
        vsub = vw.at[p, ds(base, 128), :]
        kk = {}
        def getk(n):
            if n not in kk:
                m = (n // 2) if n >= 0 else ((n + 16) // 2)
                lo, hi = _unpack((ksub if n >= 0 else kprev)[pl.ds(m, 16, stride=8), :])
                b0 = 2 * m if n >= 0 else 2 * m - 16
                kk[b0], kk[b0 + 1] = lo, hi
            return kk[n]
        kvs = KV[p % 2].at[ds(a2 * 8, 1024 - 56, 8), :]
        for m in range(8):
            vlo, vhi = _unpack(vsub[pl.ds(m, 16, stride=8), :])
            for n2, vv in ((2 * m, vlo), (2 * m + 1, vhi)):
                acc = getk(n2) * s[0] + getk(n2 - 1) * s[1] + getk(n2 - 2) * s[2] + getk(n2 - 3) * s[3]
                kvs[pl.ds(n2 * 64, 8), :] = pk(acc * vv)

    def stage_V(p, g):
        xh = ZH[p % 2].at[:, ds(g * 16, 16), :]
        xu = ZU[p % 2].at[:, ds(g * 16, 16), :]
        ys = YP[p % 2].at[ds(g * 8, 2048 - 120, 8), :]
        z = [(xh[n2, 0:8, :], xh[n2, 8:16, :]) for n2 in range(16)]
        z[0] = (z[0][0] + par[p, pl.ds(32, 8), :], z[0][1])
        H = fft16(z, -1)
        for k2 in range(16):
            xh[k2, 0:8, :] = H[k2][0]
            xh[k2, 8:16, :] = H[k2][1]
        z = [(xu[n2, 0:8, :], xu[n2, 8:16, :]) for n2 in range(16)]
        Uu = fft16(z, -1)
        Y = []
        for k2 in range(16):
            hr, hi = xh[k2, 0:8, :], xh[k2, 8:16, :]
            ur, ui = Uu[k2]
            Y.append((ur * hr - ui * hi, ur * hi + ui * hr))
        T = fft16(Y, +1)
        for n2 in range(16):
            ys[pl.ds(n2 * 128, 8), :] = pk(jnp.concatenate([T[n2][0], T[n2][1]], axis=0))

    def stage_B(t, a):
        ya_ref = YB[(2 * t) % 4].at[:, ds(a * 8, 8), :]
        yb_ref = YB[(2 * t + 1) % 4].at[:, ds(a * 8, 8), :]
        qsub = qw.at[t, ds(a * 64, 64), :]
        osub = ow.at[t, ds(a * 64, 64), :]
        gsub = gnat.at[ds(a * 128, 128), :]
        for m in range(8):
            qs = _unpack(qsub[pl.ds(m, 8, stride=8), :])
            res = []
            for u in range(2):
                n2 = 2 * m + u
                ya, yv = ya_ref[n2], yb_ref[n2]
                gg = gsub[pl.ds(n2, 8, stride=16), :]
                res.append(qs[u] * (yv + gg * (ya - yv)))
            osub[pl.ds(m, 8, stride=8), :] = pltpu.pack_elementwise((res[0], res[1]), packed_dtype=BF16)

    def gate():
        gw = gw_ref[...].reshape(1, D)
        gw8 = jnp.broadcast_to(gw, (8, D))
        for jt in range(S // 128):
            acc = None
            for t in range(NT):
                part = jax.lax.dot_general(gw8[:, 128 * t:128 * (t + 1)], qb[t, pl.ds(128 * jt, 128), :], NT_DIMS,
                                           preferred_element_type=F32)
                acc = part if acc is None else acc + part
            gs = jax.nn.sigmoid(acc)
            gnat[pl.ds(128 * jt, 128), :] = jnp.transpose(jnp.broadcast_to(gs[0:1, :], (128, 128)))

    GATE_SLOT = 5
    n_slots = NP + 5
    for s in range(n_slots):
        pT, pF, pV, pI = s, s - 1, s - 2, s - 3
        doT, doF, doV, doI = (0 <= pT < NP), (0 <= pF < NP), (0 <= pV < NP), (0 <= pI < NP)
        tB, hB = None, None
        if s >= 5 and (s - 5) // 2 < NT:
            tB, hB = (s - 5) // 2, (s - 5) % 2
        if s + 2 < NP:
            cp_h(s + 2).start(); cp_k(s + 2).start(); cp_v(s + 2).start()
        if s == 1:
            cp_gi.start()
        if s < NT:
            cp_q(s).start()
        if doT:
            cp_h(pT).wait(); cp_k(pT).wait(); cp_v(pT).wait()
        if s == 1:
            cp_g.wait()
        if s == 3:
            cp_gi.wait()
        if s == GATE_SLOT:
            for t in range(NT):
                cp_q(t).wait()
            gate()

        def body(j, carry, pT=pT, pF=pF, pV=pV, pI=pI, doT=doT, doF=doF, doV=doV, doI=doI, tB=tB, hB=hB):
            def common(i):
                if doF:
                    g = ldb(gmat, i * 128, 256)
                    ZU[pF % 2][i] = jnp.dot(g, ldb(KV[pF % 2], i * 64, 128), preferred_element_type=F32)
                    ZH[pF % 2][i] = jnp.dot(g, ldb(HP[pF % 2], i * 64, 128), preferred_element_type=F32)
                if doI:
                    lhs = jnp.concatenate([ldb(gimat, i * 128, 128), ldb(gimat, i * 128 + 64, 128)], axis=1)
                    YB[pI % 4][i] = jnp.dot(lhs, ldb(YP[pI % 2], i * 128, 256), preferred_element_type=F32)
                if doV:
                    stage_V(pV, i)
            BPOS = "A"
            common(2 * j)
            if doT:
                stage_P(pT, j)
            if tB is not None and BPOS == "A":
                stage_B(tB, hB * 8 + j)
            def second():
                common(2 * j + 1)
                if doT:
                    stage_TM(pT, j)
                if tB is not None and BPOS == "B":
                    stage_B(tB, hB * 8 + j)
            if doF or doI or doV:
                pl.when(always)(second)
            else:
                second()
            return carry
        if doT or doF or doV or doI or (tB is not None and True):
            jax.lax.fori_loop(0, 8, body, 0)
        if tB is not None and "A" == "sep":
            def bbody(j, c, tB=tB, hB=hB):
                stage_B(tB, hB * 8 + 2 * j)
                stage_B(tB, hB * 8 + 2 * j + 1)
                return c
            jax.lax.fori_loop(0, 4, bbody, 0)
        if tB is not None and hB == 1:
            cp_o(tB).start()
    for t in range(NT):
        cp_o(t).wait()


def run(A_q, A_k, A_v, A_shift_k, A_ssm_k, A_ssm_D, B_q, B_k, B_v, B_shift_k, B_ssm_k, B_ssm_D, gate_w):
    G, Ginv, Pm = _consts()
    offs = np.zeros((1,), np.int32)
    any_spec = pl.BlockSpec(memory_space=pl.ANY)
    vm = pl.BlockSpec(memory_space=pltpu.VMEM)
    return pl.pallas_call(
        kernel,
        in_specs=[pl.BlockSpec(memory_space=pltpu.SMEM)] + [any_spec] * 7 + [vm] * 5 + [any_spec, any_spec, vm],
        out_specs=any_spec,
        out_shape=jax.ShapeDtypeStruct((1, S, D), BF16),
        scratch_shapes=[
            pltpu.VMEM((NT, S, 128), BF16),
            pltpu.VMEM((NP, S + 16, 128), BF16),
            pltpu.VMEM((NP, S, 128), BF16),
            pltpu.VMEM((NP, 128, S), BF16),
            pltpu.VMEM((2048, 128), U32),
            pltpu.VMEM((2048, 128), U32),
            pltpu.VMEM((NT, S, 128), BF16),
            *[pltpu.VMEM((16, 256, 128), F32)] * 4,
            *[pltpu.VMEM((1024, 128), F32)] * 4,
            *[pltpu.VMEM((2048, 128), F32)] * 2,
            *[pltpu.VMEM((16, 128, 128), F32)] * 4,
            pltpu.VMEM((256, 128), F32),
            pltpu.VMEM((S, 128), F32),
            pltpu.VMEM((NP, 40, 128), F32),
            pltpu.SemaphoreType.DMA((3 * NP + NT + 2,)),
            pltpu.SemaphoreType.DMA((NT,)),
        ],
        compiler_params=pltpu.CompilerParams(vmem_limit_bytes=110 * 1024 * 1024, flags=_FLAGS),
    )(jnp.asarray(offs), A_q, A_k, A_v, B_k, B_v, A_ssm_k, B_ssm_k, A_shift_k.T, B_shift_k.T, A_ssm_D, B_ssm_D, gate_w,
      jnp.asarray(G), jnp.asarray(Ginv), jnp.asarray(Pm))


@jax.jit
def pallas_gated_mix__ssm_conv_h3__ssm_conv_h3__prompt_kernel(
    A_q, A_k, A_v, A_shift_k, A_ssm_k, A_ssm_D, B_q, B_k, B_v, B_shift_k, B_ssm_k, B_ssm_D, gate_w,
):
    return run(A_q, A_k, A_v, A_shift_k, A_ssm_k, A_ssm_D, B_q, B_k, B_v, B_shift_k, B_ssm_k, B_ssm_D, gate_w)
```

```python
import functools
import numpy as np
import jax
import jax.numpy as jnp
from jax.experimental import pallas as pl
from jax.experimental.pallas import tpu as pltpu

S, D, N1, N2 = 2048, 640, 128, 16
NT = D // 128
NP = 2 * NT
F32, BF16, U32 = jnp.float32, jnp.bfloat16, jnp.uint32


def _pack_rows(m):
    u = np.ascontiguousarray(m, dtype=np.float32).view(np.uint32).astype(np.uint64)
    h = ((u + 0x7FFF + ((u >> 16) & 1)) >> 16).astype(np.uint32)
    return (h[0::2] | (h[1::2] << np.uint32(16))).astype(np.uint32)


def _consts():
    n1 = np.arange(N1)[None, None, :]
    k1 = np.arange(N1)[None, :, None]
    n2 = np.arange(N2)[:, None, None]
    ph = -2 * np.pi * (n1 * k1 / 128.0 + n2 * k1 / 2048.0) + np.pi * (16 * n1 + n2) / 4096.0
    Gr, Gi = np.cos(ph), np.sin(ph)
    G = np.stack([Gr.reshape(N2, 16, 8, N1), Gi.reshape(N2, 16, 8, N1)], axis=2).reshape(N2, 256, N1)
    Ginv = np.transpose(G, (0, 2, 1)) / 2048.0
    Pm = np.zeros((128, 128), np.float32)
    for n2_ in range(16):
        for a in range(8):
            Pm[n2_ * 8 + a, 16 * a + n2_] = 1.0
    Ginv = Ginv.reshape(N2, 128, 2, 128).transpose(0, 2, 1, 3)
    return _pack_rows(G.reshape(4096, 128)), _pack_rows(Ginv.reshape(4096, 128)), _pack_rows(Pm)

_C1, _S1, _R = float(np.cos(np.pi / 8)), float(np.sin(np.pi / 8)), float(np.sqrt(0.5))


def _bfly4(x, sgn):
    (ar, ai), (br, bi), (cr, ci), (dr, di) = x
    t0r, t0i = ar + cr, ai + ci
    t1r, t1i = ar - cr, ai - ci
    t2r, t2i = br + dr, bi + di
    t3r, t3i = br - dr, bi - di
    x0 = (t0r + t2r, t0i + t2i)
    x2 = (t0r - t2r, t0i - t2i)
    if sgn < 0:
        x1 = (t1r + t3i, t1i - t3r)
        x3 = (t1r - t3i, t1i + t3r)
    else:
        x1 = (t1r - t3i, t1i + t3r)
        x3 = (t1r + t3i, t1i - t3r)
    return [x0, x1, x2, x3]


def _tw(z, e, sgn):
    a, b = z
    if e == 0:
        return z
    if sgn < 0:
        if e == 4: return (b, -a)
        if e == 2: return ((a + b) * _R, (b - a) * _R)
        if e == 6: return ((b - a) * _R, (a + b) * (-_R))
        if e == 1: return (a * _C1 + b * _S1, b * _C1 - a * _S1)
        if e == 3: return (a * _S1 + b * _C1, b * _S1 - a * _C1)
        if e == 9: return (a * (-_C1) - b * _S1, a * _S1 - b * _C1)
    else:
        if e == 4: return (-b, a)
        if e == 2: return ((a - b) * _R, (a + b) * _R)
        if e == 6: return ((a + b) * (-_R), (a - b) * _R)
        if e == 1: return (a * _C1 - b * _S1, b * _C1 + a * _S1)
        if e == 3: return (a * _S1 - b * _C1, b * _S1 + a * _C1)
        if e == 9: return (b * _S1 - a * _C1, a * (-_S1) - b * _C1)
    raise ValueError(e)


def fft16(x, sgn):
    A = [_bfly4([x[nb], x[nb + 4], x[nb + 8], x[nb + 12]], sgn) for nb in range(4)]
    B = [[_tw(A[nb][ka], nb * ka, sgn) for ka in range(4)] for nb in range(4)]
    X = [None] * 16
    for ka in range(4):
        o = _bfly4([B[0][ka], B[1][ka], B[2][ka], B[3][ka]], sgn)
        for kb in range(4):
            X[ka + 4 * kb] = o[kb]
    return X


def _unpack(w):
    lo = jax.lax.bitcast_convert_type(w << 16, F32)
    hi = jax.lax.bitcast_convert_type(w & jnp.uint32(0xFFFF0000), F32)
    return lo, hi


import os as _os2
_FLAGS = {k: True for k in _os2.environ.get('KFLAGS', '').split(',') if k} or None
NT_DIMS = (((1,), (1,)), ((), ()))


import os as _os3

XZH, XZU, XHP, XKV, XYP, XYB, XROWS = 0, 4096, 8192, 9216, 10240, 12288, 16384


def kernel(off_ref, q_hbm, ka_hbm, va_hbm, kb_hbm, vb_hbm, ha_hbm, hb_hbm, ska_ref, skb_ref,
           da_ref, db_ref, gw_ref, g_hbm, gi_hbm, pmat, o_hbm,
           qb, kb, vb, hb, gmat, gimat, ob, zh0, zh1, zu0, zu1, hp0, hp1, kv0, kv1, yp0, yp1, yb0, yb1, yb2, yb3, hh, htf, gnat, par, sems, osems):
    ZH, ZU, HP, KV, YP, YB = (zh0, zh1), (zu0, zu1), (hp0, hp1), (kv0, kv1), (yp0, yp1), (yb0, yb1, yb2, yb3)
    k_hbm, v_hbm, h_hbm = (ka_hbm, kb_hbm), (va_hbm, vb_hbm), (ha_hbm, hb_hbm)

    def cp_k(p):
        return pltpu.make_async_copy(k_hbm[p % 2].at[0, :, pl.ds(128 * (p // 2), 128)], kb.at[p, pl.ds(16, S), :], sems.at[p])
    def cp_v(p):
        return pltpu.make_async_copy(v_hbm[p % 2].at[0, :, pl.ds(128 * (p // 2), 128)], vb.at[p], sems.at[NP + p])
    def cp_h(p):
        return pltpu.make_async_copy(h_hbm[p % 2].at[pl.ds(128 * (p // 2), 128), :], hb.at[p], sems.at[2 * NP + p])
    def cp_q(t):
        return pltpu.make_async_copy(q_hbm.at[0, :, pl.ds(128 * t, 128)], qb.at[t], sems.at[3 * NP + t])
    cp_g = pltpu.make_async_copy(g_hbm, gmat, sems.at[3 * NP + NT])
    cp_gi = pltpu.make_async_copy(gi_hbm, gimat, sems.at[3 * NP + NT + 1])
    def cp_o(t):
        return pltpu.make_async_copy(ob.at[t], o_hbm.at[0, :, pl.ds(128 * t, 128)], osems.at[t])

    cp_h(0).start(); cp_k(0).start(); cp_v(0).start()

    for p in range(NP):
        kb[p, pl.ds(0, 16), :] = jnp.zeros((16, 128), BF16)
    sk = (ska_ref[...].astype(F32), skb_ref[...].astype(F32))
    dd = (da_ref[...].astype(F32).reshape(1, D), db_ref[...].astype(F32).reshape(1, D))
    for p in range(NP):
        b, t = p % 2, p // 2
        for tap in range(4):
            par[p, pl.ds(8 * tap, 8), :] = jnp.broadcast_to(sk[b][tap:tap + 1, 128 * t:128 * (t + 1)], (8, 128))
        par[p, pl.ds(32, 8), :] = jnp.broadcast_to(dd[b][:, 128 * t:128 * (t + 1)], (8, 128))

    kw, vw, qw, ow = kb.bitcast(U32), vb.bitcast(U32), qb.bitcast(U32), ob.bitcast(U32)
    always = off_ref[0] == 0

    def ds(start, n, mult=None):
        if isinstance(start, int):
            return pl.ds(start, n)
        return pl.ds(pl.multiple_of(start, mult or n), n)

    def ldb(ref, w0, nrows):
        return pltpu.bitcast(ref[ds(w0, nrows // 2, 8), :], BF16)

    def pk(v):
        return pltpu.bitcast(v.astype(BF16), F32)

    def stage_TM(p, jj):
        r = jax.lax.broadcasted_iota(jnp.int32, (128, 128), 0)
        c = jax.lax.broadcasted_iota(jnp.int32, (128, 128), 1)
        pm = pmat[...]
        R = [jax.lax.dot_general(pltpu.bitcast(pm, BF16), hb[p, :, ds(jj * 256 + 128 * u, 128)], NT_DIMS, preferred_element_type=F32)
             for u in range(2)]
        hps = HP[p % 2].at[ds(jj * 8, 1024 - 56, 8), :]
        for n2 in range(16):
            hps[pl.ds(n2 * 64, 8), :] = pk(jnp.concatenate([R[0][8 * n2:8 * n2 + 8], R[1][8 * n2:8 * n2 + 8]], axis=0))

    def stage_Tall(p):
        if True:
            pm = pltpu.bitcast(pmat[...], BF16)
            for jj in range(8):
                R = [jax.lax.dot_general(pm, hb[p, :, pl.ds(jj * 256 + 128 * u, 128)], NT_DIMS,
                                         preferred_element_type=F32) for u in range(2)]
                for n2 in range(16):
                    HP[p % 2][pl.ds(jj * 8 + n2 * 64, 8), :] = pk(
                        jnp.concatenate([R[0][8 * n2:8 * n2 + 8], R[1][8 * n2:8 * n2 + 8]], axis=0))
        else:
            for jt in range(16):
                htf[pl.ds(128 * jt, 128), :] = jnp.transpose(hb[p, :, pl.ds(128 * jt, 128)].astype(F32))
            for jj in range(8):
                for n2 in range(16):
                    HP[p % 2][pl.ds(jj * 8 + n2 * 64, 8), :] = pk(htf[pl.ds(256 * jj + n2, 16, stride=16), :])

    def stage_T1(p, jj):
        for u in range(2):
            blk = hb[p, :, ds(jj * 256 + 128 * u, 128)].astype(F32)
            ht[pl.ds(128 * u, 128), :] = jnp.transpose(blk)

    def stage_T2(p, jj):
        hps = HP[p % 2].at[ds(jj * 8, 1024 - 56, 8), :]
        for n2 in range(16):
            hps[pl.ds(n2 * 64, 8), :] = pk(ht[pl.ds(n2, 16, stride=16), :])

    def stage_P(p, a2, ms=range(8)):
        s = [jnp.concatenate([par[p, pl.ds(8 * tap, 8), :]] * 2, axis=0) for tap in range(4)]
        base = a2 * 128
        ksub = kw.at[p, ds(base + 8, 128, 8), :]
        kprev = kw.at[p, ds(base, 128), :]
        vsub = vw.at[p, ds(base, 128), :]
        kk = {}
        def getk(n):
            if n not in kk:
                m = (n // 2) if n >= 0 else ((n + 16) // 2)
                lo, hi = _unpack((ksub if n >= 0 else kprev)[pl.ds(m, 16, stride=8), :])
                b0 = 2 * m if n >= 0 else 2 * m - 16
                kk[b0], kk[b0 + 1] = lo, hi
            return kk[n]
        kvs = KV[p % 2].at[ds(a2 * 8, 1024 - 56, 8), :]
        for m in ms:
            vlo, vhi = _unpack(vsub[pl.ds(m, 16, stride=8), :])
            for n2, vv in ((2 * m, vlo), (2 * m + 1, vhi)):
                acc = getk(n2) * s[0] + getk(n2 - 1) * s[1] + getk(n2 - 2) * s[2] + getk(n2 - 3) * s[3]
                kvs[pl.ds(n2 * 64, 8), :] = pk(acc * vv)

    def stage_V(p, g):
        xh = ZH[p % 2].at[:, ds(g * 16, 16), :]
        xu = ZU[p % 2].at[:, ds(g * 16, 16), :]
        xo = hh.at[:, ds(g * 16, 16), :]
        ys = YP[p % 2].at[ds(g * 8, 2048 - 120, 8), :]
        z = [(xh[n2, 0:8, :], xh[n2, 8:16, :]) for n2 in range(16)]
        z[0] = (z[0][0] + par[p, pl.ds(32, 8), :], z[0][1])
        H = fft16(z, -1)
        for k2 in range(16):
            xo[k2, 0:8, :] = H[k2][0]
            xo[k2, 8:16, :] = H[k2][1]
        z = [(xu[n2, 0:8, :], xu[n2, 8:16, :]) for n2 in range(16)]
        Uu = fft16(z, -1)
        Y = []
        for k2 in range(16):
            hr, hi = xo[k2, 0:8, :], xo[k2, 8:16, :]
            ur, ui = Uu[k2]
            Y.append((ur * hr - ui * hi, ur * hi + ui * hr))
        T = fft16(Y, +1)
        for n2 in range(16):
            ys[pl.ds(n2 * 128, 8), :] = pk(jnp.concatenate([T[n2][0], T[n2][1]], axis=0))

    def stage_B(t, a):
        ya_ref = YB[(2 * t) % 4].at[:, ds(a * 8, 8), :]
        yb_ref = YB[(2 * t + 1) % 4].at[:, ds(a * 8, 8), :]
        qsub = qw.at[t, ds(a * 64, 64), :]
        osub = ow.at[t, ds(a * 64, 64), :]
        gsub = gnat.at[ds(a * 128, 128), :]
        for m in range(8):
            qs = _unpack(qsub[pl.ds(m, 8, stride=8), :])
            res = []
            for u in range(2):
                n2 = 2 * m + u
                ya, yv = ya_ref[n2], yb_ref[n2]
                gg = gsub[pl.ds(n2, 8, stride=16), :]
                res.append(qs[u] * (yv + gg * (ya - yv)))
            osub[pl.ds(m, 8, stride=8), :] = pltpu.pack_elementwise((res[0], res[1]), packed_dtype=BF16)

    def gate():
        gw = gw_ref[...].reshape(1, D)
        gw8 = jnp.broadcast_to(gw, (8, D))
        for jt in range(S // 128):
            acc = None
            for t in range(NT):
                part = jax.lax.dot_general(gw8[:, 128 * t:128 * (t + 1)], qb[t, pl.ds(128 * jt, 128), :], NT_DIMS,
                                           preferred_element_type=F32)
                acc = part if acc is None else acc + part
            gs = jax.nn.sigmoid(acc)
            gnat[pl.ds(128 * jt, 128), :] = jnp.transpose(jnp.broadcast_to(gs[0:1, :], (128, 128)))

    GATE_SLOT = 5
    n_slots = NP + 5
    for s in range(n_slots):
        pT, pF, pV, pI = s, s - 1, s - 2, s - 3
        doT, doF, doV, doI = (0 <= pT < NP), (0 <= pF < NP), (0 <= pV < NP), (0 <= pI < NP)
        tB, hB = None, None
        if s >= 5 and (s - 5) // 2 < NT:
            tB, hB = (s - 5) // 2, (s - 5) % 2
        if s == 1:
            cp_g.wait()
        if s == 3:
            cp_gi.wait()
        if s == GATE_SLOT:
            for t in range(NT):
                cp_q(t).wait()
            gate()
        if doT:
            cp_h(pT).wait()
            stage_Tall(pT)
        if s == 0:
            cp_g.start()
            cp_h(1).start(); cp_k(1).start(); cp_v(1).start()
        if s + 2 < NP:
            cp_h(s + 2).start(); cp_k(s + 2).start(); cp_v(s + 2).start()
        if s == 1:
            cp_gi.start()
        if s < NT:
            cp_q(s).start()
        if doT:
            cp_k(pT).wait(); cp_v(pT).wait()

        def dot_F(p, i):
            g = ldb(gmat, i * 128, 256)
            ZU[p % 2][i] = jnp.dot(g, ldb(KV[p % 2], i * 64, 128), preferred_element_type=F32)
            ZH[p % 2][i] = jnp.dot(g, ldb(HP[p % 2], i * 64, 128), preferred_element_type=F32)

        def dot_I(p, i):
            lhs = jnp.concatenate([ldb(gimat, i * 128, 128), ldb(gimat, i * 128 + 64, 128)], axis=1)
            YB[p % 4][i] = jnp.dot(lhs, ldb(YP[p % 2], i * 128, 256), preferred_element_type=F32)

        if not doV and (doF or doI):
            for i in range(16):
                if doF:
                    dot_F(pF, i)
                if doI:
                    dot_I(pI, i)
            doF = doI = False

        def body(j, carry, pT=pT, pF=pF, pV=pV, pI=pI, doT=doT, doF=doF, doV=doV, doI=doI, tB=tB, hB=hB):
            def common(i):
                if doV:
                    stage_V(pV, i)
                if doF:
                    dot_F(pF, i)
                if doI:
                    dot_I(pI, i)
            BPOS = "B"
            common(2 * j)
            if doT:
                stage_P(pT, j, range(8))
            if tB is not None and BPOS == "A":
                stage_B(tB, hB * 8 + j)
            def second():
                common(2 * j + 1)
                if False:
                    stage_P(pT, j, range(4, 8))
                if tB is not None and BPOS == "B":
                    stage_B(tB, hB * 8 + j)
            if doF or doI or doV:
                pl.when(always)(second)
            else:
                second()
            return carry
        if doT or doF or doV or doI or (tB is not None and True):
            jax.lax.fori_loop(0, 8, body, 0)
        if tB is not None and "A" == "sep":
            def bbody(j, c, tB=tB, hB=hB):
                stage_B(tB, hB * 8 + 2 * j)
                stage_B(tB, hB * 8 + 2 * j + 1)
                return c
            jax.lax.fori_loop(0, 4, bbody, 0)
        if tB is not None and hB == 1:
            cp_o(tB).start()
    for t in range(NT):
        cp_o(t).wait()


def run(A_q, A_k, A_v, A_shift_k, A_ssm_k, A_ssm_D, B_q, B_k, B_v, B_shift_k, B_ssm_k, B_ssm_D, gate_w):
    G, Ginv, Pm = _consts()
    offs = np.zeros((1,), np.int32)
    any_spec = pl.BlockSpec(memory_space=pl.ANY)
    vm = pl.BlockSpec(memory_space=pltpu.VMEM)
    return pl.pallas_call(
        kernel,
        in_specs=[pl.BlockSpec(memory_space=pltpu.SMEM)] + [any_spec] * 7 + [vm] * 5 + [any_spec, any_spec, vm],
        out_specs=any_spec,
        out_shape=jax.ShapeDtypeStruct((1, S, D), BF16),
        scratch_shapes=[
            pltpu.VMEM((NT, S, 128), BF16),
            pltpu.VMEM((NP, S + 16, 128), BF16),
            pltpu.VMEM((NP, S, 128), BF16),
            pltpu.VMEM((NP, 128, S), BF16),
            pltpu.VMEM((2048, 128), U32),
            pltpu.VMEM((2048, 128), U32),
            pltpu.VMEM((NT, S, 128), BF16),
            *[pltpu.VMEM((16, 256, 128), F32)] * 4,
            *[pltpu.VMEM((1024, 128), F32)] * 4,
            *[pltpu.VMEM((2048, 128), F32)] * 2,
            *[pltpu.VMEM((16, 128, 128), F32)] * 4,
            pltpu.VMEM((16, 256, 128), F32),
            pltpu.VMEM((S, 128), F32),
            pltpu.VMEM((S, 128), F32),
            pltpu.VMEM((NP, 40, 128), F32),
            pltpu.SemaphoreType.DMA((3 * NP + NT + 2,)),
            pltpu.SemaphoreType.DMA((NT,)),
        ],
        compiler_params=pltpu.CompilerParams(vmem_limit_bytes=110 * 1024 * 1024, flags=_FLAGS),
    )(jnp.asarray(offs), A_q, A_k, A_v, B_k, B_v, A_ssm_k, B_ssm_k, A_shift_k.T, B_shift_k.T, A_ssm_D, B_ssm_D, gate_w,
      jnp.asarray(G), jnp.asarray(Ginv), jnp.asarray(Pm))


@jax.jit
def pallas_gated_mix__ssm_conv_h3__ssm_conv_h3__prompt_kernel(
    A_q, A_k, A_v, A_shift_k, A_ssm_k, A_ssm_D, B_q, B_k, B_v, B_shift_k, B_ssm_k, B_ssm_D, gate_w,
):
    return run(A_q, A_k, A_v, A_shift_k, A_ssm_k, A_ssm_D, B_q, B_k, B_v, B_shift_k, B_ssm_k, B_ssm_D, gate_w)
```

```python
import functools
import numpy as np
import jax
import jax.numpy as jnp
from jax.experimental import pallas as pl
from jax.experimental.pallas import tpu as pltpu

S, D, N1, N2 = 2048, 640, 128, 16
NT = D // 128
NP = 2 * NT
F32, BF16, U32 = jnp.float32, jnp.bfloat16, jnp.uint32


def _pack_rows(m):
    u = np.ascontiguousarray(m, dtype=np.float32).view(np.uint32).astype(np.uint64)
    h = ((u + 0x7FFF + ((u >> 16) & 1)) >> 16).astype(np.uint32)
    return (h[0::2] | (h[1::2] << np.uint32(16))).astype(np.uint32)


def _consts():
    n1 = np.arange(N1)[None, None, :]
    k1 = np.arange(N1)[None, :, None]
    n2 = np.arange(N2)[:, None, None]
    ph = -2 * np.pi * (n1 * k1 / 128.0 + n2 * k1 / 2048.0) + np.pi * (16 * n1 + n2) / 4096.0
    Gr, Gi = np.cos(ph), np.sin(ph)
    G = np.stack([Gr.reshape(N2, 16, 8, N1), Gi.reshape(N2, 16, 8, N1)], axis=2).reshape(N2, 256, N1)
    Ginv = np.transpose(G, (0, 2, 1)) / 2048.0
    Pm = np.zeros((128, 128), np.float32)
    for n2_ in range(16):
        for a in range(8):
            Pm[n2_ * 8 + a, 16 * a + n2_] = 1.0
    Ginv = Ginv.reshape(N2, 128, 2, 128).transpose(0, 2, 1, 3)
    return _pack_rows(G.reshape(4096, 128)), _pack_rows(Ginv.reshape(4096, 128)), _pack_rows(Pm)

_C1, _S1, _R = float(np.cos(np.pi / 8)), float(np.sin(np.pi / 8)), float(np.sqrt(0.5))


def _bfly4(x, sgn):
    (ar, ai), (br, bi), (cr, ci), (dr, di) = x
    t0r, t0i = ar + cr, ai + ci
    t1r, t1i = ar - cr, ai - ci
    t2r, t2i = br + dr, bi + di
    t3r, t3i = br - dr, bi - di
    x0 = (t0r + t2r, t0i + t2i)
    x2 = (t0r - t2r, t0i - t2i)
    if sgn < 0:
        x1 = (t1r + t3i, t1i - t3r)
        x3 = (t1r - t3i, t1i + t3r)
    else:
        x1 = (t1r - t3i, t1i + t3r)
        x3 = (t1r + t3i, t1i - t3r)
    return [x0, x1, x2, x3]


def _tw(z, e, sgn):
    a, b = z
    if e == 0:
        return z
    if sgn < 0:
        if e == 4: return (b, -a)
        if e == 2: return ((a + b) * _R, (b - a) * _R)
        if e == 6: return ((b - a) * _R, (a + b) * (-_R))
        if e == 1: return (a * _C1 + b * _S1, b * _C1 - a * _S1)
        if e == 3: return (a * _S1 + b * _C1, b * _S1 - a * _C1)
        if e == 9: return (a * (-_C1) - b * _S1, a * _S1 - b * _C1)
    else:
        if e == 4: return (-b, a)
        if e == 2: return ((a - b) * _R, (a + b) * _R)
        if e == 6: return ((a + b) * (-_R), (a - b) * _R)
        if e == 1: return (a * _C1 - b * _S1, b * _C1 + a * _S1)
        if e == 3: return (a * _S1 - b * _C1, b * _S1 + a * _C1)
        if e == 9: return (b * _S1 - a * _C1, a * (-_S1) - b * _C1)
    raise ValueError(e)


def fft16(x, sgn):
    A = [_bfly4([x[nb], x[nb + 4], x[nb + 8], x[nb + 12]], sgn) for nb in range(4)]
    B = [[_tw(A[nb][ka], nb * ka, sgn) for ka in range(4)] for nb in range(4)]
    X = [None] * 16
    for ka in range(4):
        o = _bfly4([B[0][ka], B[1][ka], B[2][ka], B[3][ka]], sgn)
        for kb in range(4):
            X[ka + 4 * kb] = o[kb]
    return X


def _unpack(w):
    lo = jax.lax.bitcast_convert_type(w << 16, F32)
    hi = jax.lax.bitcast_convert_type(w & jnp.uint32(0xFFFF0000), F32)
    return lo, hi


import os as _os2
_FLAGS = {k: True for k in _os2.environ.get('KFLAGS', '').split(',') if k} or None
NT_DIMS = (((1,), (1,)), ((), ()))


import os as _os3

XZH, XZU, XHP, XKV, XYP, XYB, XROWS = 0, 4096, 8192, 9216, 10240, 12288, 16384


def kernel(off_ref, q_hbm, ka_hbm, va_hbm, kb_hbm, vb_hbm, ha_hbm, hb_hbm, ska_ref, skb_ref,
           da_ref, db_ref, gw_ref, g_hbm, gi_hbm, pmat, o_hbm,
           qb, kb, vb, hb, gmat, gimat, ob, zh0, zh1, zu0, zu1, hp0, hp1, kv0, kv1, yp0, yp1, yb0, yb1, yb2, yb3, hh, htf, gnat, par, sems, osems):
    ZH, ZU, HP, KV, YP, YB = (zh0, zh1), (zu0, zu1), (hp0, hp1), (kv0, kv1), (yp0, yp1), (yb0, yb1, yb2, yb3)
    k_hbm, v_hbm, h_hbm = (ka_hbm, kb_hbm), (va_hbm, vb_hbm), (ha_hbm, hb_hbm)

    def cp_k(p):
        return pltpu.make_async_copy(k_hbm[p % 2].at[0, :, pl.ds(128 * (p // 2), 128)], kb.at[p, pl.ds(16, S), :], sems.at[p])
    def cp_v(p):
        return pltpu.make_async_copy(v_hbm[p % 2].at[0, :, pl.ds(128 * (p // 2), 128)], vb.at[p], sems.at[NP + p])
    def cp_h(p):
        return pltpu.make_async_copy(h_hbm[p % 2].at[pl.ds(128 * (p // 2), 128), :], hb.at[p], sems.at[2 * NP + p])
    def cp_q(t):
        return pltpu.make_async_copy(q_hbm.at[0, :, pl.ds(128 * t, 128)], qb.at[t], sems.at[3 * NP + t])
    cp_g = pltpu.make_async_copy(g_hbm, gmat, sems.at[3 * NP + NT])
    cp_gi = pltpu.make_async_copy(gi_hbm, gimat, sems.at[3 * NP + NT + 1])
    def cp_o(t, hf):
        rows = pl.ds(hf * (S // 2), S // 2)
        return pltpu.make_async_copy(ob.at[t, rows, :], o_hbm.at[0, rows, pl.ds(128 * t, 128)], osems.at[2 * t + hf])

    cp_h(0).start(); cp_k(0).start(); cp_v(0).start(); cp_g.start()
    cp_h(1).start(); cp_k(1).start(); cp_v(1).start()

    for p in range(NP):
        kb[p, pl.ds(0, 16), :] = jnp.zeros((16, 128), BF16)
    sk = (ska_ref[...].astype(F32), skb_ref[...].astype(F32))
    dd = (da_ref[...].astype(F32).reshape(1, D), db_ref[...].astype(F32).reshape(1, D))
    for p in range(NP):
        b, t = p % 2, p // 2
        for tap in range(4):
            par[p, pl.ds(8 * tap, 8), :] = jnp.broadcast_to(sk[b][tap:tap + 1, 128 * t:128 * (t + 1)], (8, 128))
        par[p, pl.ds(32, 8), :] = jnp.broadcast_to(dd[b][:, 128 * t:128 * (t + 1)], (8, 128))

    kw, vw, qw, ow = kb.bitcast(U32), vb.bitcast(U32), qb.bitcast(U32), ob.bitcast(U32)
    always = off_ref[0] == 0

    def ds(start, n, mult=None):
        if isinstance(start, int):
            return pl.ds(start, n)
        return pl.ds(pl.multiple_of(start, mult or n), n)

    def ldb(ref, w0, nrows):
        return pltpu.bitcast(ref[ds(w0, nrows // 2, 8), :], BF16)

    def pk(v):
        return pltpu.bitcast(v.astype(BF16), F32)

    def stage_TM(p, jj):
        r = jax.lax.broadcasted_iota(jnp.int32, (128, 128), 0)
        c = jax.lax.broadcasted_iota(jnp.int32, (128, 128), 1)
        pm = pmat[...]
        R = [jax.lax.dot_general(pltpu.bitcast(pm, BF16), hb[p, :, ds(jj * 256 + 128 * u, 128)], NT_DIMS, preferred_element_type=F32)
             for u in range(2)]
        hps = HP[p % 2].at[ds(jj * 8, 1024 - 56, 8), :]
        for n2 in range(16):
            hps[pl.ds(n2 * 64, 8), :] = pk(jnp.concatenate([R[0][8 * n2:8 * n2 + 8], R[1][8 * n2:8 * n2 + 8]], axis=0))

    def stage_Tall(p):
        if True:
            pm = pltpu.bitcast(pmat[...], BF16)
            for jj in range(8):
                R = [jax.lax.dot_general(pm, hb[p, :, pl.ds(jj * 256 + 128 * u, 128)], NT_DIMS,
                                         preferred_element_type=F32) for u in range(2)]
                for n2 in range(16):
                    HP[p % 2][pl.ds(jj * 8 + n2 * 64, 8), :] = pk(
                        jnp.concatenate([R[0][8 * n2:8 * n2 + 8], R[1][8 * n2:8 * n2 + 8]], axis=0))
        else:
            for jt in range(16):
                htf[pl.ds(128 * jt, 128), :] = jnp.transpose(hb[p, :, pl.ds(128 * jt, 128)].astype(F32))
            for jj in range(8):
                for n2 in range(16):
                    HP[p % 2][pl.ds(jj * 8 + n2 * 64, 8), :] = pk(htf[pl.ds(256 * jj + n2, 16, stride=16), :])

    def stage_T1(p, jj):
        for u in range(2):
            blk = hb[p, :, ds(jj * 256 + 128 * u, 128)].astype(F32)
            ht[pl.ds(128 * u, 128), :] = jnp.transpose(blk)

    def stage_T2(p, jj):
        hps = HP[p % 2].at[ds(jj * 8, 1024 - 56, 8), :]
        for n2 in range(16):
            hps[pl.ds(n2 * 64, 8), :] = pk(ht[pl.ds(n2, 16, stride=16), :])

    def stage_P(p, a2, ms=range(8)):
        s = [jnp.concatenate([par[p, pl.ds(8 * tap, 8), :]] * 2, axis=0) for tap in range(4)]
        base = a2 * 128
        ksub = kw.at[p, ds(base + 8, 128, 8), :]
        kprev = kw.at[p, ds(base, 128), :]
        vsub = vw.at[p, ds(base, 128), :]
        kk = {}
        def getk(n):
            if n not in kk:
                m = (n // 2) if n >= 0 else ((n + 16) // 2)
                lo, hi = _unpack((ksub if n >= 0 else kprev)[pl.ds(m, 16, stride=8), :])
                b0 = 2 * m if n >= 0 else 2 * m - 16
                kk[b0], kk[b0 + 1] = lo, hi
            return kk[n]
        kvs = KV[p % 2].at[ds(a2 * 8, 1024 - 56, 8), :]
        for m in ms:
            vlo, vhi = _unpack(vsub[pl.ds(m, 16, stride=8), :])
            for n2, vv in ((2 * m, vlo), (2 * m + 1, vhi)):
                acc = getk(n2) * s[0] + getk(n2 - 1) * s[1] + getk(n2 - 2) * s[2] + getk(n2 - 3) * s[3]
                kvs[pl.ds(n2 * 64, 8), :] = pk(acc * vv)

    def stage_V(p, g):
        xh = ZH[p % 2].at[:, ds(g * 16, 16), :]
        xu = ZU[p % 2].at[:, ds(g * 16, 16), :]
        xo = hh.at[:, ds(g * 16, 16), :]
        ys = YP[p % 2].at[ds(g * 8, 2048 - 120, 8), :]
        z = [(xh[n2, 0:8, :], xh[n2, 8:16, :]) for n2 in range(16)]
        z[0] = (z[0][0] + par[p, pl.ds(32, 8), :], z[0][1])
        H = fft16(z, -1)
        for k2 in range(16):
            xo[k2, 0:8, :] = H[k2][0]
            xo[k2, 8:16, :] = H[k2][1]
        z = [(xu[n2, 0:8, :], xu[n2, 8:16, :]) for n2 in range(16)]
        Uu = fft16(z, -1)
        Y = []
        for k2 in range(16):
            hr, hi = xo[k2, 0:8, :], xo[k2, 8:16, :]
            ur, ui = Uu[k2]
            Y.append((ur * hr - ui * hi, ur * hi + ui * hr))
        T = fft16(Y, +1)
        for n2 in range(16):
            ys[pl.ds(n2 * 128, 8), :] = pk(jnp.concatenate([T[n2][0], T[n2][1]], axis=0))

    def stage_B(t, a):
        ya_ref = YB[(2 * t) % 4].at[:, ds(a * 8, 8), :]
        yb_ref = YB[(2 * t + 1) % 4].at[:, ds(a * 8, 8), :]
        qsub = qw.at[t, ds(a * 64, 64), :]
        osub = ow.at[t, ds(a * 64, 64), :]
        gsub = gnat.at[ds(a * 128, 128), :]
        for m in range(8):
            qs = _unpack(qsub[pl.ds(m, 8, stride=8), :])
            res = []
            for u in range(2):
                n2 = 2 * m + u
                ya, yv = ya_ref[n2], yb_ref[n2]
                gg = gsub[pl.ds(n2, 8, stride=16), :]
                res.append(qs[u] * (yv + gg * (ya - yv)))
            osub[pl.ds(m, 8, stride=8), :] = pltpu.pack_elementwise((res[0], res[1]), packed_dtype=BF16)

    def gate():
        gw = gw_ref[...].reshape(1, D)
        gw8 = jnp.broadcast_to(gw, (8, D))
        for jt in range(S // 128):
            acc = None
            for t in range(NT):
                part = jax.lax.dot_general(gw8[:, 128 * t:128 * (t + 1)], qb[t, pl.ds(128 * jt, 128), :], NT_DIMS,
                                           preferred_element_type=F32)
                acc = part if acc is None else acc + part
            gs = jax.nn.sigmoid(acc)
            gnat[pl.ds(128 * jt, 128), :] = jnp.transpose(jnp.broadcast_to(gs[0:1, :], (128, 128)))

    GATE_SLOT = 5
    n_slots = NP + 5
    for s in range(n_slots):
        pT, pF, pV, pI = s, s - 1, s - 2, s - 3
        doT, doF, doV, doI = (0 <= pT < NP), (0 <= pF < NP), (0 <= pV < NP), (0 <= pI < NP)
        tB, hB = None, None
        if s >= 5 and (s - 5) // 2 < NT:
            tB, hB = (s - 5) // 2, (s - 5) % 2
        if s + 2 < NP:
            cp_h(s + 2).start(); cp_k(s + 2).start(); cp_v(s + 2).start()
        if s == 1:
            cp_gi.start()
        if s < NT:
            cp_q(s).start()
        if s == 1:
            with jax.named_scope('gwait'):
                cp_g.wait()
        if s == 3:
            cp_gi.wait()
        if s == GATE_SLOT:
            for t in range(NT):
                cp_q(t).wait()
            gate()
        def dot_F(p, i):
            g = ldb(gmat, i * 128, 256)
            ZU[p % 2][i] = jnp.dot(g, ldb(KV[p % 2], i * 64, 128), preferred_element_type=F32)
            ZH[p % 2][i] = jnp.dot(g, ldb(HP[p % 2], i * 64, 128), preferred_element_type=F32)

        def dot_I(p, i):
            lhs = jnp.concatenate([ldb(gimat, i * 128, 128), ldb(gimat, i * 128 + 64, 128)], axis=1)
            YB[p % 4][i] = jnp.dot(lhs, ldb(YP[p % 2], i * 128, 256), preferred_element_type=F32)

        if not doV and (doF or doI):
            with jax.named_scope(f's{s:02d}_mxu'):
              for i in range(16):
                if doF:
                    dot_F(pF, i)
                if doI:
                    dot_I(pI, i)
            doF = doI = False

        if doT:
            with jax.named_scope(f's{s:02d}_hwait'):
                cp_h(pT).wait()
            with jax.named_scope(f's{s:02d}_T'):
                stage_Tall(pT)
        if doT:
            with jax.named_scope(f's{s:02d}_kvwait'):
                cp_k(pT).wait(); cp_v(pT).wait()

        def body(j, carry, pT=pT, pF=pF, pV=pV, pI=pI, doT=doT, doF=doF, doV=doV, doI=doI, tB=tB, hB=hB):
            def common(i):
                if doV:
                    stage_V(pV, i)
                if doF:
                    dot_F(pF, i)
                if doI:
                    dot_I(pI, i)
            BPOS = "B"
            common(2 * j)
            if doT:
                stage_P(pT, j, range(8))
            if tB is not None and BPOS == "A":
                stage_B(tB, hB * 8 + j)
            def second():
                common(2 * j + 1)
                if False:
                    stage_P(pT, j, range(4, 8))
                if tB is not None and BPOS == "B":
                    stage_B(tB, hB * 8 + j)
            if doF or doI or doV:
                pl.when(always)(second)
            else:
                second()
            return carry
        if doT or doF or doV or doI or (tB is not None and True):
            with jax.named_scope(f's{s:02d}_loop'):
                jax.lax.fori_loop(0, 8, body, 0)
        if tB is not None and "A" == "sep":
            def bbody(j, c, tB=tB, hB=hB):
                stage_B(tB, hB * 8 + 2 * j)
                stage_B(tB, hB * 8 + 2 * j + 1)
                return c
            jax.lax.fori_loop(0, 4, bbody, 0)
        if tB is not None:
            cp_o(tB, hB).start()
    with jax.named_scope('owait'):
        for t in range(NT):
            cp_o(t, 0).wait(); cp_o(t, 1).wait()


def run(A_q, A_k, A_v, A_shift_k, A_ssm_k, A_ssm_D, B_q, B_k, B_v, B_shift_k, B_ssm_k, B_ssm_D, gate_w):
    G, Ginv, Pm = _consts()
    offs = np.zeros((1,), np.int32)
    any_spec = pl.BlockSpec(memory_space=pl.ANY)
    vm = pl.BlockSpec(memory_space=pltpu.VMEM)
    return pl.pallas_call(
        kernel,
        in_specs=[pl.BlockSpec(memory_space=pltpu.SMEM)] + [any_spec] * 7 + [vm] * 5 + [any_spec, any_spec, vm],
        out_specs=any_spec,
        out_shape=jax.ShapeDtypeStruct((1, S, D), BF16),
        scratch_shapes=[
            pltpu.VMEM((NT, S, 128), BF16),
            pltpu.VMEM((NP, S + 16, 128), BF16),
            pltpu.VMEM((NP, S, 128), BF16),
            pltpu.VMEM((NP, 128, S), BF16),
            pltpu.VMEM((2048, 128), U32),
            pltpu.VMEM((2048, 128), U32),
            pltpu.VMEM((NT, S, 128), BF16),
            *[pltpu.VMEM((16, 256, 128), F32)] * 4,
            *[pltpu.VMEM((1024, 128), F32)] * 4,
            *[pltpu.VMEM((2048, 128), F32)] * 2,
            *[pltpu.VMEM((16, 128, 128), F32)] * 4,
            pltpu.VMEM((16, 256, 128), F32),
            pltpu.VMEM((S, 128), F32),
            pltpu.VMEM((S, 128), F32),
            pltpu.VMEM((NP, 40, 128), F32),
            pltpu.SemaphoreType.DMA((3 * NP + NT + 2,)),
            pltpu.SemaphoreType.DMA((2 * NT,)),
        ],
        compiler_params=pltpu.CompilerParams(vmem_limit_bytes=110 * 1024 * 1024, flags=_FLAGS),
    )(jnp.asarray(offs), A_q, A_k, A_v, B_k, B_v, A_ssm_k, B_ssm_k, A_shift_k.T, B_shift_k.T, A_ssm_D, B_ssm_D, gate_w,
      jnp.asarray(G), jnp.asarray(Ginv), jnp.asarray(Pm))


@jax.jit
def pallas_gated_mix__ssm_conv_h3__ssm_conv_h3__prompt_kernel(
    A_q, A_k, A_v, A_shift_k, A_ssm_k, A_ssm_D, B_q, B_k, B_v, B_shift_k, B_ssm_k, B_ssm_D, gate_w,
):
    return run(A_q, A_k, A_v, A_shift_k, A_ssm_k, A_ssm_D, B_q, B_k, B_v, B_shift_k, B_ssm_k, B_ssm_D, gate_w)
```

```python
import functools
import numpy as np
import jax
import jax.numpy as jnp
from jax.experimental import pallas as pl
from jax.experimental.pallas import tpu as pltpu

S, D, N1, N2 = 2048, 640, 128, 16
NT = D // 128
NP = 2 * NT
F32, BF16, U32 = jnp.float32, jnp.bfloat16, jnp.uint32


def _pack_rows(m):
    u = np.ascontiguousarray(m, dtype=np.float32).view(np.uint32).astype(np.uint64)
    h = ((u + 0x7FFF + ((u >> 16) & 1)) >> 16).astype(np.uint32)
    return (h[0::2] | (h[1::2] << np.uint32(16))).astype(np.uint32)


def _consts():
    n1 = np.arange(N1)[None, None, :]
    k1 = np.arange(N1)[None, :, None]
    n2 = np.arange(N2)[:, None, None]
    ph = -2 * np.pi * (n1 * k1 / 128.0 + n2 * k1 / 2048.0) + np.pi * (16 * n1 + n2) / 4096.0
    Gr, Gi = np.cos(ph), np.sin(ph)
    G = np.stack([Gr.reshape(N2, 16, 8, N1), Gi.reshape(N2, 16, 8, N1)], axis=2).reshape(N2, 256, N1)
    Ginv = np.transpose(G, (0, 2, 1)) / 2048.0
    Pm = np.zeros((128, 128), np.float32)
    for n2_ in range(16):
        for a in range(8):
            Pm[n2_ * 8 + a, 16 * a + n2_] = 1.0
    Ginv = Ginv.reshape(N2, 128, 2, 128).transpose(0, 2, 1, 3)
    ph0 = -2 * np.pi * (n1[0] * k1[0] / 128.0) + np.pi * (16 * n1[0]) / 4096.0
    g0 = np.concatenate([np.cos(ph0), np.sin(ph0)], axis=0).astype(np.float32)
    phe = -2 * np.pi * np.arange(N1) / 2048.0 + np.pi / 4096.0
    e1 = np.zeros((128, 128), np.float32)
    e1[:, 0], e1[:, 1] = np.cos(phe), np.sin(phe)
    return g0, e1, _pack_rows(Ginv.reshape(4096, 128)), _pack_rows(Pm)

_C1, _S1, _R = float(np.cos(np.pi / 8)), float(np.sin(np.pi / 8)), float(np.sqrt(0.5))


def _bfly4(x, sgn):
    (ar, ai), (br, bi), (cr, ci), (dr, di) = x
    t0r, t0i = ar + cr, ai + ci
    t1r, t1i = ar - cr, ai - ci
    t2r, t2i = br + dr, bi + di
    t3r, t3i = br - dr, bi - di
    x0 = (t0r + t2r, t0i + t2i)
    x2 = (t0r - t2r, t0i - t2i)
    if sgn < 0:
        x1 = (t1r + t3i, t1i - t3r)
        x3 = (t1r - t3i, t1i + t3r)
    else:
        x1 = (t1r - t3i, t1i + t3r)
        x3 = (t1r + t3i, t1i - t3r)
    return [x0, x1, x2, x3]


def _tw(z, e, sgn):
    a, b = z
    if e == 0:
        return z
    if sgn < 0:
        if e == 4: return (b, -a)
        if e == 2: return ((a + b) * _R, (b - a) * _R)
        if e == 6: return ((b - a) * _R, (a + b) * (-_R))
        if e == 1: return (a * _C1 + b * _S1, b * _C1 - a * _S1)
        if e == 3: return (a * _S1 + b * _C1, b * _S1 - a * _C1)
        if e == 9: return (a * (-_C1) - b * _S1, a * _S1 - b * _C1)
    else:
        if e == 4: return (-b, a)
        if e == 2: return ((a - b) * _R, (a + b) * _R)
        if e == 6: return ((a + b) * (-_R), (a - b) * _R)
        if e == 1: return (a * _C1 - b * _S1, b * _C1 + a * _S1)
        if e == 3: return (a * _S1 - b * _C1, b * _S1 + a * _C1)
        if e == 9: return (b * _S1 - a * _C1, a * (-_S1) - b * _C1)
    raise ValueError(e)


def fft16(x, sgn):
    A = [_bfly4([x[nb], x[nb + 4], x[nb + 8], x[nb + 12]], sgn) for nb in range(4)]
    B = [[_tw(A[nb][ka], nb * ka, sgn) for ka in range(4)] for nb in range(4)]
    X = [None] * 16
    for ka in range(4):
        o = _bfly4([B[0][ka], B[1][ka], B[2][ka], B[3][ka]], sgn)
        for kb in range(4):
            X[ka + 4 * kb] = o[kb]
    return X


def _unpack(w):
    lo = jax.lax.bitcast_convert_type(w << 16, F32)
    hi = jax.lax.bitcast_convert_type(w & jnp.uint32(0xFFFF0000), F32)
    return lo, hi


import os as _os2
_FLAGS = {k: True for k in _os2.environ.get('KFLAGS', '').split(',') if k} or None
NT_DIMS = (((1,), (1,)), ((), ()))


import os as _os3

XZH, XZU, XHP, XKV, XYP, XYB, XROWS = 0, 4096, 8192, 9216, 10240, 12288, 16384


def kernel(off_ref, q_hbm, ka_hbm, va_hbm, kb_hbm, vb_hbm, ha_hbm, hb_hbm, ska_ref, skb_ref,
           da_ref, db_ref, gw_ref, g0_ref, e1_ref, gi_hbm, pmat, o_hbm,
           qb, kb, vb, hb, gmat, gimat, ob, zh0, zh1, zu0, zu1, hp0, hp1, kv0, kv1, yp0, yp1, yb0, yb1, yb2, yb3, hh, htf, gnat, par, sems, osems):
    ZH, ZU, HP, KV, YP, YB = (zh0, zh1), (zu0, zu1), (hp0, hp1), (kv0, kv1), (yp0, yp1), (yb0, yb1, yb2, yb3)
    k_hbm, v_hbm, h_hbm = (ka_hbm, kb_hbm), (va_hbm, vb_hbm), (ha_hbm, hb_hbm)

    def cp_k(p):
        return pltpu.make_async_copy(k_hbm[p % 2].at[0, :, pl.ds(128 * (p // 2), 128)], kb.at[p, pl.ds(16, S), :], sems.at[p])
    def cp_v(p):
        return pltpu.make_async_copy(v_hbm[p % 2].at[0, :, pl.ds(128 * (p // 2), 128)], vb.at[p], sems.at[NP + p])
    def cp_h(p):
        return pltpu.make_async_copy(h_hbm[p % 2].at[pl.ds(128 * (p // 2), 128), :], hb.at[p], sems.at[2 * NP + p])
    def cp_q(t):
        return pltpu.make_async_copy(q_hbm.at[0, :, pl.ds(128 * t, 128)], qb.at[t], sems.at[3 * NP + t])
    cp_gi = pltpu.make_async_copy(gi_hbm, gimat, sems.at[3 * NP + NT])
    def cp_o(t, hf):
        rows = pl.ds(hf * (S // 2), S // 2)
        return pltpu.make_async_copy(ob.at[t, rows, :], o_hbm.at[0, rows, pl.ds(128 * t, 128)], osems.at[2 * t + hf])

    cp_h(0).start(); cp_k(0).start(); cp_v(0).start();
    cp_h(1).start(); cp_k(1).start(); cp_v(1).start()

    for p in range(NP):
        kb[p, pl.ds(0, 16), :] = jnp.zeros((16, 128), BF16)
    sk = (ska_ref[...].astype(F32), skb_ref[...].astype(F32))
    dd = (da_ref[...].astype(F32).reshape(1, D), db_ref[...].astype(F32).reshape(1, D))
    for p in range(NP):
        b, t = p % 2, p // 2
        for tap in range(4):
            par[p, pl.ds(8 * tap, 8), :] = jnp.broadcast_to(sk[b][tap:tap + 1, 128 * t:128 * (t + 1)], (8, 128))
        par[p, pl.ds(32, 8), :] = jnp.broadcast_to(dd[b][:, 128 * t:128 * (t + 1)], (8, 128))

    kw, vw, qw, ow = kb.bitcast(U32), vb.bitcast(U32), qb.bitcast(U32), ob.bitcast(U32)
    always = off_ref[0] == 0

    def ds(start, n, mult=None):
        if isinstance(start, int):
            return pl.ds(start, n)
        return pl.ds(pl.multiple_of(start, mult or n), n)

    def ldb(ref, w0, nrows):
        return pltpu.bitcast(ref[ds(w0, nrows // 2, 8), :], BF16)

    def pk(v):
        return pltpu.bitcast(v.astype(BF16), F32)

    def stage_TM(p, jj):
        r = jax.lax.broadcasted_iota(jnp.int32, (128, 128), 0)
        c = jax.lax.broadcasted_iota(jnp.int32, (128, 128), 1)
        pm = pmat[...]
        R = [jax.lax.dot_general(pltpu.bitcast(pm, BF16), hb[p, :, ds(jj * 256 + 128 * u, 128)], NT_DIMS, preferred_element_type=F32)
             for u in range(2)]
        hps = HP[p % 2].at[ds(jj * 8, 1024 - 56, 8), :]
        for n2 in range(16):
            hps[pl.ds(n2 * 64, 8), :] = pk(jnp.concatenate([R[0][8 * n2:8 * n2 + 8], R[1][8 * n2:8 * n2 + 8]], axis=0))

    def stage_Tall(p):
        if True:
            pm = pltpu.bitcast(pmat[...], BF16)
            for jj in range(8):
                R = [jax.lax.dot_general(pm, hb[p, :, pl.ds(jj * 256 + 128 * u, 128)], NT_DIMS,
                                         preferred_element_type=F32) for u in range(2)]
                for n2 in range(16):
                    HP[p % 2][pl.ds(jj * 8 + n2 * 64, 8), :] = pk(
                        jnp.concatenate([R[0][8 * n2:8 * n2 + 8], R[1][8 * n2:8 * n2 + 8]], axis=0))
        else:
            for jt in range(16):
                htf[pl.ds(128 * jt, 128), :] = jnp.transpose(hb[p, :, pl.ds(128 * jt, 128)].astype(F32))
            for jj in range(8):
                for n2 in range(16):
                    HP[p % 2][pl.ds(jj * 8 + n2 * 64, 8), :] = pk(htf[pl.ds(256 * jj + n2, 16, stride=16), :])

    def stage_T1(p, jj):
        for u in range(2):
            blk = hb[p, :, ds(jj * 256 + 128 * u, 128)].astype(F32)
            ht[pl.ds(128 * u, 128), :] = jnp.transpose(blk)

    def stage_T2(p, jj):
        hps = HP[p % 2].at[ds(jj * 8, 1024 - 56, 8), :]
        for n2 in range(16):
            hps[pl.ds(n2 * 64, 8), :] = pk(ht[pl.ds(n2, 16, stride=16), :])

    def stage_P(p, a2, ms=range(8)):
        s = [jnp.concatenate([par[p, pl.ds(8 * tap, 8), :]] * 2, axis=0) for tap in range(4)]
        base = a2 * 128
        ksub = kw.at[p, ds(base + 8, 128, 8), :]
        kprev = kw.at[p, ds(base, 128), :]
        vsub = vw.at[p, ds(base, 128), :]
        kk = {}
        def getk(n):
            if n not in kk:
                m = (n // 2) if n >= 0 else ((n + 16) // 2)
                lo, hi = _unpack((ksub if n >= 0 else kprev)[pl.ds(m, 16, stride=8), :])
                b0 = 2 * m if n >= 0 else 2 * m - 16
                kk[b0], kk[b0 + 1] = lo, hi
            return kk[n]
        kvs = KV[p % 2].at[ds(a2 * 8, 1024 - 56, 8), :]
        for m in ms:
            vlo, vhi = _unpack(vsub[pl.ds(m, 16, stride=8), :])
            for n2, vv in ((2 * m, vlo), (2 * m + 1, vhi)):
                acc = getk(n2) * s[0] + getk(n2 - 1) * s[1] + getk(n2 - 2) * s[2] + getk(n2 - 3) * s[3]
                kvs[pl.ds(n2 * 64, 8), :] = pk(acc * vv)

    def stage_V(p, g):
        xh = ZH[p % 2].at[:, ds(g * 16, 16), :]
        xu = ZU[p % 2].at[:, ds(g * 16, 16), :]
        xo = hh.at[:, ds(g * 16, 16), :]
        ys = YP[p % 2].at[ds(g * 8, 2048 - 120, 8), :]
        z = [(xh[n2, 0:8, :], xh[n2, 8:16, :]) for n2 in range(16)]
        z[0] = (z[0][0] + par[p, pl.ds(32, 8), :], z[0][1])
        H = fft16(z, -1)
        for k2 in range(16):
            xo[k2, 0:8, :] = H[k2][0]
            xo[k2, 8:16, :] = H[k2][1]
        z = [(xu[n2, 0:8, :], xu[n2, 8:16, :]) for n2 in range(16)]
        Uu = fft16(z, -1)
        Y = []
        for k2 in range(16):
            hr, hi = xo[k2, 0:8, :], xo[k2, 8:16, :]
            ur, ui = Uu[k2]
            Y.append((ur * hr - ui * hi, ur * hi + ui * hr))
        T = fft16(Y, +1)
        for n2 in range(16):
            ys[pl.ds(n2 * 128, 8), :] = pk(jnp.concatenate([T[n2][0], T[n2][1]], axis=0))

    def stage_B(t, a):
        ya_ref = YB[(2 * t) % 4].at[:, ds(a * 8, 8), :]
        yb_ref = YB[(2 * t + 1) % 4].at[:, ds(a * 8, 8), :]
        qsub = qw.at[t, ds(a * 64, 64), :]
        osub = ow.at[t, ds(a * 64, 64), :]
        gsub = gnat.at[ds(a * 128, 128), :]
        for m in range(8):
            qs = _unpack(qsub[pl.ds(m, 8, stride=8), :])
            res = []
            for u in range(2):
                n2 = 2 * m + u
                ya, yv = ya_ref[n2], yb_ref[n2]
                gg = gsub[pl.ds(n2, 8, stride=16), :]
                res.append(qs[u] * (yv + gg * (ya - yv)))
            osub[pl.ds(m, 8, stride=8), :] = pltpu.pack_elementwise((res[0], res[1]), packed_dtype=BF16)

    def gate():
        gw = gw_ref[...].reshape(1, D)
        gw8 = jnp.broadcast_to(gw, (8, D))
        for jt in range(S // 128):
            acc = None
            for t in range(NT):
                part = jax.lax.dot_general(gw8[:, 128 * t:128 * (t + 1)], qb[t, pl.ds(128 * jt, 128), :], NT_DIMS,
                                           preferred_element_type=F32)
                acc = part if acc is None else acc + part
            gs = jax.nn.sigmoid(acc)
            gnat[pl.ds(128 * jt, 128), :] = jnp.transpose(jnp.broadcast_to(gs[0:1, :], (128, 128)))

    def gen_g(g, carry):
        r = ds(g * 8, 8)
        gr, gi = g0_ref[r, :], g0_ref[ds(128 + g * 8, 8), :]
        e = e1_ref[r, :]
        er, ei = jnp.broadcast_to(e[:, 0:1], (8, 128)), jnp.broadcast_to(e[:, 1:2], (8, 128))
        dst = gmat.at[ds(g * 8, 2048 - 120, 8), :]
        for n2 in range(16):
            dst[pl.ds(n2 * 128, 8), :] = pltpu.bitcast(jnp.concatenate([gr, gi], axis=0).astype(BF16), U32)
            if n2 < 15:
                gr, gi = gr * er - gi * ei, gr * ei + gi * er
        return carry
    jax.lax.fori_loop(0, 16, gen_g, 0)

    GATE_SLOT = 5
    n_slots = NP + 5
    for s in range(n_slots):
        pT, pF, pV, pI = s, s - 1, s - 2, s - 3
        doT, doF, doV, doI = (0 <= pT < NP), (0 <= pF < NP), (0 <= pV < NP), (0 <= pI < NP)
        tB, hB = None, None
        if s >= 5 and (s - 5) // 2 < NT:
            tB, hB = (s - 5) // 2, (s - 5) % 2
        if s + 2 < NP:
            cp_h(s + 2).start(); cp_k(s + 2).start(); cp_v(s + 2).start()
        if s == 1:
            cp_gi.start()
        if s < NT:
            cp_q(s).start()
        if s == 3:
            cp_gi.wait()
        if s == GATE_SLOT:
            for t in range(NT):
                cp_q(t).wait()
            gate()
        def dot_F(p, i):
            g = ldb(gmat, i * 128, 256)
            ZU[p % 2][i] = jnp.dot(g, ldb(KV[p % 2], i * 64, 128), preferred_element_type=F32)
            ZH[p % 2][i] = jnp.dot(g, ldb(HP[p % 2], i * 64, 128), preferred_element_type=F32)

        def dot_I(p, i):
            lhs = jnp.concatenate([ldb(gimat, i * 128, 128), ldb(gimat, i * 128 + 64, 128)], axis=1)
            YB[p % 4][i] = jnp.dot(lhs, ldb(YP[p % 2], i * 128, 256), preferred_element_type=F32)

        if not doV and (doF or doI):
            with jax.named_scope(f's{s:02d}_mxu'):
              for i in range(16):
                if doF:
                    dot_F(pF, i)
                if doI:
                    dot_I(pI, i)
            doF = doI = False

        if doT:
            with jax.named_scope(f's{s:02d}_hwait'):
                cp_h(pT).wait()
            with jax.named_scope(f's{s:02d}_T'):
                stage_Tall(pT)
        if doT:
            with jax.named_scope(f's{s:02d}_kvwait'):
                cp_k(pT).wait(); cp_v(pT).wait()

        def body(j, carry, pT=pT, pF=pF, pV=pV, pI=pI, doT=doT, doF=doF, doV=doV, doI=doI, tB=tB, hB=hB):
            def common(i):
                if doV:
                    stage_V(pV, i)
                if doF:
                    dot_F(pF, i)
                if doI:
                    dot_I(pI, i)
            BPOS = "B"
            common(2 * j)
            if doT:
                stage_P(pT, j, range(8))
            if tB is not None and BPOS == "A":
                stage_B(tB, hB * 8 + j)
            def second():
                common(2 * j + 1)
                if False:
                    stage_P(pT, j, range(4, 8))
                if tB is not None and BPOS == "B":
                    stage_B(tB, hB * 8 + j)
            if doF or doI or doV:
                pl.when(always)(second)
            else:
                second()
            return carry
        if doT or doF or doV or doI or (tB is not None and True):
            with jax.named_scope(f's{s:02d}_loop'):
                jax.lax.fori_loop(0, 8, body, 0)
        if tB is not None and "A" == "sep":
            def bbody(j, c, tB=tB, hB=hB):
                stage_B(tB, hB * 8 + 2 * j)
                stage_B(tB, hB * 8 + 2 * j + 1)
                return c
            jax.lax.fori_loop(0, 4, bbody, 0)
        if tB is not None:
            cp_o(tB, hB).start()
    with jax.named_scope('owait'):
        for t in range(NT):
            cp_o(t, 0).wait(); cp_o(t, 1).wait()


def run(A_q, A_k, A_v, A_shift_k, A_ssm_k, A_ssm_D, B_q, B_k, B_v, B_shift_k, B_ssm_k, B_ssm_D, gate_w):
    G0, E1, Ginv, Pm = _consts()
    offs = np.zeros((1,), np.int32)
    any_spec = pl.BlockSpec(memory_space=pl.ANY)
    vm = pl.BlockSpec(memory_space=pltpu.VMEM)
    return pl.pallas_call(
        kernel,
        in_specs=[pl.BlockSpec(memory_space=pltpu.SMEM)] + [any_spec] * 7 + [vm] * 7 + [any_spec, vm],
        out_specs=any_spec,
        out_shape=jax.ShapeDtypeStruct((1, S, D), BF16),
        scratch_shapes=[
            pltpu.VMEM((NT, S, 128), BF16),
            pltpu.VMEM((NP, S + 16, 128), BF16),
            pltpu.VMEM((NP, S, 128), BF16),
            pltpu.VMEM((NP, 128, S), BF16),
            pltpu.VMEM((2048, 128), U32),
            pltpu.VMEM((2048, 128), U32),
            pltpu.VMEM((NT, S, 128), BF16),
            *[pltpu.VMEM((16, 256, 128), F32)] * 4,
            *[pltpu.VMEM((1024, 128), F32)] * 4,
            *[pltpu.VMEM((2048, 128), F32)] * 2,
            *[pltpu.VMEM((16, 128, 128), F32)] * 4,
            pltpu.VMEM((16, 256, 128), F32),
            pltpu.VMEM((S, 128), F32),
            pltpu.VMEM((S, 128), F32),
            pltpu.VMEM((NP, 40, 128), F32),
            pltpu.SemaphoreType.DMA((3 * NP + NT + 1,)),
            pltpu.SemaphoreType.DMA((2 * NT,)),
        ],
        compiler_params=pltpu.CompilerParams(vmem_limit_bytes=110 * 1024 * 1024, flags=_FLAGS),
    )(jnp.asarray(offs), A_q, A_k, A_v, B_k, B_v, A_ssm_k, B_ssm_k, A_shift_k.T, B_shift_k.T, A_ssm_D, B_ssm_D, gate_w,
      jnp.asarray(G0), jnp.asarray(E1), jnp.asarray(Ginv), jnp.asarray(Pm))


@jax.jit
def pallas_gated_mix__ssm_conv_h3__ssm_conv_h3__prompt_kernel(
    A_q, A_k, A_v, A_shift_k, A_ssm_k, A_ssm_D, B_q, B_k, B_v, B_shift_k, B_ssm_k, B_ssm_D, gate_w,
):
    return run(A_q, A_k, A_v, A_shift_k, A_ssm_k, A_ssm_D, B_q, B_k, B_v, B_shift_k, B_ssm_k, B_ssm_D, gate_w)
```

```python
import functools
import numpy as np
import jax
import jax.numpy as jnp
from jax.experimental import pallas as pl
from jax.experimental.pallas import tpu as pltpu

S, D, N1, N2 = 2048, 640, 128, 16
NT = D // 128
NP = 2 * NT
F32, BF16, U32 = jnp.float32, jnp.bfloat16, jnp.uint32


def _pack_rows(m):
    u = np.ascontiguousarray(m, dtype=np.float32).view(np.uint32).astype(np.uint64)
    h = ((u + 0x7FFF + ((u >> 16) & 1)) >> 16).astype(np.uint32)
    return (h[0::2] | (h[1::2] << np.uint32(16))).astype(np.uint32)


def _consts():
    n1 = np.arange(N1)[None, None, :]
    k1 = np.arange(N1)[None, :, None]
    n2 = np.arange(N2)[:, None, None]
    ph = -2 * np.pi * (n1 * k1 / 128.0 + n2 * k1 / 2048.0) + np.pi * (16 * n1 + n2) / 4096.0
    Gr, Gi = np.cos(ph), np.sin(ph)
    G = np.stack([Gr.reshape(N2, 16, 8, N1), Gi.reshape(N2, 16, 8, N1)], axis=2).reshape(N2, 256, N1)
    Ginv = np.transpose(G, (0, 2, 1)) / 2048.0
    Pm = np.zeros((128, 128), np.float32)
    for n2_ in range(16):
        for a in range(8):
            Pm[n2_ * 8 + a, 16 * a + n2_] = 1.0
    Ginv = Ginv.reshape(N2, 128, 2, 128).transpose(0, 2, 1, 3)
    ph0 = -2 * np.pi * (n1[0] * k1[0] / 128.0) + np.pi * (16 * n1[0]) / 4096.0
    g0 = np.concatenate([np.cos(ph0), np.sin(ph0)], axis=0).astype(np.float32)
    phe = -2 * np.pi * np.arange(N1) / 2048.0 + np.pi / 4096.0
    e1 = np.zeros((128, 128), np.float32)
    e1[:, 0], e1[:, 1] = np.cos(phe), np.sin(phe)
    return g0, e1, _pack_rows(Ginv.reshape(4096, 128)), _pack_rows(Pm)

_C1, _S1, _R = float(np.cos(np.pi / 8)), float(np.sin(np.pi / 8)), float(np.sqrt(0.5))


def _bfly4(x, sgn):
    (ar, ai), (br, bi), (cr, ci), (dr, di) = x
    t0r, t0i = ar + cr, ai + ci
    t1r, t1i = ar - cr, ai - ci
    t2r, t2i = br + dr, bi + di
    t3r, t3i = br - dr, bi - di
    x0 = (t0r + t2r, t0i + t2i)
    x2 = (t0r - t2r, t0i - t2i)
    if sgn < 0:
        x1 = (t1r + t3i, t1i - t3r)
        x3 = (t1r - t3i, t1i + t3r)
    else:
        x1 = (t1r - t3i, t1i + t3r)
        x3 = (t1r + t3i, t1i - t3r)
    return [x0, x1, x2, x3]


def _tw(z, e, sgn):
    a, b = z
    if e == 0:
        return z
    if sgn < 0:
        if e == 4: return (b, -a)
        if e == 2: return ((a + b) * _R, (b - a) * _R)
        if e == 6: return ((b - a) * _R, (a + b) * (-_R))
        if e == 1: return (a * _C1 + b * _S1, b * _C1 - a * _S1)
        if e == 3: return (a * _S1 + b * _C1, b * _S1 - a * _C1)
        if e == 9: return (a * (-_C1) - b * _S1, a * _S1 - b * _C1)
    else:
        if e == 4: return (-b, a)
        if e == 2: return ((a - b) * _R, (a + b) * _R)
        if e == 6: return ((a + b) * (-_R), (a - b) * _R)
        if e == 1: return (a * _C1 - b * _S1, b * _C1 + a * _S1)
        if e == 3: return (a * _S1 - b * _C1, b * _S1 + a * _C1)
        if e == 9: return (b * _S1 - a * _C1, a * (-_S1) - b * _C1)
    raise ValueError(e)


def fft16(x, sgn):
    A = [_bfly4([x[nb], x[nb + 4], x[nb + 8], x[nb + 12]], sgn) for nb in range(4)]
    B = [[_tw(A[nb][ka], nb * ka, sgn) for ka in range(4)] for nb in range(4)]
    X = [None] * 16
    for ka in range(4):
        o = _bfly4([B[0][ka], B[1][ka], B[2][ka], B[3][ka]], sgn)
        for kb in range(4):
            X[ka + 4 * kb] = o[kb]
    return X


def _unpack(w):
    lo = jax.lax.bitcast_convert_type(w << 16, F32)
    hi = jax.lax.bitcast_convert_type(w & jnp.uint32(0xFFFF0000), F32)
    return lo, hi


import os as _os2
_FLAGS = {k: True for k in _os2.environ.get('KFLAGS', '').split(',') if k} or None
NT_DIMS = (((1,), (1,)), ((), ()))


import os as _os3

XZH, XZU, XHP, XKV, XYP, XYB, XROWS = 0, 4096, 8192, 9216, 10240, 12288, 16384


def kernel(off_ref, q_hbm, ka_hbm, va_hbm, kb_hbm, vb_hbm, ha_hbm, hb_hbm, ska_ref, skb_ref,
           da_ref, db_ref, gw_ref, g0_ref, e1_ref, gi_hbm, pmat, o_hbm,
           qb, kb, vb, hb, gmat, gimat, ob, zh0, zh1, zu0, zu1, hp0, hp1, kv0, kv1, yp0, yp1, yb0, yb1, yb2, yb3, hh, htf, gnat, par, sems, osems):
    ZH, ZU, HP, KV, YP, YB = (zh0, zh1), (zu0, zu1), (hp0, hp1), (kv0, kv1), (yp0, yp1), (yb0, yb1, yb2, yb3)
    k_hbm, v_hbm, h_hbm = (ka_hbm, kb_hbm), (va_hbm, vb_hbm), (ha_hbm, hb_hbm)

    def cp_k(p):
        return pltpu.make_async_copy(k_hbm[p % 2].at[0, :, pl.ds(128 * (p // 2), 128)], kb.at[p, pl.ds(16, S), :], sems.at[p])
    def cp_v(p):
        return pltpu.make_async_copy(v_hbm[p % 2].at[0, :, pl.ds(128 * (p // 2), 128)], vb.at[p], sems.at[NP + p])
    def cp_h(p):
        return pltpu.make_async_copy(h_hbm[p % 2].at[pl.ds(128 * (p // 2), 128), :], hb.at[p], sems.at[2 * NP + p])
    def cp_q(t):
        return pltpu.make_async_copy(q_hbm.at[0, :, pl.ds(128 * t, 128)], qb.at[t], sems.at[3 * NP + t])
    cp_gi = pltpu.make_async_copy(gi_hbm, gimat, sems.at[3 * NP + NT])
    def cp_o(t, hf):
        rows = pl.ds(hf * (S // 2), S // 2)
        return pltpu.make_async_copy(ob.at[t, rows, :], o_hbm.at[0, rows, pl.ds(128 * t, 128)], osems.at[2 * t + hf])

    cp_h(0).start(); cp_k(0).start(); cp_v(0).start();
    cp_h(1).start(); cp_k(1).start(); cp_v(1).start()

    for p in range(NP):
        kb[p, pl.ds(0, 16), :] = jnp.zeros((16, 128), BF16)
    sk = (ska_ref[...].astype(F32), skb_ref[...].astype(F32))
    dd = (da_ref[...].astype(F32).reshape(1, D), db_ref[...].astype(F32).reshape(1, D))
    for p in range(NP):
        b, t = p % 2, p // 2
        for tap in range(4):
            par[p, pl.ds(8 * tap, 8), :] = jnp.broadcast_to(sk[b][tap:tap + 1, 128 * t:128 * (t + 1)], (8, 128))
        par[p, pl.ds(32, 8), :] = jnp.broadcast_to(dd[b][:, 128 * t:128 * (t + 1)], (8, 128))

    kw, vw, qw, ow = kb.bitcast(U32), vb.bitcast(U32), qb.bitcast(U32), ob.bitcast(U32)
    always = off_ref[0] == 0

    def ds(start, n, mult=None):
        if isinstance(start, int):
            return pl.ds(start, n)
        return pl.ds(pl.multiple_of(start, mult or n), n)

    def ldb(ref, w0, nrows):
        return pltpu.bitcast(ref[ds(w0, nrows // 2, 8), :], BF16)

    def pk(v):
        return pltpu.bitcast(v.astype(BF16), F32)

    def stage_TM(p, jj):
        r = jax.lax.broadcasted_iota(jnp.int32, (128, 128), 0)
        c = jax.lax.broadcasted_iota(jnp.int32, (128, 128), 1)
        pm = pmat[...]
        R = [jax.lax.dot_general(pltpu.bitcast(pm, BF16), hb[p, :, ds(jj * 256 + 128 * u, 128)], NT_DIMS, preferred_element_type=F32)
             for u in range(2)]
        hps = HP[p % 2].at[ds(jj * 8, 1024 - 56, 8), :]
        for n2 in range(16):
            hps[pl.ds(n2 * 64, 8), :] = pk(jnp.concatenate([R[0][8 * n2:8 * n2 + 8], R[1][8 * n2:8 * n2 + 8]], axis=0))

    def stage_Tall(p):
        if True:
            pm = pltpu.bitcast(pmat[...], BF16)
            for jj in range(8):
                R = [jax.lax.dot_general(pm, hb[p, :, pl.ds(jj * 256 + 128 * u, 128)], NT_DIMS,
                                         preferred_element_type=F32) for u in range(2)]
                for n2 in range(16):
                    HP[p % 2][pl.ds(jj * 8 + n2 * 64, 8), :] = pk(
                        jnp.concatenate([R[0][8 * n2:8 * n2 + 8], R[1][8 * n2:8 * n2 + 8]], axis=0))
        else:
            for jt in range(16):
                htf[pl.ds(128 * jt, 128), :] = jnp.transpose(hb[p, :, pl.ds(128 * jt, 128)].astype(F32))
            for jj in range(8):
                for n2 in range(16):
                    HP[p % 2][pl.ds(jj * 8 + n2 * 64, 8), :] = pk(htf[pl.ds(256 * jj + n2, 16, stride=16), :])

    def stage_T1(p, jj):
        for u in range(2):
            blk = hb[p, :, ds(jj * 256 + 128 * u, 128)].astype(F32)
            ht[pl.ds(128 * u, 128), :] = jnp.transpose(blk)

    def stage_T2(p, jj):
        hps = HP[p % 2].at[ds(jj * 8, 1024 - 56, 8), :]
        for n2 in range(16):
            hps[pl.ds(n2 * 64, 8), :] = pk(ht[pl.ds(n2, 16, stride=16), :])

    def stage_P(p, a2, ms=range(8)):
        s = [jnp.concatenate([par[p, pl.ds(8 * tap, 8), :]] * 2, axis=0) for tap in range(4)]
        base = a2 * 128
        ksub = kw.at[p, ds(base + 8, 128, 8), :]
        kprev = kw.at[p, ds(base, 128), :]
        vsub = vw.at[p, ds(base, 128), :]
        kk = {}
        def getk(n):
            if n not in kk:
                m = (n // 2) if n >= 0 else ((n + 16) // 2)
                lo, hi = _unpack((ksub if n >= 0 else kprev)[pl.ds(m, 16, stride=8), :])
                b0 = 2 * m if n >= 0 else 2 * m - 16
                kk[b0], kk[b0 + 1] = lo, hi
            return kk[n]
        kvs = KV[p % 2].at[ds(a2 * 8, 1024 - 56, 8), :]
        for m in ms:
            vlo, vhi = _unpack(vsub[pl.ds(m, 16, stride=8), :])
            for n2, vv in ((2 * m, vlo), (2 * m + 1, vhi)):
                acc = getk(n2) * s[0] + getk(n2 - 1) * s[1] + getk(n2 - 2) * s[2] + getk(n2 - 3) * s[3]
                kvs[pl.ds(n2 * 64, 8), :] = pk(acc * vv)

    def stage_V(p, g):
        xh = ZH[p % 2].at[:, ds(g * 16, 16), :]
        xu = ZU[p % 2].at[:, ds(g * 16, 16), :]
        xo = hh.at[:, ds(g * 16, 16), :]
        ys = YP[p % 2].at[ds(g * 8, 2048 - 120, 8), :]
        z = [(xh[n2, 0:8, :], xh[n2, 8:16, :]) for n2 in range(16)]
        z[0] = (z[0][0] + par[p, pl.ds(32, 8), :], z[0][1])
        H = fft16(z, -1)
        for k2 in range(16):
            xo[k2, 0:8, :] = H[k2][0]
            xo[k2, 8:16, :] = H[k2][1]
        z = [(xu[n2, 0:8, :], xu[n2, 8:16, :]) for n2 in range(16)]
        Uu = fft16(z, -1)
        Y = []
        for k2 in range(16):
            hr, hi = xo[k2, 0:8, :], xo[k2, 8:16, :]
            ur, ui = Uu[k2]
            Y.append((ur * hr - ui * hi, ur * hi + ui * hr))
        T = fft16(Y, +1)
        for n2 in range(16):
            ys[pl.ds(n2 * 128, 8), :] = pk(jnp.concatenate([T[n2][0], T[n2][1]], axis=0))

    def stage_B(t, a):
        ya_ref = YB[(2 * t) % 4].at[:, ds(a * 8, 8), :]
        yb_ref = YB[(2 * t + 1) % 4].at[:, ds(a * 8, 8), :]
        qsub = qw.at[t, ds(a * 64, 64), :]
        osub = ow.at[t, ds(a * 64, 64), :]
        gsub = gnat.at[ds(a * 128, 128), :]
        for m in range(8):
            qs = _unpack(qsub[pl.ds(m, 8, stride=8), :])
            res = []
            for u in range(2):
                n2 = 2 * m + u
                ya, yv = ya_ref[n2], yb_ref[n2]
                gg = gsub[pl.ds(n2, 8, stride=16), :]
                res.append(qs[u] * (yv + gg * (ya - yv)))
            osub[pl.ds(m, 8, stride=8), :] = pltpu.pack_elementwise((res[0], res[1]), packed_dtype=BF16)

    def gate():
        gw = gw_ref[...].reshape(1, D)
        gw8 = jnp.broadcast_to(gw, (8, D))
        for jt in range(S // 128):
            acc = None
            for t in range(NT):
                part = jax.lax.dot_general(gw8[:, 128 * t:128 * (t + 1)], qb[t, pl.ds(128 * jt, 128), :], NT_DIMS,
                                           preferred_element_type=F32)
                acc = part if acc is None else acc + part
            gs = jax.nn.sigmoid(acc)
            gnat[pl.ds(128 * jt, 128), :] = jnp.transpose(jnp.broadcast_to(gs[0:1, :], (128, 128)))

    def gen_g(gq, carry):
        st = []
        for w in range(4):
            g = 4 * gq + w
            e = e1_ref[ds(g * 8, 8), :]
            st.append([g0_ref[ds(g * 8, 8), :], g0_ref[ds(128 + g * 8, 8), :],
                       jnp.broadcast_to(e[:, 0:1], (8, 128)), jnp.broadcast_to(e[:, 1:2], (8, 128))])
        dst = gmat.at[ds(gq * 32, 2048 - 96, 32), :]
        for n2 in range(16):
            for w in range(4):
                gr, gi, er, ei = st[w]
                dst[pl.ds(n2 * 128 + w * 8, 8), :] = pltpu.bitcast(jnp.concatenate([gr, gi], axis=0).astype(BF16), U32)
                if n2 < 15:
                    st[w][0], st[w][1] = gr * er - gi * ei, gr * ei + gi * er
        return carry
    jax.lax.fori_loop(0, 4, gen_g, 0)

    GATE_SLOT = 5
    n_slots = NP + 5
    for s in range(n_slots):
        pT, pF, pV, pI = s, s - 1, s - 2, s - 3
        doT, doF, doV, doI = (0 <= pT < NP), (0 <= pF < NP), (0 <= pV < NP), (0 <= pI < NP)
        tB, hB = None, None
        if s >= 5 and (s - 5) // 2 < NT:
            tB, hB = (s - 5) // 2, (s - 5) % 2
        if s + 2 < NP:
            cp_h(s + 2).start(); cp_k(s + 2).start(); cp_v(s + 2).start()
        if s == 1:
            cp_gi.start()
        if s < NT:
            cp_q(s).start()
        if s == 3:
            cp_gi.wait()
        if s == GATE_SLOT:
            for t in range(NT):
                cp_q(t).wait()
            gate()
        def dot_F(p, i):
            g = ldb(gmat, i * 128, 256)
            ZU[p % 2][i] = jnp.dot(g, ldb(KV[p % 2], i * 64, 128), preferred_element_type=F32)
            ZH[p % 2][i] = jnp.dot(g, ldb(HP[p % 2], i * 64, 128), preferred_element_type=F32)

        def dot_I(p, i):
            lhs = jnp.concatenate([ldb(gimat, i * 128, 128), ldb(gimat, i * 128 + 64, 128)], axis=1)
            YB[p % 4][i] = jnp.dot(lhs, ldb(YP[p % 2], i * 128, 256), preferred_element_type=F32)

        if not doV and (doF or doI):
            with jax.named_scope(f's{s:02d}_mxu'):
              for i in range(16):
                if doF:
                    dot_F(pF, i)
                if doI:
                    dot_I(pI, i)
            doF = doI = False

        if doT:
            with jax.named_scope(f's{s:02d}_hwait'):
                cp_h(pT).wait()
            with jax.named_scope(f's{s:02d}_T'):
                stage_Tall(pT)
        if doT:
            with jax.named_scope(f's{s:02d}_kvwait'):
                cp_k(pT).wait(); cp_v(pT).wait()

        def body(j, carry, pT=pT, pF=pF, pV=pV, pI=pI, doT=doT, doF=doF, doV=doV, doI=doI, tB=tB, hB=hB):
            def common(i):
                if doV:
                    stage_V(pV, i)
                if doF:
                    dot_F(pF, i)
                if doI:
                    dot_I(pI, i)
            BPOS = "B"
            common(2 * j)
            if doT:
                stage_P(pT, j, range(8))
            if tB is not None and BPOS == "A":
                stage_B(tB, hB * 8 + j)
            def second():
                common(2 * j + 1)
                if False:
                    stage_P(pT, j, range(4, 8))
                if tB is not None and BPOS == "B":
                    stage_B(tB, hB * 8 + j)
            if doF or doI or doV:
                pl.when(always)(second)
            else:
                second()
            return carry
        if doT or doF or doV or doI or (tB is not None and True):
            with jax.named_scope(f's{s:02d}_loop'):
                jax.lax.fori_loop(0, 8, body, 0)
        if tB is not None and "A" == "sep":
            def bbody(j, c, tB=tB, hB=hB):
                stage_B(tB, hB * 8 + 2 * j)
                stage_B(tB, hB * 8 + 2 * j + 1)
                return c
            jax.lax.fori_loop(0, 4, bbody, 0)
        if tB is not None:
            cp_o(tB, hB).start()
    with jax.named_scope('owait'):
        for t in range(NT):
            cp_o(t, 0).wait(); cp_o(t, 1).wait()


def run(A_q, A_k, A_v, A_shift_k, A_ssm_k, A_ssm_D, B_q, B_k, B_v, B_shift_k, B_ssm_k, B_ssm_D, gate_w):
    G0, E1, Ginv, Pm = _consts()
    offs = np.zeros((1,), np.int32)
    any_spec = pl.BlockSpec(memory_space=pl.ANY)
    vm = pl.BlockSpec(memory_space=pltpu.VMEM)
    return pl.pallas_call(
        kernel,
        in_specs=[pl.BlockSpec(memory_space=pltpu.SMEM)] + [any_spec] * 7 + [vm] * 7 + [any_spec, vm],
        out_specs=any_spec,
        out_shape=jax.ShapeDtypeStruct((1, S, D), BF16),
        scratch_shapes=[
            pltpu.VMEM((NT, S, 128), BF16),
            pltpu.VMEM((NP, S + 16, 128), BF16),
            pltpu.VMEM((NP, S, 128), BF16),
            pltpu.VMEM((NP, 128, S), BF16),
            pltpu.VMEM((2048, 128), U32),
            pltpu.VMEM((2048, 128), U32),
            pltpu.VMEM((NT, S, 128), BF16),
            *[pltpu.VMEM((16, 256, 128), F32)] * 4,
            *[pltpu.VMEM((1024, 128), F32)] * 4,
            *[pltpu.VMEM((2048, 128), F32)] * 2,
            *[pltpu.VMEM((16, 128, 128), F32)] * 4,
            pltpu.VMEM((16, 256, 128), F32),
            pltpu.VMEM((S, 128), F32),
            pltpu.VMEM((S, 128), F32),
            pltpu.VMEM((NP, 40, 128), F32),
            pltpu.SemaphoreType.DMA((3 * NP + NT + 1,)),
            pltpu.SemaphoreType.DMA((2 * NT,)),
        ],
        compiler_params=pltpu.CompilerParams(vmem_limit_bytes=110 * 1024 * 1024, flags=_FLAGS),
    )(jnp.asarray(offs), A_q, A_k, A_v, B_k, B_v, A_ssm_k, B_ssm_k, A_shift_k.T, B_shift_k.T, A_ssm_D, B_ssm_D, gate_w,
      jnp.asarray(G0), jnp.asarray(E1), jnp.asarray(Ginv), jnp.asarray(Pm))


@jax.jit
def pallas_gated_mix__ssm_conv_h3__ssm_conv_h3__prompt_kernel(
    A_q, A_k, A_v, A_shift_k, A_ssm_k, A_ssm_D, B_q, B_k, B_v, B_shift_k, B_ssm_k, B_ssm_D, gate_w,
):
    return run(A_q, A_k, A_v, A_shift_k, A_ssm_k, A_ssm_D, B_q, B_k, B_v, B_shift_k, B_ssm_k, B_ssm_D, gate_w)
```

```python
import functools
import numpy as np
import jax
import jax.numpy as jnp
from jax.experimental import pallas as pl
from jax.experimental.pallas import tpu as pltpu

S, D, N1, N2 = 2048, 640, 128, 16
NT = D // 128
NP = 2 * NT
F32, BF16, U32 = jnp.float32, jnp.bfloat16, jnp.uint32


def _pack_rows(m):
    u = np.ascontiguousarray(m, dtype=np.float32).view(np.uint32).astype(np.uint64)
    h = ((u + 0x7FFF + ((u >> 16) & 1)) >> 16).astype(np.uint32)
    return (h[0::2] | (h[1::2] << np.uint32(16))).astype(np.uint32)


def _consts():
    n1 = np.arange(N1)[None, None, :]
    k1 = np.arange(N1)[None, :, None]
    n2 = np.arange(N2)[:, None, None]
    ph = -2 * np.pi * (n1 * k1 / 128.0 + n2 * k1 / 2048.0) + np.pi * (16 * n1 + n2) / 4096.0
    Gr, Gi = np.cos(ph), np.sin(ph)
    G = np.stack([Gr.reshape(N2, 16, 8, N1), Gi.reshape(N2, 16, 8, N1)], axis=2).reshape(N2, 256, N1)
    Ginv = np.transpose(G, (0, 2, 1)) / 2048.0
    Pm = np.zeros((128, 128), np.float32)
    for n2_ in range(16):
        for a in range(8):
            Pm[n2_ * 8 + a, 16 * a + n2_] = 1.0
    Ginv = Ginv.reshape(N2, 128, 2, 128).transpose(0, 2, 1, 3)
    ph0 = -2 * np.pi * (n1[0] * k1[0] / 128.0) + np.pi * (16 * n1[0]) / 4096.0
    g0 = np.concatenate([np.cos(ph0), np.sin(ph0)], axis=0).astype(np.float32)
    phe = -2 * np.pi * np.arange(N1) / 2048.0 + np.pi / 4096.0
    e1 = np.zeros((128, 128), np.float32)
    e1[:, 0], e1[:, 1] = np.cos(phe), np.sin(phe)
    return g0, e1, _pack_rows(Ginv.reshape(4096, 128)), _pack_rows(Pm)

_C1, _S1, _R = float(np.cos(np.pi / 8)), float(np.sin(np.pi / 8)), float(np.sqrt(0.5))


def _bfly4(x, sgn):
    (ar, ai), (br, bi), (cr, ci), (dr, di) = x
    t0r, t0i = ar + cr, ai + ci
    t1r, t1i = ar - cr, ai - ci
    t2r, t2i = br + dr, bi + di
    t3r, t3i = br - dr, bi - di
    x0 = (t0r + t2r, t0i + t2i)
    x2 = (t0r - t2r, t0i - t2i)
    if sgn < 0:
        x1 = (t1r + t3i, t1i - t3r)
        x3 = (t1r - t3i, t1i + t3r)
    else:
        x1 = (t1r - t3i, t1i + t3r)
        x3 = (t1r + t3i, t1i - t3r)
    return [x0, x1, x2, x3]


def _tw(z, e, sgn):
    a, b = z
    if e == 0:
        return z
    if sgn < 0:
        if e == 4: return (b, -a)
        if e == 2: return ((a + b) * _R, (b - a) * _R)
        if e == 6: return ((b - a) * _R, (a + b) * (-_R))
        if e == 1: return (a * _C1 + b * _S1, b * _C1 - a * _S1)
        if e == 3: return (a * _S1 + b * _C1, b * _S1 - a * _C1)
        if e == 9: return (a * (-_C1) - b * _S1, a * _S1 - b * _C1)
    else:
        if e == 4: return (-b, a)
        if e == 2: return ((a - b) * _R, (a + b) * _R)
        if e == 6: return ((a + b) * (-_R), (a - b) * _R)
        if e == 1: return (a * _C1 - b * _S1, b * _C1 + a * _S1)
        if e == 3: return (a * _S1 - b * _C1, b * _S1 + a * _C1)
        if e == 9: return (b * _S1 - a * _C1, a * (-_S1) - b * _C1)
    raise ValueError(e)


def fft16(x, sgn):
    A = [_bfly4([x[nb], x[nb + 4], x[nb + 8], x[nb + 12]], sgn) for nb in range(4)]
    B = [[_tw(A[nb][ka], nb * ka, sgn) for ka in range(4)] for nb in range(4)]
    X = [None] * 16
    for ka in range(4):
        o = _bfly4([B[0][ka], B[1][ka], B[2][ka], B[3][ka]], sgn)
        for kb in range(4):
            X[ka + 4 * kb] = o[kb]
    return X


def _unpack(w):
    lo = jax.lax.bitcast_convert_type(w << 16, F32)
    hi = jax.lax.bitcast_convert_type(w & jnp.uint32(0xFFFF0000), F32)
    return lo, hi


import os as _os2
_FLAGS = {k: True for k in _os2.environ.get('KFLAGS', '').split(',') if k} or None
NT_DIMS = (((1,), (1,)), ((), ()))


import os as _os3

XZH, XZU, XHP, XKV, XYP, XYB, XROWS = 0, 4096, 8192, 9216, 10240, 12288, 16384


def kernel(off_ref, q_hbm, ka_hbm, va_hbm, kb_hbm, vb_hbm, ha_hbm, hb_hbm, ska_ref, skb_ref,
           da_ref, db_ref, gw_ref, g0_ref, e1_ref, gi_hbm, pmat, o_hbm,
           qb, kb, vb, hb, gmat, gimat, ob, zh0, zh1, zu0, zu1, hp0, hp1, kv0, kv1, yp0, yp1, yb0, yb1, yb2, yb3, hh, htf, gnat, par, sems, osems):
    ZH, ZU, HP, KV, YP, YB = (zh0, zh1), (zu0, zu1), (hp0, hp1), (kv0, kv1), (yp0, yp1), (yb0, yb1, yb2, yb3)
    k_hbm, v_hbm, h_hbm = (ka_hbm, kb_hbm), (va_hbm, vb_hbm), (ha_hbm, hb_hbm)

    def cp_k(p):
        return pltpu.make_async_copy(k_hbm[p % 2].at[0, :, pl.ds(128 * (p // 2), 128)], kb.at[p, pl.ds(16, S), :], sems.at[p])
    def cp_v(p):
        return pltpu.make_async_copy(v_hbm[p % 2].at[0, :, pl.ds(128 * (p // 2), 128)], vb.at[p], sems.at[NP + p])
    def cp_h(p):
        return pltpu.make_async_copy(h_hbm[p % 2].at[pl.ds(128 * (p // 2), 128), :], hb.at[p], sems.at[2 * NP + p])
    def cp_q(t):
        return pltpu.make_async_copy(q_hbm.at[0, :, pl.ds(128 * t, 128)], qb.at[t], sems.at[3 * NP + t])
    cp_gi = pltpu.make_async_copy(gi_hbm, gimat, sems.at[3 * NP + NT])
    def cp_o(t, hf):
        rows = pl.ds(hf * (S // 2), S // 2)
        return pltpu.make_async_copy(ob.at[t, rows, :], o_hbm.at[0, rows, pl.ds(128 * t, 128)], osems.at[2 * t + hf])

    cp_h(0).start(); cp_k(0).start(); cp_v(0).start();

    for p in range(NP):
        kb[p, pl.ds(0, 16), :] = jnp.zeros((16, 128), BF16)
    sk = (ska_ref[...].astype(F32), skb_ref[...].astype(F32))
    dd = (da_ref[...].astype(F32).reshape(1, D), db_ref[...].astype(F32).reshape(1, D))
    for p in range(NP):
        b, t = p % 2, p // 2
        for tap in range(4):
            par[p, pl.ds(8 * tap, 8), :] = jnp.broadcast_to(sk[b][tap:tap + 1, 128 * t:128 * (t + 1)], (8, 128))
        par[p, pl.ds(32, 8), :] = jnp.broadcast_to(dd[b][:, 128 * t:128 * (t + 1)], (8, 128))

    kw, vw, qw, ow = kb.bitcast(U32), vb.bitcast(U32), qb.bitcast(U32), ob.bitcast(U32)
    always = off_ref[0] == 0

    def ds(start, n, mult=None):
        if isinstance(start, int):
            return pl.ds(start, n)
        return pl.ds(pl.multiple_of(start, mult or n), n)

    def ldb(ref, w0, nrows):
        return pltpu.bitcast(ref[ds(w0, nrows // 2, 8), :], BF16)

    def pk(v):
        return pltpu.bitcast(v.astype(BF16), F32)

    def stage_TM(p, jj):
        r = jax.lax.broadcasted_iota(jnp.int32, (128, 128), 0)
        c = jax.lax.broadcasted_iota(jnp.int32, (128, 128), 1)
        pm = pmat[...]
        R = [jax.lax.dot_general(pltpu.bitcast(pm, BF16), hb[p, :, ds(jj * 256 + 128 * u, 128)], NT_DIMS, preferred_element_type=F32)
             for u in range(2)]
        hps = HP[p % 2].at[ds(jj * 8, 1024 - 56, 8), :]
        for n2 in range(16):
            hps[pl.ds(n2 * 64, 8), :] = pk(jnp.concatenate([R[0][8 * n2:8 * n2 + 8], R[1][8 * n2:8 * n2 + 8]], axis=0))

    def stage_Tall(p):
        if True:
            pm = pltpu.bitcast(pmat[...], BF16)
            for jj in range(8):
                R = [jax.lax.dot_general(pm, hb[p, :, pl.ds(jj * 256 + 128 * u, 128)], NT_DIMS,
                                         preferred_element_type=F32) for u in range(2)]
                for n2 in range(16):
                    HP[p % 2][pl.ds(jj * 8 + n2 * 64, 8), :] = pk(
                        jnp.concatenate([R[0][8 * n2:8 * n2 + 8], R[1][8 * n2:8 * n2 + 8]], axis=0))
        else:
            for jt in range(16):
                htf[pl.ds(128 * jt, 128), :] = jnp.transpose(hb[p, :, pl.ds(128 * jt, 128)].astype(F32))
            for jj in range(8):
                for n2 in range(16):
                    HP[p % 2][pl.ds(jj * 8 + n2 * 64, 8), :] = pk(htf[pl.ds(256 * jj + n2, 16, stride=16), :])

    def stage_T1(p, jj):
        for u in range(2):
            blk = hb[p, :, ds(jj * 256 + 128 * u, 128)].astype(F32)
            ht[pl.ds(128 * u, 128), :] = jnp.transpose(blk)

    def stage_T2(p, jj):
        hps = HP[p % 2].at[ds(jj * 8, 1024 - 56, 8), :]
        for n2 in range(16):
            hps[pl.ds(n2 * 64, 8), :] = pk(ht[pl.ds(n2, 16, stride=16), :])

    def stage_P(p, a2, ms=range(8)):
        s = [jnp.concatenate([par[p, pl.ds(8 * tap, 8), :]] * 2, axis=0) for tap in range(4)]
        base = a2 * 128
        ksub = kw.at[p, ds(base + 8, 128, 8), :]
        kprev = kw.at[p, ds(base, 128), :]
        vsub = vw.at[p, ds(base, 128), :]
        kk = {}
        def getk(n):
            if n not in kk:
                m = (n // 2) if n >= 0 else ((n + 16) // 2)
                lo, hi = _unpack((ksub if n >= 0 else kprev)[pl.ds(m, 16, stride=8), :])
                b0 = 2 * m if n >= 0 else 2 * m - 16
                kk[b0], kk[b0 + 1] = lo, hi
            return kk[n]
        kvs = KV[p % 2].at[ds(a2 * 8, 1024 - 56, 8), :]
        for m in ms:
            vlo, vhi = _unpack(vsub[pl.ds(m, 16, stride=8), :])
            for n2, vv in ((2 * m, vlo), (2 * m + 1, vhi)):
                acc = getk(n2) * s[0] + getk(n2 - 1) * s[1] + getk(n2 - 2) * s[2] + getk(n2 - 3) * s[3]
                kvs[pl.ds(n2 * 64, 8), :] = pk(acc * vv)

    def stage_V(p, g):
        xh = ZH[p % 2].at[:, ds(g * 16, 16), :]
        xu = ZU[p % 2].at[:, ds(g * 16, 16), :]
        xo = hh.at[:, ds(g * 16, 16), :]
        ys = YP[p % 2].at[ds(g * 8, 2048 - 120, 8), :]
        z = [(xh[n2, 0:8, :], xh[n2, 8:16, :]) for n2 in range(16)]
        z[0] = (z[0][0] + par[p, pl.ds(32, 8), :], z[0][1])
        H = fft16(z, -1)
        for k2 in range(16):
            xo[k2, 0:8, :] = H[k2][0]
            xo[k2, 8:16, :] = H[k2][1]
        z = [(xu[n2, 0:8, :], xu[n2, 8:16, :]) for n2 in range(16)]
        Uu = fft16(z, -1)
        Y = []
        for k2 in range(16):
            hr, hi = xo[k2, 0:8, :], xo[k2, 8:16, :]
            ur, ui = Uu[k2]
            Y.append((ur * hr - ui * hi, ur * hi + ui * hr))
        T = fft16(Y, +1)
        for n2 in range(16):
            ys[pl.ds(n2 * 128, 8), :] = pk(jnp.concatenate([T[n2][0], T[n2][1]], axis=0))

    def stage_B(t, a):
        ya_ref = YB[(2 * t) % 4].at[:, ds(a * 8, 8), :]
        yb_ref = YB[(2 * t + 1) % 4].at[:, ds(a * 8, 8), :]
        qsub = qw.at[t, ds(a * 64, 64), :]
        osub = ow.at[t, ds(a * 64, 64), :]
        gsub = gnat.at[ds(a * 128, 128), :]
        for m in range(8):
            qs = _unpack(qsub[pl.ds(m, 8, stride=8), :])
            res = []
            for u in range(2):
                n2 = 2 * m + u
                ya, yv = ya_ref[n2], yb_ref[n2]
                gg = gsub[pl.ds(n2, 8, stride=16), :]
                res.append(qs[u] * (yv + gg * (ya - yv)))
            osub[pl.ds(m, 8, stride=8), :] = pltpu.pack_elementwise((res[0], res[1]), packed_dtype=BF16)

    def gate():
        gw = gw_ref[...].reshape(1, D)
        gw8 = jnp.broadcast_to(gw, (8, D))
        for jt in range(S // 128):
            acc = None
            for t in range(NT):
                part = jax.lax.dot_general(gw8[:, 128 * t:128 * (t + 1)], qb[t, pl.ds(128 * jt, 128), :], NT_DIMS,
                                           preferred_element_type=F32)
                acc = part if acc is None else acc + part
            gs = jax.nn.sigmoid(acc)
            gnat[pl.ds(128 * jt, 128), :] = jnp.transpose(jnp.broadcast_to(gs[0:1, :], (128, 128)))

    def gen_g(gq, carry):
        st = []
        for w in range(4):
            g = 4 * gq + w
            e = e1_ref[ds(g * 8, 8), :]
            st.append([g0_ref[ds(g * 8, 8), :], g0_ref[ds(128 + g * 8, 8), :],
                       jnp.broadcast_to(e[:, 0:1], (8, 128)), jnp.broadcast_to(e[:, 1:2], (8, 128))])
        dst = gmat.at[ds(gq * 32, 2048 - 96, 32), :]
        for n2 in range(16):
            for w in range(4):
                gr, gi, er, ei = st[w]
                dst[pl.ds(n2 * 128 + w * 8, 8), :] = pltpu.bitcast(jnp.concatenate([gr, gi], axis=0).astype(BF16), U32)
                if n2 < 15:
                    st[w][0], st[w][1] = gr * er - gi * ei, gr * ei + gi * er
        return carry
    jax.lax.fori_loop(0, 4, gen_g, 0)

    GATE_SLOT = 5
    n_slots = NP + 5
    for s in range(n_slots):
        pT, pF, pV, pI = s, s - 1, s - 2, s - 3
        doT, doF, doV, doI = (0 <= pT < NP), (0 <= pF < NP), (0 <= pV < NP), (0 <= pI < NP)
        tB, hB = None, None
        if s >= 5 and (s - 5) // 2 < NT:
            tB, hB = (s - 5) // 2, (s - 5) % 2
        for pp in ([] if s == 0 else [2, 3] if s == 1 else [s + 2]):
            if pp < NP:
                cp_h(pp).start(); cp_k(pp).start(); cp_v(pp).start()
        if s == 2:
            cp_gi.start()
        if 1 <= s <= 3:
            for t in ([0] if s == 1 else [1, 2] if s == 2 else [3, 4]):
                cp_q(t).start()
        if s == 3:
            cp_gi.wait()
        if s == GATE_SLOT:
            for t in range(NT):
                cp_q(t).wait()
            gate()
        def dot_F(p, i):
            g = ldb(gmat, i * 128, 256)
            ZU[p % 2][i] = jnp.dot(g, ldb(KV[p % 2], i * 64, 128), preferred_element_type=F32)
            ZH[p % 2][i] = jnp.dot(g, ldb(HP[p % 2], i * 64, 128), preferred_element_type=F32)

        def dot_I(p, i):
            lhs = jnp.concatenate([ldb(gimat, i * 128, 128), ldb(gimat, i * 128 + 64, 128)], axis=1)
            YB[p % 4][i] = jnp.dot(lhs, ldb(YP[p % 2], i * 128, 256), preferred_element_type=F32)

        if not doV and (doF or doI):
            with jax.named_scope(f's{s:02d}_mxu'):
              for i in range(16):
                if doF:
                    dot_F(pF, i)
                if doI:
                    dot_I(pI, i)
            doF = doI = False

        if doT:
            with jax.named_scope(f's{s:02d}_hwait'):
                cp_h(pT).wait()
            with jax.named_scope(f's{s:02d}_T'):
                stage_Tall(pT)
        if s == 0:
            cp_h(1).start(); cp_k(1).start(); cp_v(1).start()
        if doT:
            with jax.named_scope(f's{s:02d}_kvwait'):
                cp_k(pT).wait(); cp_v(pT).wait()

        def body(j, carry, pT=pT, pF=pF, pV=pV, pI=pI, doT=doT, doF=doF, doV=doV, doI=doI, tB=tB, hB=hB):
            def common(i):
                if doV:
                    stage_V(pV, i)
                if doF:
                    dot_F(pF, i)
                if doI:
                    dot_I(pI, i)
            BPOS = "B"
            common(2 * j)
            if doT:
                stage_P(pT, j, range(8))
            if tB is not None and BPOS == "A":
                stage_B(tB, hB * 8 + j)
            def second():
                common(2 * j + 1)
                if False:
                    stage_P(pT, j, range(4, 8))
                if tB is not None and BPOS == "B":
                    stage_B(tB, hB * 8 + j)
            if doF or doI or doV:
                pl.when(always)(second)
            else:
                second()
            return carry
        if doT or doF or doV or doI or (tB is not None and True):
            with jax.named_scope(f's{s:02d}_loop'):
                jax.lax.fori_loop(0, 8, body, 0)
        if tB is not None and "A" == "sep":
            def bbody(j, c, tB=tB, hB=hB):
                stage_B(tB, hB * 8 + 2 * j)
                stage_B(tB, hB * 8 + 2 * j + 1)
                return c
            jax.lax.fori_loop(0, 4, bbody, 0)
        if tB is not None:
            cp_o(tB, hB).start()
    with jax.named_scope('owait'):
        for t in range(NT):
            cp_o(t, 0).wait(); cp_o(t, 1).wait()


def run(A_q, A_k, A_v, A_shift_k, A_ssm_k, A_ssm_D, B_q, B_k, B_v, B_shift_k, B_ssm_k, B_ssm_D, gate_w):
    G0, E1, Ginv, Pm = _consts()
    offs = np.zeros((1,), np.int32)
    any_spec = pl.BlockSpec(memory_space=pl.ANY)
    vm = pl.BlockSpec(memory_space=pltpu.VMEM)
    return pl.pallas_call(
        kernel,
        in_specs=[pl.BlockSpec(memory_space=pltpu.SMEM)] + [any_spec] * 7 + [vm] * 7 + [any_spec, vm],
        out_specs=any_spec,
        out_shape=jax.ShapeDtypeStruct((1, S, D), BF16),
        scratch_shapes=[
            pltpu.VMEM((NT, S, 128), BF16),
            pltpu.VMEM((NP, S + 16, 128), BF16),
            pltpu.VMEM((NP, S, 128), BF16),
            pltpu.VMEM((NP, 128, S), BF16),
            pltpu.VMEM((2048, 128), U32),
            pltpu.VMEM((2048, 128), U32),
            pltpu.VMEM((NT, S, 128), BF16),
            *[pltpu.VMEM((16, 256, 128), F32)] * 4,
            *[pltpu.VMEM((1024, 128), F32)] * 4,
            *[pltpu.VMEM((2048, 128), F32)] * 2,
            *[pltpu.VMEM((16, 128, 128), F32)] * 4,
            pltpu.VMEM((16, 256, 128), F32),
            pltpu.VMEM((S, 128), F32),
            pltpu.VMEM((S, 128), F32),
            pltpu.VMEM((NP, 40, 128), F32),
            pltpu.SemaphoreType.DMA((3 * NP + NT + 1,)),
            pltpu.SemaphoreType.DMA((2 * NT,)),
        ],
        compiler_params=pltpu.CompilerParams(vmem_limit_bytes=110 * 1024 * 1024, flags=_FLAGS),
    )(jnp.asarray(offs), A_q, A_k, A_v, B_k, B_v, A_ssm_k, B_ssm_k, A_shift_k.T, B_shift_k.T, A_ssm_D, B_ssm_D, gate_w,
      jnp.asarray(G0), jnp.asarray(E1), jnp.asarray(Ginv), jnp.asarray(Pm))


@jax.jit
def pallas_gated_mix__ssm_conv_h3__ssm_conv_h3__prompt_kernel(
    A_q, A_k, A_v, A_shift_k, A_ssm_k, A_ssm_D, B_q, B_k, B_v, B_shift_k, B_ssm_k, B_ssm_D, gate_w,
):
    return run(A_q, A_k, A_v, A_shift_k, A_ssm_k, A_ssm_D, B_q, B_k, B_v, B_shift_k, B_ssm_k, B_ssm_D, gate_w)
```

```python
import functools
import numpy as np
import jax
import jax.numpy as jnp
from jax.experimental import pallas as pl
from jax.experimental.pallas import tpu as pltpu

S, D, N1, N2 = 2048, 640, 128, 16
NT = D // 128
NP = 2 * NT
F32, BF16, U32 = jnp.float32, jnp.bfloat16, jnp.uint32


def _pack_rows(m):
    u = np.ascontiguousarray(m, dtype=np.float32).view(np.uint32).astype(np.uint64)
    h = ((u + 0x7FFF + ((u >> 16) & 1)) >> 16).astype(np.uint32)
    return (h[0::2] | (h[1::2] << np.uint32(16))).astype(np.uint32)


def _consts():
    n1 = np.arange(N1)[None, None, :]
    k1 = np.arange(N1)[None, :, None]
    n2 = np.arange(N2)[:, None, None]
    ph = -2 * np.pi * (n1 * k1 / 128.0 + n2 * k1 / 2048.0) + np.pi * (16 * n1 + n2) / 4096.0
    Gr, Gi = np.cos(ph), np.sin(ph)
    G = np.stack([Gr.reshape(N2, 16, 8, N1), Gi.reshape(N2, 16, 8, N1)], axis=2).reshape(N2, 256, N1)
    Ginv = np.transpose(G, (0, 2, 1)) / 2048.0
    Pm = np.zeros((128, 128), np.float32)
    for n2_ in range(16):
        for a in range(8):
            Pm[n2_ * 8 + a, 16 * a + n2_] = 1.0
    Ginv = Ginv.reshape(N2, 128, 2, 128).transpose(0, 2, 1, 3)
    ph0 = -2 * np.pi * (n1[0] * k1[0] / 128.0) + np.pi * (16 * n1[0]) / 4096.0
    g0 = np.concatenate([np.cos(ph0), np.sin(ph0)], axis=0).astype(np.float32)
    phe = -2 * np.pi * np.arange(N1) / 2048.0 + np.pi / 4096.0
    e1 = np.zeros((128, 128), np.float32)
    e1[:, 0], e1[:, 1] = np.cos(phe), np.sin(phe)
    return g0, e1, _pack_rows(Ginv.reshape(4096, 128)), _pack_rows(Pm)

_C1, _S1, _R = float(np.cos(np.pi / 8)), float(np.sin(np.pi / 8)), float(np.sqrt(0.5))


def _bfly4(x, sgn):
    (ar, ai), (br, bi), (cr, ci), (dr, di) = x
    t0r, t0i = ar + cr, ai + ci
    t1r, t1i = ar - cr, ai - ci
    t2r, t2i = br + dr, bi + di
    t3r, t3i = br - dr, bi - di
    x0 = (t0r + t2r, t0i + t2i)
    x2 = (t0r - t2r, t0i - t2i)
    if sgn < 0:
        x1 = (t1r + t3i, t1i - t3r)
        x3 = (t1r - t3i, t1i + t3r)
    else:
        x1 = (t1r - t3i, t1i + t3r)
        x3 = (t1r + t3i, t1i - t3r)
    return [x0, x1, x2, x3]


def _tw(z, e, sgn):
    a, b = z
    if e == 0:
        return z
    if sgn < 0:
        if e == 4: return (b, -a)
        if e == 2: return ((a + b) * _R, (b - a) * _R)
        if e == 6: return ((b - a) * _R, (a + b) * (-_R))
        if e == 1: return (a * _C1 + b * _S1, b * _C1 - a * _S1)
        if e == 3: return (a * _S1 + b * _C1, b * _S1 - a * _C1)
        if e == 9: return (a * (-_C1) - b * _S1, a * _S1 - b * _C1)
    else:
        if e == 4: return (-b, a)
        if e == 2: return ((a - b) * _R, (a + b) * _R)
        if e == 6: return ((a + b) * (-_R), (a - b) * _R)
        if e == 1: return (a * _C1 - b * _S1, b * _C1 + a * _S1)
        if e == 3: return (a * _S1 - b * _C1, b * _S1 + a * _C1)
        if e == 9: return (b * _S1 - a * _C1, a * (-_S1) - b * _C1)
    raise ValueError(e)


def fft16(x, sgn):
    A = [_bfly4([x[nb], x[nb + 4], x[nb + 8], x[nb + 12]], sgn) for nb in range(4)]
    B = [[_tw(A[nb][ka], nb * ka, sgn) for ka in range(4)] for nb in range(4)]
    X = [None] * 16
    for ka in range(4):
        o = _bfly4([B[0][ka], B[1][ka], B[2][ka], B[3][ka]], sgn)
        for kb in range(4):
            X[ka + 4 * kb] = o[kb]
    return X


def _unpack(w):
    lo = jax.lax.bitcast_convert_type(w << 16, F32)
    hi = jax.lax.bitcast_convert_type(w & jnp.uint32(0xFFFF0000), F32)
    return lo, hi


NT_DIMS = (((1,), (1,)), ((), ()))


def kernel(off_ref, q_hbm, ka_hbm, va_hbm, kb_hbm, vb_hbm, ha_hbm, hb_hbm, ska_ref, skb_ref,
           da_ref, db_ref, gw_ref, g0_ref, e1_ref, gi_hbm, pmat, o_hbm,
           qb, kb, vb, hb, gmat, gimat, ob, zh0, zh1, zu0, zu1, hp0, hp1, kv0, kv1, yp0, yp1, yb0, yb1, yb2, yb3, hh, gnat, par, sems, osems):
    ZH, ZU, HP, KV, YP, YB = (zh0, zh1), (zu0, zu1), (hp0, hp1), (kv0, kv1), (yp0, yp1), (yb0, yb1, yb2, yb3)
    k_hbm, v_hbm, h_hbm = (ka_hbm, kb_hbm), (va_hbm, vb_hbm), (ha_hbm, hb_hbm)

    def cp_k(p):
        return pltpu.make_async_copy(k_hbm[p % 2].at[0, :, pl.ds(128 * (p // 2), 128)], kb.at[p, pl.ds(16, S), :], sems.at[p])
    def cp_v(p):
        return pltpu.make_async_copy(v_hbm[p % 2].at[0, :, pl.ds(128 * (p // 2), 128)], vb.at[p], sems.at[NP + p])
    def cp_h(p):
        return pltpu.make_async_copy(h_hbm[p % 2].at[pl.ds(128 * (p // 2), 128), :], hb.at[p], sems.at[2 * NP + p])
    def cp_q(t):
        return pltpu.make_async_copy(q_hbm.at[0, :, pl.ds(128 * t, 128)], qb.at[t], sems.at[3 * NP + t])
    cp_gi = pltpu.make_async_copy(gi_hbm, gimat, sems.at[3 * NP + NT])
    def cp_o(t, hf):
        rows = pl.ds(hf * (S // 2), S // 2)
        return pltpu.make_async_copy(ob.at[t, rows, :], o_hbm.at[0, rows, pl.ds(128 * t, 128)], osems.at[2 * t + hf])

    for p in range(NP):
        kb[p, pl.ds(0, 16), :] = jnp.zeros((16, 128), BF16)
    cp_h(0).start(); cp_k(0).start(); cp_v(0).start();
    cp_h(1).start(); cp_k(1).start(); cp_v(1).start()

    sk = (ska_ref[...].astype(F32), skb_ref[...].astype(F32))
    dd = (da_ref[...].astype(F32).reshape(1, D), db_ref[...].astype(F32).reshape(1, D))
    for p in range(NP):
        b, t = p % 2, p // 2
        for tap in range(4):
            par[p, pl.ds(8 * tap, 8), :] = jnp.broadcast_to(sk[b][tap:tap + 1, 128 * t:128 * (t + 1)], (8, 128))
        par[p, pl.ds(32, 8), :] = jnp.broadcast_to(dd[b][:, 128 * t:128 * (t + 1)], (8, 128))

    kw, vw, qw, ow = kb.bitcast(U32), vb.bitcast(U32), qb.bitcast(U32), ob.bitcast(U32)
    always = off_ref[0] == 0

    def ds(start, n, mult=None):
        if isinstance(start, int):
            return pl.ds(start, n)
        return pl.ds(pl.multiple_of(start, mult or n), n)

    def ldb(ref, w0, nrows):
        return pltpu.bitcast(ref[ds(w0, nrows // 2, 8), :], BF16)

    def pk(v):
        return pltpu.bitcast(v.astype(BF16), F32)

    def stage_Tall(p):
        if True:
            pm = pltpu.bitcast(pmat[...], BF16)
            for jj in range(8):
                R = [jax.lax.dot_general(pm, hb[p, :, pl.ds(jj * 256 + 128 * u, 128)], NT_DIMS,
                                         preferred_element_type=F32) for u in range(2)]
                for n2 in range(16):
                    HP[p % 2][pl.ds(jj * 8 + n2 * 64, 8), :] = pk(
                        jnp.concatenate([R[0][8 * n2:8 * n2 + 8], R[1][8 * n2:8 * n2 + 8]], axis=0))
    def stage_P(p, a2, ms=range(8)):
        s = [jnp.concatenate([par[p, pl.ds(8 * tap, 8), :]] * 2, axis=0) for tap in range(4)]
        base = a2 * 128
        ksub = kw.at[p, ds(base + 8, 128, 8), :]
        kprev = kw.at[p, ds(base, 128), :]
        vsub = vw.at[p, ds(base, 128), :]
        kk = {}
        def getk(n):
            if n not in kk:
                m = (n // 2) if n >= 0 else ((n + 16) // 2)
                lo, hi = _unpack((ksub if n >= 0 else kprev)[pl.ds(m, 16, stride=8), :])
                b0 = 2 * m if n >= 0 else 2 * m - 16
                kk[b0], kk[b0 + 1] = lo, hi
            return kk[n]
        kvs = KV[p % 2].at[ds(a2 * 8, 1024 - 56, 8), :]
        for m in ms:
            vlo, vhi = _unpack(vsub[pl.ds(m, 16, stride=8), :])
            for n2, vv in ((2 * m, vlo), (2 * m + 1, vhi)):
                acc = getk(n2) * s[0] + getk(n2 - 1) * s[1] + getk(n2 - 2) * s[2] + getk(n2 - 3) * s[3]
                kvs[pl.ds(n2 * 64, 8), :] = pk(acc * vv)

    def stage_V(p, g):
        xh = ZH[p % 2].at[:, ds(g * 16, 16), :]
        xu = ZU[p % 2].at[:, ds(g * 16, 16), :]
        xo = hh.at[:, ds(g * 16, 16), :]
        ys = YP[p % 2].at[ds(g * 8, 2048 - 120, 8), :]
        z = [(xh[n2, 0:8, :], xh[n2, 8:16, :]) for n2 in range(16)]
        z[0] = (z[0][0] + par[p, pl.ds(32, 8), :], z[0][1])
        H = fft16(z, -1)
        for k2 in range(16):
            xo[k2, 0:8, :] = H[k2][0]
            xo[k2, 8:16, :] = H[k2][1]
        z = [(xu[n2, 0:8, :], xu[n2, 8:16, :]) for n2 in range(16)]
        Uu = fft16(z, -1)
        Y = []
        for k2 in range(16):
            hr, hi = xo[k2, 0:8, :], xo[k2, 8:16, :]
            ur, ui = Uu[k2]
            Y.append((ur * hr - ui * hi, ur * hi + ui * hr))
        T = fft16(Y, +1)
        for n2 in range(16):
            ys[pl.ds(n2 * 128, 8), :] = pk(jnp.concatenate([T[n2][0], T[n2][1]], axis=0))

    def stage_B(t, a):
        ya_ref = YB[(2 * t) % 4].at[:, ds(a * 8, 8), :]
        yb_ref = YB[(2 * t + 1) % 4].at[:, ds(a * 8, 8), :]
        qsub = qw.at[t, ds(a * 64, 64), :]
        osub = ow.at[t, ds(a * 64, 64), :]
        gsub = gnat.at[ds(a * 128, 128), :]
        for m in range(8):
            qs = _unpack(qsub[pl.ds(m, 8, stride=8), :])
            res = []
            for u in range(2):
                n2 = 2 * m + u
                ya, yv = ya_ref[n2], yb_ref[n2]
                gg = gsub[pl.ds(n2, 8, stride=16), :]
                res.append(qs[u] * (yv + gg * (ya - yv)))
            osub[pl.ds(m, 8, stride=8), :] = pltpu.pack_elementwise((res[0], res[1]), packed_dtype=BF16)

    def gate():
        gw = gw_ref[...].reshape(1, D)
        gw8 = jnp.broadcast_to(gw, (8, D))
        for jt in range(S // 128):
            acc = None
            for t in range(NT):
                part = jax.lax.dot_general(gw8[:, 128 * t:128 * (t + 1)], qb[t, pl.ds(128 * jt, 128), :], NT_DIMS,
                                           preferred_element_type=F32)
                acc = part if acc is None else acc + part
            gs = jax.nn.sigmoid(acc)
            gnat[pl.ds(128 * jt, 128), :] = jnp.transpose(jnp.broadcast_to(gs[0:1, :], (128, 128)))

    def gen_g(gq, carry):
        st = []
        for w in range(4):
            g = 4 * gq + w
            e = e1_ref[ds(g * 8, 8), :]
            st.append([g0_ref[ds(g * 8, 8), :], g0_ref[ds(128 + g * 8, 8), :],
                       jnp.broadcast_to(e[:, 0:1], (8, 128)), jnp.broadcast_to(e[:, 1:2], (8, 128))])
        dst = gmat.at[ds(gq * 32, 2048 - 96, 32), :]
        for n2 in range(16):
            for w in range(4):
                gr, gi, er, ei = st[w]
                dst[pl.ds(n2 * 128 + w * 8, 8), :] = pltpu.bitcast(jnp.concatenate([gr, gi], axis=0).astype(BF16), U32)
                if n2 < 15:
                    st[w][0], st[w][1] = gr * er - gi * ei, gr * ei + gi * er
        return carry
    jax.lax.fori_loop(0, 4, gen_g, 0)

    GATE_SLOT = 5
    n_slots = NP + 5
    for s in range(n_slots):
        pT, pF, pV, pI = s, s - 1, s - 2, s - 3
        doT, doF, doV, doI = (0 <= pT < NP), (0 <= pF < NP), (0 <= pV < NP), (0 <= pI < NP)
        tB, hB = None, None
        if s >= 5 and (s - 5) // 2 < NT:
            tB, hB = (s - 5) // 2, (s - 5) % 2
        if s + 2 < NP:
            cp_h(s + 2).start(); cp_k(s + 2).start(); cp_v(s + 2).start()
        if s == 1:
            cp_gi.start()
        if s < NT:
            cp_q(s).start()
        if s == 3:
            cp_gi.wait()
        if s == GATE_SLOT:
            for t in range(NT):
                cp_q(t).wait()
            gate()
        def dot_F(p, i):
            g = ldb(gmat, i * 128, 256)
            ZU[p % 2][i] = jnp.dot(g, ldb(KV[p % 2], i * 64, 128), preferred_element_type=F32)
            ZH[p % 2][i] = jnp.dot(g, ldb(HP[p % 2], i * 64, 128), preferred_element_type=F32)

        def dot_I(p, i):
            lhs = jnp.concatenate([ldb(gimat, i * 128, 128), ldb(gimat, i * 128 + 64, 128)], axis=1)
            YB[p % 4][i] = jnp.dot(lhs, ldb(YP[p % 2], i * 128, 256), preferred_element_type=F32)

        if not doV and (doF or doI):
            with jax.named_scope(f's{s:02d}_mxu'):
              for i in range(16):
                if doF:
                    dot_F(pF, i)
                if doI:
                    dot_I(pI, i)
            doF = doI = False

        if doT:
            with jax.named_scope(f's{s:02d}_hwait'):
                cp_h(pT).wait()
            with jax.named_scope(f's{s:02d}_T'):
                stage_Tall(pT)
        if doT:
            with jax.named_scope(f's{s:02d}_kvwait'):
                cp_k(pT).wait(); cp_v(pT).wait()

        def body(j, carry, pT=pT, pF=pF, pV=pV, pI=pI, doT=doT, doF=doF, doV=doV, doI=doI, tB=tB, hB=hB):
            def common(i):
                if doV:
                    stage_V(pV, i)
                if doF:
                    dot_F(pF, i)
                if doI:
                    dot_I(pI, i)
            common(2 * j)
            if doT:
                stage_P(pT, j, range(8))
            def second():
                common(2 * j + 1)
                if tB is not None:
                    stage_B(tB, hB * 8 + j)
            if doF or doI or doV:
                pl.when(always)(second)
            else:
                second()
            return carry
        if tB is not None and not (doT or doF or doV or doI):
            def bbody(j, c, tB=tB, hB=hB):
                stage_B(tB, hB * 8 + 2 * j)
                stage_B(tB, hB * 8 + 2 * j + 1)
                return c
            jax.lax.fori_loop(0, 4, bbody, 0)
        elif doT or doF or doV or doI or tB is not None:
            with jax.named_scope(f's{s:02d}_loop'):
                jax.lax.fori_loop(0, 8, body, 0)
        if tB is not None and "A" == "sep":
            def bbody(j, c, tB=tB, hB=hB):
                stage_B(tB, hB * 8 + 2 * j)
                stage_B(tB, hB * 8 + 2 * j + 1)
                return c
            jax.lax.fori_loop(0, 4, bbody, 0)
        if tB is not None:
            cp_o(tB, hB).start()
    with jax.named_scope('owait'):
        for t in range(NT):
            cp_o(t, 0).wait(); cp_o(t, 1).wait()


def run(A_q, A_k, A_v, A_shift_k, A_ssm_k, A_ssm_D, B_q, B_k, B_v, B_shift_k, B_ssm_k, B_ssm_D, gate_w):
    G0, E1, Ginv, Pm = _consts()
    offs = np.zeros((1,), np.int32)
    any_spec = pl.BlockSpec(memory_space=pl.ANY)
    vm = pl.BlockSpec(memory_space=pltpu.VMEM)
    return pl.pallas_call(
        kernel,
        in_specs=[pl.BlockSpec(memory_space=pltpu.SMEM)] + [any_spec] * 7 + [vm] * 7 + [any_spec, vm],
        out_specs=any_spec,
        out_shape=jax.ShapeDtypeStruct((1, S, D), BF16),
        scratch_shapes=[
            pltpu.VMEM((NT, S, 128), BF16),
            pltpu.VMEM((NP, S + 16, 128), BF16),
            pltpu.VMEM((NP, S, 128), BF16),
            pltpu.VMEM((NP, 128, S), BF16),
            pltpu.VMEM((2048, 128), U32),
            pltpu.VMEM((2048, 128), U32),
            pltpu.VMEM((NT, S, 128), BF16),
            *[pltpu.VMEM((16, 256, 128), F32)] * 4,
            *[pltpu.VMEM((1024, 128), F32)] * 4,
            *[pltpu.VMEM((2048, 128), F32)] * 2,
            *[pltpu.VMEM((16, 128, 128), F32)] * 4,
            pltpu.VMEM((16, 256, 128), F32),
            pltpu.VMEM((S, 128), F32),
            pltpu.VMEM((NP, 40, 128), F32),
            pltpu.SemaphoreType.DMA((3 * NP + NT + 1,)),
            pltpu.SemaphoreType.DMA((2 * NT,)),
        ],
        compiler_params=pltpu.CompilerParams(vmem_limit_bytes=110 * 1024 * 1024),
    )(jnp.asarray(offs), A_q, A_k, A_v, B_k, B_v, A_ssm_k, B_ssm_k, A_shift_k.T, B_shift_k.T, A_ssm_D, B_ssm_D, gate_w,
      jnp.asarray(G0), jnp.asarray(E1), jnp.asarray(Ginv), jnp.asarray(Pm))


@jax.jit
def pallas_gated_mix__ssm_conv_h3__ssm_conv_h3__prompt_kernel(
    A_q, A_k, A_v, A_shift_k, A_ssm_k, A_ssm_D, B_q, B_k, B_v, B_shift_k, B_ssm_k, B_ssm_D, gate_w,
):
    return run(A_q, A_k, A_v, A_shift_k, A_ssm_k, A_ssm_D, B_q, B_k, B_v, B_shift_k, B_ssm_k, B_ssm_D, gate_w)
```

```python
import functools
import numpy as np
import jax
import jax.numpy as jnp
from jax.experimental import pallas as pl
from jax.experimental.pallas import tpu as pltpu

S, D, N1, N2 = 2048, 640, 128, 16
NT = D // 128
NP = 2 * NT
F32, BF16, U32 = jnp.float32, jnp.bfloat16, jnp.uint32


def _pack_rows(m):
    u = np.ascontiguousarray(m, dtype=np.float32).view(np.uint32).astype(np.uint64)
    h = ((u + 0x7FFF + ((u >> 16) & 1)) >> 16).astype(np.uint32)
    return (h[0::2] | (h[1::2] << np.uint32(16))).astype(np.uint32)


def _consts():
    n1 = np.arange(N1)[None, None, :]
    k1 = np.arange(N1)[None, :, None]
    n2 = np.arange(N2)[:, None, None]
    ph = -2 * np.pi * (n1 * k1 / 128.0 + n2 * k1 / 2048.0) + np.pi * (16 * n1 + n2) / 4096.0
    Gr, Gi = np.cos(ph), np.sin(ph)
    G = np.stack([Gr.reshape(N2, 16, 8, N1), Gi.reshape(N2, 16, 8, N1)], axis=2).reshape(N2, 256, N1)
    Ginv = np.transpose(G, (0, 2, 1)) / 2048.0
    Pm = np.zeros((128, 128), np.float32)
    for n2_ in range(16):
        for a in range(8):
            Pm[n2_ * 8 + a, 16 * a + n2_] = 1.0
    Ginv = Ginv.reshape(N2, 128, 2, 128).transpose(0, 2, 1, 3)
    ph0 = -2 * np.pi * (n1[0] * k1[0] / 128.0) + np.pi * (16 * n1[0]) / 4096.0
    g0 = np.concatenate([np.cos(ph0), np.sin(ph0)], axis=0).astype(np.float32)
    phe = -2 * np.pi * np.arange(N1) / 2048.0 + np.pi / 4096.0
    e1 = np.zeros((128, 128), np.float32)
    e1[:, 0], e1[:, 1] = np.cos(phe), np.sin(phe)
    return g0, e1, _pack_rows(Ginv.reshape(4096, 128)), _pack_rows(Pm)

_C1, _S1, _R = float(np.cos(np.pi / 8)), float(np.sin(np.pi / 8)), float(np.sqrt(0.5))


def _bfly4(x, sgn):
    (ar, ai), (br, bi), (cr, ci), (dr, di) = x
    t0r, t0i = ar + cr, ai + ci
    t1r, t1i = ar - cr, ai - ci
    t2r, t2i = br + dr, bi + di
    t3r, t3i = br - dr, bi - di
    x0 = (t0r + t2r, t0i + t2i)
    x2 = (t0r - t2r, t0i - t2i)
    if sgn < 0:
        x1 = (t1r + t3i, t1i - t3r)
        x3 = (t1r - t3i, t1i + t3r)
    else:
        x1 = (t1r - t3i, t1i + t3r)
        x3 = (t1r + t3i, t1i - t3r)
    return [x0, x1, x2, x3]


def _tw(z, e, sgn):
    a, b = z
    if e == 0:
        return z
    if sgn < 0:
        if e == 4: return (b, -a)
        if e == 2: return ((a + b) * _R, (b - a) * _R)
        if e == 6: return ((b - a) * _R, (a + b) * (-_R))
        if e == 1: return (a * _C1 + b * _S1, b * _C1 - a * _S1)
        if e == 3: return (a * _S1 + b * _C1, b * _S1 - a * _C1)
        if e == 9: return (a * (-_C1) - b * _S1, a * _S1 - b * _C1)
    else:
        if e == 4: return (-b, a)
        if e == 2: return ((a - b) * _R, (a + b) * _R)
        if e == 6: return ((a + b) * (-_R), (a - b) * _R)
        if e == 1: return (a * _C1 - b * _S1, b * _C1 + a * _S1)
        if e == 3: return (a * _S1 - b * _C1, b * _S1 + a * _C1)
        if e == 9: return (b * _S1 - a * _C1, a * (-_S1) - b * _C1)
    raise ValueError(e)


def fft16(x, sgn):
    A = [_bfly4([x[nb], x[nb + 4], x[nb + 8], x[nb + 12]], sgn) for nb in range(4)]
    B = [[_tw(A[nb][ka], nb * ka, sgn) for ka in range(4)] for nb in range(4)]
    X = [None] * 16
    for ka in range(4):
        o = _bfly4([B[0][ka], B[1][ka], B[2][ka], B[3][ka]], sgn)
        for kb in range(4):
            X[ka + 4 * kb] = o[kb]
    return X


def _unpack(w):
    lo = jax.lax.bitcast_convert_type(w << 16, F32)
    hi = jax.lax.bitcast_convert_type(w & jnp.uint32(0xFFFF0000), F32)
    return lo, hi


NT_DIMS = (((1,), (1,)), ((), ()))


def kernel(off_ref, q_hbm, ka_hbm, va_hbm, kb_hbm, vb_hbm, ha_hbm, hb_hbm, ska_ref, skb_ref,
           da_ref, db_ref, gw_ref, g0_ref, e1_ref, gi_hbm, pmat, o_hbm,
           qb, kb, vb, hb, gmat, gimat, ob, zh0, zh1, zu0, zu1, hp0, hp1, kv0, kv1, yp0, yp1, yb0, yb1, yb2, yb3, hh, gnat, par, sems, osems):
    ZH, ZU, HP, KV, YP, YB = (zh0, zh1), (zu0, zu1), (hp0, hp1), (kv0, kv1), (yp0, yp1), (yb0, yb1, yb2, yb3)
    k_hbm, v_hbm, h_hbm = (ka_hbm, kb_hbm), (va_hbm, vb_hbm), (ha_hbm, hb_hbm)

    def cp_k(p):
        return pltpu.make_async_copy(k_hbm[p % 2].at[0, :, pl.ds(128 * (p // 2), 128)], kb.at[p, pl.ds(16, S), :], sems.at[p])
    def cp_v(p):
        return pltpu.make_async_copy(v_hbm[p % 2].at[0, :, pl.ds(128 * (p // 2), 128)], vb.at[p], sems.at[NP + p])
    def cp_h(p):
        return pltpu.make_async_copy(h_hbm[p % 2].at[pl.ds(128 * (p // 2), 128), :], hb.at[p], sems.at[2 * NP + p])
    def cp_q(t):
        return pltpu.make_async_copy(q_hbm.at[0, :, pl.ds(128 * t, 128)], qb.at[t], sems.at[3 * NP + t])
    cp_gi = pltpu.make_async_copy(gi_hbm, gimat, sems.at[3 * NP + NT])
    def cp_o(t, hf):
        rows = pl.ds(hf * (S // 2), S // 2)
        return pltpu.make_async_copy(ob.at[t, rows, :], o_hbm.at[0, rows, pl.ds(128 * t, 128)], osems.at[2 * t + hf])

    for p in range(NP):
        kb[p, pl.ds(0, 16), :] = jnp.zeros((16, 128), BF16)
    cp_h(0).start(); cp_k(0).start(); cp_v(0).start();
    cp_h(1).start(); cp_k(1).start(); cp_v(1).start()

    sk = (ska_ref[...].astype(F32), skb_ref[...].astype(F32))
    dd = (da_ref[...].astype(F32).reshape(1, D), db_ref[...].astype(F32).reshape(1, D))
    for p in range(NP):
        b, t = p % 2, p // 2
        for tap in range(4):
            par[p, pl.ds(8 * tap, 8), :] = jnp.broadcast_to(sk[b][tap:tap + 1, 128 * t:128 * (t + 1)], (8, 128))
        par[p, pl.ds(32, 8), :] = jnp.broadcast_to(dd[b][:, 128 * t:128 * (t + 1)], (8, 128))

    kw, vw, qw, ow = kb.bitcast(U32), vb.bitcast(U32), qb.bitcast(U32), ob.bitcast(U32)
    always = off_ref[0] == 0

    def ds(start, n, mult=None):
        if isinstance(start, int):
            return pl.ds(start, n)
        return pl.ds(pl.multiple_of(start, mult or n), n)

    def ldb(ref, w0, nrows):
        return pltpu.bitcast(ref[ds(w0, nrows // 2, 8), :], BF16)

    def pk(v):
        return pltpu.bitcast(v.astype(BF16), F32)

    def stage_Tall(p):
        if True:
            pm = pltpu.bitcast(pmat[...], BF16)
            for jj in range(8):
                R = [jax.lax.dot_general(pm, hb[p, :, pl.ds(jj * 256 + 128 * u, 128)], NT_DIMS,
                                         preferred_element_type=F32) for u in range(2)]
                for n2 in range(16):
                    HP[p % 2][pl.ds(jj * 8 + n2 * 64, 8), :] = pk(
                        jnp.concatenate([R[0][8 * n2:8 * n2 + 8], R[1][8 * n2:8 * n2 + 8]], axis=0))
    def stage_P(p, a2, ms=range(8)):
        s = [jnp.concatenate([par[p, pl.ds(8 * tap, 8), :]] * 2, axis=0) for tap in range(4)]
        base = a2 * 128
        ksub = kw.at[p, ds(base + 8, 128, 8), :]
        kprev = kw.at[p, ds(base, 128), :]
        vsub = vw.at[p, ds(base, 128), :]
        kk = {}
        def getk(n):
            if n not in kk:
                m = (n // 2) if n >= 0 else ((n + 16) // 2)
                lo, hi = _unpack((ksub if n >= 0 else kprev)[pl.ds(m, 16, stride=8), :])
                b0 = 2 * m if n >= 0 else 2 * m - 16
                kk[b0], kk[b0 + 1] = lo, hi
            return kk[n]
        kvs = KV[p % 2].at[ds(a2 * 8, 1024 - 56, 8), :]
        for m in ms:
            vlo, vhi = _unpack(vsub[pl.ds(m, 16, stride=8), :])
            for n2, vv in ((2 * m, vlo), (2 * m + 1, vhi)):
                acc = getk(n2) * s[0] + getk(n2 - 1) * s[1] + getk(n2 - 2) * s[2] + getk(n2 - 3) * s[3]
                kvs[pl.ds(n2 * 64, 8), :] = pk(acc * vv)

    def stage_V(p, g):
        xh = ZH[p % 2].at[:, ds(g * 16, 16), :]
        xu = ZU[p % 2].at[:, ds(g * 16, 16), :]
        xo = hh.at[:, ds(g * 16, 16), :]
        ys = YP[p % 2].at[ds(g * 8, 2048 - 120, 8), :]
        z = [(xh[n2, 0:8, :], xh[n2, 8:16, :]) for n2 in range(16)]
        z[0] = (z[0][0] + par[p, pl.ds(32, 8), :], z[0][1])
        H = fft16(z, -1)
        for k2 in range(16):
            xo[k2, 0:8, :] = H[k2][0]
            xo[k2, 8:16, :] = H[k2][1]
        z = [(xu[n2, 0:8, :], xu[n2, 8:16, :]) for n2 in range(16)]
        Uu = fft16(z, -1)
        Y = []
        for k2 in range(16):
            hr, hi = xo[k2, 0:8, :], xo[k2, 8:16, :]
            ur, ui = Uu[k2]
            Y.append((ur * hr - ui * hi, ur * hi + ui * hr))
        T = fft16(Y, +1)
        for n2 in range(16):
            ys[pl.ds(n2 * 128, 8), :] = pk(jnp.concatenate([T[n2][0], T[n2][1]], axis=0))

    def stage_B(t, a):
        ya_ref = YB[(2 * t) % 4].at[:, ds(a * 8, 8), :]
        yb_ref = YB[(2 * t + 1) % 4].at[:, ds(a * 8, 8), :]
        qsub = qw.at[t, ds(a * 64, 64), :]
        osub = ow.at[t, ds(a * 64, 64), :]
        gsub = gnat.at[ds(a * 128, 128), :]
        for m in range(8):
            qs = _unpack(qsub[pl.ds(m, 8, stride=8), :])
            res = []
            for u in range(2):
                n2 = 2 * m + u
                ya, yv = ya_ref[n2], yb_ref[n2]
                gg = gsub[pl.ds(n2, 8, stride=16), :]
                res.append(qs[u] * (yv + gg * (ya - yv)))
            osub[pl.ds(m, 8, stride=8), :] = pltpu.pack_elementwise((res[0], res[1]), packed_dtype=BF16)

    def gate():
        gw = gw_ref[...].reshape(1, D)
        gw8 = jnp.broadcast_to(gw, (8, D))
        for jt in range(S // 128):
            acc = None
            for t in range(NT):
                part = jax.lax.dot_general(gw8[:, 128 * t:128 * (t + 1)], qb[t, pl.ds(128 * jt, 128), :], NT_DIMS,
                                           preferred_element_type=F32)
                acc = part if acc is None else acc + part
            gs = jax.nn.sigmoid(acc)
            gnat[pl.ds(128 * jt, 128), :] = jnp.transpose(jnp.broadcast_to(gs[0:1, :], (128, 128)))

    def gen_g(gq, carry):
        st = []
        for w in range(4):
            g = 4 * gq + w
            e = e1_ref[ds(g * 8, 8), :]
            st.append([g0_ref[ds(g * 8, 8), :], g0_ref[ds(128 + g * 8, 8), :],
                       jnp.broadcast_to(e[:, 0:1], (8, 128)), jnp.broadcast_to(e[:, 1:2], (8, 128))])
        dst = gmat.at[ds(gq * 32, 2048 - 96, 32), :]
        for n2 in range(16):
            for w in range(4):
                gr, gi, er, ei = st[w]
                dst[pl.ds(n2 * 128 + w * 8, 8), :] = pltpu.bitcast(jnp.concatenate([gr, gi], axis=0).astype(BF16), U32)
                if n2 < 15:
                    st[w][0], st[w][1] = gr * er - gi * ei, gr * ei + gi * er
        return carry
    jax.lax.fori_loop(0, 4, gen_g, 0)

    GATE_SLOT = 5
    n_slots = NP + 5
    for s in range(n_slots):
        pT, pF, pV, pI = s, s - 1, s - 2, s - 3
        doT, doF, doV, doI = (0 <= pT < NP), (0 <= pF < NP), (0 <= pV < NP), (0 <= pI < NP)
        tB, hB = None, None
        if s >= 5 and (s - 5) // 2 < NT:
            tB, hB = (s - 5) // 2, (s - 5) % 2
        if s + 2 < NP:
            cp_h(s + 2).start(); cp_k(s + 2).start(); cp_v(s + 2).start()
        if s == 1:
            cp_gi.start()
        if s < NT:
            cp_q(s).start()
        if s == 3:
            cp_gi.wait()
        if s == GATE_SLOT:
            for t in range(NT):
                cp_q(t).wait()
            gate()
        def dot_F(p, i):
            g = ldb(gmat, i * 128, 256)
            ZU[p % 2][i] = jnp.dot(g, ldb(KV[p % 2], i * 64, 128), preferred_element_type=F32)
            ZH[p % 2][i] = jnp.dot(g, ldb(HP[p % 2], i * 64, 128), preferred_element_type=F32)

        def dot_I(p, i):
            lhs = jnp.concatenate([ldb(gimat, i * 128, 128), ldb(gimat, i * 128 + 64, 128)], axis=1)
            YB[p % 4][i] = jnp.dot(lhs, ldb(YP[p % 2], i * 128, 256), preferred_element_type=F32)

        if not doV and (doF or doI):
            for i in range(16):
              if doF:
                  dot_F(pF, i)
              if doI:
                  dot_I(pI, i)
            doF = doI = False

        if doT:
            cp_h(pT).wait()
            stage_Tall(pT)
        if doT:
            cp_k(pT).wait(); cp_v(pT).wait()

        def body(j, carry, pT=pT, pF=pF, pV=pV, pI=pI, doT=doT, doF=doF, doV=doV, doI=doI, tB=tB, hB=hB):
            def common(i):
                if doV:
                    stage_V(pV, i)
                if doF:
                    dot_F(pF, i)
                if doI:
                    dot_I(pI, i)
            common(2 * j)
            if doT:
                stage_P(pT, j, range(8))
            def second():
                common(2 * j + 1)
                if tB is not None:
                    stage_B(tB, hB * 8 + j)
            if doF or doI or doV:
                pl.when(always)(second)
            else:
                second()
            return carry
        if tB is not None and not (doT or doF or doV or doI):
            def bbody(j, c, tB=tB, hB=hB):
                stage_B(tB, hB * 8 + 2 * j)
                stage_B(tB, hB * 8 + 2 * j + 1)
                return c
            jax.lax.fori_loop(0, 4, bbody, 0)
        elif doT or doF or doV or doI or tB is not None:
            jax.lax.fori_loop(0, 8, body, 0)
        if tB is not None and "A" == "sep":
            def bbody(j, c, tB=tB, hB=hB):
                stage_B(tB, hB * 8 + 2 * j)
                stage_B(tB, hB * 8 + 2 * j + 1)
                return c
            jax.lax.fori_loop(0, 4, bbody, 0)
        if tB is not None:
            cp_o(tB, hB).start()
    for t in range(NT):
        cp_o(t, 0).wait(); cp_o(t, 1).wait()


def run(A_q, A_k, A_v, A_shift_k, A_ssm_k, A_ssm_D, B_q, B_k, B_v, B_shift_k, B_ssm_k, B_ssm_D, gate_w):
    G0, E1, Ginv, Pm = _consts()
    offs = np.zeros((1,), np.int32)
    any_spec = pl.BlockSpec(memory_space=pl.ANY)
    vm = pl.BlockSpec(memory_space=pltpu.VMEM)
    return pl.pallas_call(
        kernel,
        in_specs=[pl.BlockSpec(memory_space=pltpu.SMEM)] + [any_spec] * 7 + [vm] * 7 + [any_spec, vm],
        out_specs=any_spec,
        out_shape=jax.ShapeDtypeStruct((1, S, D), BF16),
        scratch_shapes=[
            pltpu.VMEM((NT, S, 128), BF16),
            pltpu.VMEM((NP, S + 16, 128), BF16),
            pltpu.VMEM((NP, S, 128), BF16),
            pltpu.VMEM((NP, 128, S), BF16),
            pltpu.VMEM((2048, 128), U32),
            pltpu.VMEM((2048, 128), U32),
            pltpu.VMEM((NT, S, 128), BF16),
            *[pltpu.VMEM((16, 256, 128), F32)] * 4,
            *[pltpu.VMEM((1024, 128), F32)] * 4,
            *[pltpu.VMEM((2048, 128), F32)] * 2,
            *[pltpu.VMEM((16, 128, 128), F32)] * 4,
            pltpu.VMEM((16, 256, 128), F32),
            pltpu.VMEM((S, 128), F32),
            pltpu.VMEM((NP, 40, 128), F32),
            pltpu.SemaphoreType.DMA((3 * NP + NT + 1,)),
            pltpu.SemaphoreType.DMA((2 * NT,)),
        ],
        compiler_params=pltpu.CompilerParams(vmem_limit_bytes=110 * 1024 * 1024),
    )(jnp.asarray(offs), A_q, A_k, A_v, B_k, B_v, A_ssm_k, B_ssm_k, A_shift_k.T, B_shift_k.T, A_ssm_D, B_ssm_D, gate_w,
      jnp.asarray(G0), jnp.asarray(E1), jnp.asarray(Ginv), jnp.asarray(Pm))


@jax.jit
def pallas_gated_mix__ssm_conv_h3__ssm_conv_h3__prompt_kernel(
    A_q, A_k, A_v, A_shift_k, A_ssm_k, A_ssm_D, B_q, B_k, B_v, B_shift_k, B_ssm_k, B_ssm_D, gate_w,
):
    return run(A_q, A_k, A_v, A_shift_k, A_ssm_k, A_ssm_D, B_q, B_k, B_v, B_shift_k, B_ssm_k, B_ssm_D, gate_w)
```

```python
import numpy as np
import jax
import jax.numpy as jnp
from jax.experimental import pallas as pl
from jax.experimental.pallas import tpu as pltpu

S, D, N1, N2 = 2048, 640, 128, 16
NT = D // 128
NP = 2 * NT
F32, BF16, U32 = jnp.float32, jnp.bfloat16, jnp.uint32


def _pack_rows(m):
    u = np.ascontiguousarray(m, dtype=np.float32).view(np.uint32).astype(np.uint64)
    h = ((u + 0x7FFF + ((u >> 16) & 1)) >> 16).astype(np.uint32)
    return (h[0::2] | (h[1::2] << np.uint32(16))).astype(np.uint32)


def _consts():
    n1 = np.arange(N1)[None, None, :]
    k1 = np.arange(N1)[None, :, None]
    n2 = np.arange(N2)[:, None, None]
    ph = -2 * np.pi * (n1 * k1 / 128.0 + n2 * k1 / 2048.0) + np.pi * (16 * n1 + n2) / 4096.0
    Gr, Gi = np.cos(ph), np.sin(ph)
    G = np.stack([Gr.reshape(N2, 16, 8, N1), Gi.reshape(N2, 16, 8, N1)], axis=2).reshape(N2, 256, N1)
    Ginv = np.transpose(G, (0, 2, 1)) / 2048.0
    Pm = np.zeros((128, 128), np.float32)
    for n2_ in range(16):
        for a in range(8):
            Pm[n2_ * 8 + a, 16 * a + n2_] = 1.0
    Ginv = Ginv.reshape(N2, 128, 2, 128).transpose(0, 2, 1, 3)
    ph0 = -2 * np.pi * (n1[0] * k1[0] / 128.0) + np.pi * (16 * n1[0]) / 4096.0
    g0 = np.concatenate([np.cos(ph0), np.sin(ph0)], axis=0).astype(np.float32)
    phe = -2 * np.pi * np.arange(N1) / 2048.0 + np.pi / 4096.0
    e1 = np.zeros((128, 128), np.float32)
    e1[:, 0], e1[:, 1] = np.cos(phe), np.sin(phe)
    return g0, e1, _pack_rows(Ginv.reshape(4096, 128)), _pack_rows(Pm)

_C1, _S1, _R = float(np.cos(np.pi / 8)), float(np.sin(np.pi / 8)), float(np.sqrt(0.5))


def _bfly4(x, sgn):
    (ar, ai), (br, bi), (cr, ci), (dr, di) = x
    t0r, t0i = ar + cr, ai + ci
    t1r, t1i = ar - cr, ai - ci
    t2r, t2i = br + dr, bi + di
    t3r, t3i = br - dr, bi - di
    x0 = (t0r + t2r, t0i + t2i)
    x2 = (t0r - t2r, t0i - t2i)
    if sgn < 0:
        x1 = (t1r + t3i, t1i - t3r)
        x3 = (t1r - t3i, t1i + t3r)
    else:
        x1 = (t1r - t3i, t1i + t3r)
        x3 = (t1r + t3i, t1i - t3r)
    return [x0, x1, x2, x3]


def _tw(z, e, sgn):
    a, b = z
    if e == 0:
        return z
    if sgn < 0:
        if e == 4: return (b, -a)
        if e == 2: return ((a + b) * _R, (b - a) * _R)
        if e == 6: return ((b - a) * _R, (a + b) * (-_R))
        if e == 1: return (a * _C1 + b * _S1, b * _C1 - a * _S1)
        if e == 3: return (a * _S1 + b * _C1, b * _S1 - a * _C1)
        if e == 9: return (a * (-_C1) - b * _S1, a * _S1 - b * _C1)
    else:
        if e == 4: return (-b, a)
        if e == 2: return ((a - b) * _R, (a + b) * _R)
        if e == 6: return ((a + b) * (-_R), (a - b) * _R)
        if e == 1: return (a * _C1 - b * _S1, b * _C1 + a * _S1)
        if e == 3: return (a * _S1 - b * _C1, b * _S1 + a * _C1)
        if e == 9: return (b * _S1 - a * _C1, a * (-_S1) - b * _C1)
    raise ValueError(e)


def fft16(x, sgn):
    A = [_bfly4([x[nb], x[nb + 4], x[nb + 8], x[nb + 12]], sgn) for nb in range(4)]
    B = [[_tw(A[nb][ka], nb * ka, sgn) for ka in range(4)] for nb in range(4)]
    X = [None] * 16
    for ka in range(4):
        o = _bfly4([B[0][ka], B[1][ka], B[2][ka], B[3][ka]], sgn)
        for kb in range(4):
            X[ka + 4 * kb] = o[kb]
    return X


def _unpack(w):
    lo = jax.lax.bitcast_convert_type(w << 16, F32)
    hi = jax.lax.bitcast_convert_type(w & jnp.uint32(0xFFFF0000), F32)
    return lo, hi


NT_DIMS = (((1,), (1,)), ((), ()))


def kernel(off_ref, q_hbm, ka_hbm, va_hbm, kb_hbm, vb_hbm, ha_hbm, hb_hbm, ska_ref, skb_ref,
           da_ref, db_ref, gw_ref, g0_ref, e1_ref, gi_hbm, pmat, o_hbm,
           qb, kb, vb, hb, gmat, gimat, ob, zh0, zh1, zu0, zu1, hp0, hp1, kv0, kv1, yp0, yp1, yb0, yb1, yb2, yb3, hh, gnat, par, sems, osems):
    ZH, ZU, HP, KV, YP, YB = (zh0, zh1), (zu0, zu1), (hp0, hp1), (kv0, kv1), (yp0, yp1), (yb0, yb1, yb2, yb3)
    k_hbm, v_hbm, h_hbm = (ka_hbm, kb_hbm), (va_hbm, vb_hbm), (ha_hbm, hb_hbm)

    def cp_k(p):
        return pltpu.make_async_copy(k_hbm[p % 2].at[0, :, pl.ds(128 * (p // 2), 128)], kb.at[p, pl.ds(16, S), :], sems.at[p])
    def cp_v(p):
        return pltpu.make_async_copy(v_hbm[p % 2].at[0, :, pl.ds(128 * (p // 2), 128)], vb.at[p], sems.at[NP + p])
    def cp_h(p):
        return pltpu.make_async_copy(h_hbm[p % 2].at[pl.ds(128 * (p // 2), 128), :], hb.at[p], sems.at[2 * NP + p])
    def cp_q(t):
        return pltpu.make_async_copy(q_hbm.at[0, :, pl.ds(128 * t, 128)], qb.at[t], sems.at[3 * NP + t])
    cp_gi = pltpu.make_async_copy(gi_hbm, gimat, sems.at[3 * NP + NT])
    def cp_o(t, hf):
        rows = pl.ds(hf * (S // 2), S // 2)
        return pltpu.make_async_copy(ob.at[t, rows, :], o_hbm.at[0, rows, pl.ds(128 * t, 128)], osems.at[2 * t + hf])

    for p in range(NP):
        kb[p, pl.ds(0, 16), :] = jnp.zeros((16, 128), BF16)
    cp_h(0).start(); cp_k(0).start(); cp_v(0).start();
    cp_h(1).start(); cp_k(1).start(); cp_v(1).start()

    sk = (ska_ref[...].astype(F32), skb_ref[...].astype(F32))
    dd = (da_ref[...].astype(F32).reshape(1, D), db_ref[...].astype(F32).reshape(1, D))
    for p in range(NP):
        b, t = p % 2, p // 2
        for tap in range(4):
            par[p, pl.ds(8 * tap, 8), :] = jnp.broadcast_to(sk[b][tap:tap + 1, 128 * t:128 * (t + 1)], (8, 128))
        par[p, pl.ds(32, 8), :] = jnp.broadcast_to(dd[b][:, 128 * t:128 * (t + 1)], (8, 128))

    kw, vw, qw, ow = kb.bitcast(U32), vb.bitcast(U32), qb.bitcast(U32), ob.bitcast(U32)
    always = off_ref[0] == 0

    def ds(start, n, mult=None):
        if isinstance(start, int):
            return pl.ds(start, n)
        return pl.ds(pl.multiple_of(start, mult or n), n)

    def ldb(ref, w0, nrows):
        return pltpu.bitcast(ref[ds(w0, nrows // 2, 8), :], BF16)

    def pk(v):
        return pltpu.bitcast(v.astype(BF16), F32)

    def stage_Tall(p):
        pm = pltpu.bitcast(pmat[...], BF16)
        for jj in range(8):
            R = [jax.lax.dot_general(pm, hb[p, :, pl.ds(jj * 256 + 128 * u, 128)], NT_DIMS,
                                     preferred_element_type=F32) for u in range(2)]
            for n2 in range(16):
                HP[p % 2][pl.ds(jj * 8 + n2 * 64, 8), :] = pk(
                    jnp.concatenate([R[0][8 * n2:8 * n2 + 8], R[1][8 * n2:8 * n2 + 8]], axis=0))
    def stage_P(p, a2, ms=range(8)):
        s = [jnp.concatenate([par[p, pl.ds(8 * tap, 8), :]] * 2, axis=0) for tap in range(4)]
        base = a2 * 128
        ksub = kw.at[p, ds(base + 8, 128, 8), :]
        kprev = kw.at[p, ds(base, 128), :]
        vsub = vw.at[p, ds(base, 128), :]
        kk = {}
        def getk(n):
            if n not in kk:
                m = (n // 2) if n >= 0 else ((n + 16) // 2)
                lo, hi = _unpack((ksub if n >= 0 else kprev)[pl.ds(m, 16, stride=8), :])
                b0 = 2 * m if n >= 0 else 2 * m - 16
                kk[b0], kk[b0 + 1] = lo, hi
            return kk[n]
        kvs = KV[p % 2].at[ds(a2 * 8, 1024 - 56, 8), :]
        for m in ms:
            vlo, vhi = _unpack(vsub[pl.ds(m, 16, stride=8), :])
            for n2, vv in ((2 * m, vlo), (2 * m + 1, vhi)):
                acc = getk(n2) * s[0] + getk(n2 - 1) * s[1] + getk(n2 - 2) * s[2] + getk(n2 - 3) * s[3]
                kvs[pl.ds(n2 * 64, 8), :] = pk(acc * vv)

    def stage_V(p, g):
        xh = ZH[p % 2].at[:, ds(g * 16, 16), :]
        xu = ZU[p % 2].at[:, ds(g * 16, 16), :]
        xo = hh.at[:, ds(g * 16, 16), :]
        ys = YP[p % 2].at[ds(g * 8, 2048 - 120, 8), :]
        z = [(xh[n2, 0:8, :], xh[n2, 8:16, :]) for n2 in range(16)]
        z[0] = (z[0][0] + par[p, pl.ds(32, 8), :], z[0][1])
        H = fft16(z, -1)
        for k2 in range(16):
            xo[k2, 0:8, :] = H[k2][0]
            xo[k2, 8:16, :] = H[k2][1]
        z = [(xu[n2, 0:8, :], xu[n2, 8:16, :]) for n2 in range(16)]
        Uu = fft16(z, -1)
        Y = []
        for k2 in range(16):
            hr, hi = xo[k2, 0:8, :], xo[k2, 8:16, :]
            ur, ui = Uu[k2]
            Y.append((ur * hr - ui * hi, ur * hi + ui * hr))
        T = fft16(Y, +1)
        for n2 in range(16):
            ys[pl.ds(n2 * 128, 8), :] = pk(jnp.concatenate([T[n2][0], T[n2][1]], axis=0))

    def stage_B(t, a):
        ya_ref = YB[(2 * t) % 4].at[:, ds(a * 8, 8), :]
        yb_ref = YB[(2 * t + 1) % 4].at[:, ds(a * 8, 8), :]
        qsub = qw.at[t, ds(a * 64, 64), :]
        osub = ow.at[t, ds(a * 64, 64), :]
        gsub = gnat.at[ds(a * 128, 128), :]
        for m in range(8):
            qs = _unpack(qsub[pl.ds(m, 8, stride=8), :])
            res = []
            for u in range(2):
                n2 = 2 * m + u
                ya, yv = ya_ref[n2], yb_ref[n2]
                gg = gsub[pl.ds(n2, 8, stride=16), :]
                res.append(qs[u] * (yv + gg * (ya - yv)))
            osub[pl.ds(m, 8, stride=8), :] = pltpu.pack_elementwise((res[0], res[1]), packed_dtype=BF16)

    def gate():
        gw = gw_ref[...].reshape(1, D)
        gw8 = jnp.broadcast_to(gw, (8, D))
        for jt in range(S // 128):
            acc = None
            for t in range(NT):
                part = jax.lax.dot_general(gw8[:, 128 * t:128 * (t + 1)], qb[t, pl.ds(128 * jt, 128), :], NT_DIMS,
                                           preferred_element_type=F32)
                acc = part if acc is None else acc + part
            gs = jax.nn.sigmoid(acc)
            gnat[pl.ds(128 * jt, 128), :] = jnp.transpose(jnp.broadcast_to(gs[0:1, :], (128, 128)))

    def gen_g(gq, carry):
        st = []
        for w in range(4):
            g = 4 * gq + w
            e = e1_ref[ds(g * 8, 8), :]
            st.append([g0_ref[ds(g * 8, 8), :], g0_ref[ds(128 + g * 8, 8), :],
                       jnp.broadcast_to(e[:, 0:1], (8, 128)), jnp.broadcast_to(e[:, 1:2], (8, 128))])
        dst = gmat.at[ds(gq * 32, 2048 - 96, 32), :]
        for n2 in range(16):
            for w in range(4):
                gr, gi, er, ei = st[w]
                dst[pl.ds(n2 * 128 + w * 8, 8), :] = pltpu.bitcast(jnp.concatenate([gr, gi], axis=0).astype(BF16), U32)
                if n2 < 15:
                    st[w][0], st[w][1] = gr * er - gi * ei, gr * ei + gi * er
        return carry
    jax.lax.fori_loop(0, 4, gen_g, 0)

    GATE_SLOT = 5
    n_slots = NP + 5
    for s in range(n_slots):
        pT, pF, pV, pI = s, s - 1, s - 2, s - 3
        doT, doF, doV, doI = (0 <= pT < NP), (0 <= pF < NP), (0 <= pV < NP), (0 <= pI < NP)
        tB, hB = None, None
        if s >= 5 and (s - 5) // 2 < NT:
            tB, hB = (s - 5) // 2, (s - 5) % 2
        if s + 2 < NP:
            cp_h(s + 2).start(); cp_k(s + 2).start(); cp_v(s + 2).start()
        if s == 1:
            cp_gi.start()
        if s < NT:
            cp_q(s).start()
        if s == 3:
            cp_gi.wait()
        if s == GATE_SLOT:
            for t in range(NT):
                cp_q(t).wait()
            gate()
        def dot_F(p, i):
            g = ldb(gmat, i * 128, 256)
            ZU[p % 2][i] = jnp.dot(g, ldb(KV[p % 2], i * 64, 128), preferred_element_type=F32)
            ZH[p % 2][i] = jnp.dot(g, ldb(HP[p % 2], i * 64, 128), preferred_element_type=F32)

        def dot_I(p, i):
            lhs = jnp.concatenate([ldb(gimat, i * 128, 128), ldb(gimat, i * 128 + 64, 128)], axis=1)
            YB[p % 4][i] = jnp.dot(lhs, ldb(YP[p % 2], i * 128, 256), preferred_element_type=F32)

        if not doV and (doF or doI):
            for i in range(16):
              if doF:
                  dot_F(pF, i)
              if doI:
                  dot_I(pI, i)
            doF = doI = False

        if doT:
            cp_h(pT).wait()
            stage_Tall(pT)
        if doT:
            cp_k(pT).wait(); cp_v(pT).wait()

        def body(j, carry, pT=pT, pF=pF, pV=pV, pI=pI, doT=doT, doF=doF, doV=doV, doI=doI, tB=tB, hB=hB):
            def common(i):
                if doV:
                    stage_V(pV, i)
                if doF:
                    dot_F(pF, i)
                if doI:
                    dot_I(pI, i)
            common(2 * j)
            if doT:
                stage_P(pT, j, range(8))
            def second():
                common(2 * j + 1)
                if tB is not None:
                    stage_B(tB, hB * 8 + j)
            if doF or doI or doV:
                pl.when(always)(second)
            else:
                second()
            return carry
        if tB is not None and not (doT or doF or doV or doI):
            def bbody(j, c, tB=tB, hB=hB):
                stage_B(tB, hB * 8 + 2 * j)
                stage_B(tB, hB * 8 + 2 * j + 1)
                return c
            jax.lax.fori_loop(0, 4, bbody, 0)
        elif doT or doF or doV or doI or tB is not None:
            jax.lax.fori_loop(0, 8, body, 0)
        if tB is not None and "A" == "sep":
            def bbody(j, c, tB=tB, hB=hB):
                stage_B(tB, hB * 8 + 2 * j)
                stage_B(tB, hB * 8 + 2 * j + 1)
                return c
            jax.lax.fori_loop(0, 4, bbody, 0)
        if tB is not None:
            cp_o(tB, hB).start()
    for t in range(NT):
        cp_o(t, 0).wait(); cp_o(t, 1).wait()


def run(A_q, A_k, A_v, A_shift_k, A_ssm_k, A_ssm_D, B_q, B_k, B_v, B_shift_k, B_ssm_k, B_ssm_D, gate_w):
    G0, E1, Ginv, Pm = _consts()
    offs = np.zeros((1,), np.int32)
    any_spec = pl.BlockSpec(memory_space=pl.ANY)
    vm = pl.BlockSpec(memory_space=pltpu.VMEM)
    return pl.pallas_call(
        kernel,
        in_specs=[pl.BlockSpec(memory_space=pltpu.SMEM)] + [any_spec] * 7 + [vm] * 7 + [any_spec, vm],
        out_specs=any_spec,
        out_shape=jax.ShapeDtypeStruct((1, S, D), BF16),
        scratch_shapes=[
            pltpu.VMEM((NT, S, 128), BF16),
            pltpu.VMEM((NP, S + 16, 128), BF16),
            pltpu.VMEM((NP, S, 128), BF16),
            pltpu.VMEM((NP, 128, S), BF16),
            pltpu.VMEM((2048, 128), U32),
            pltpu.VMEM((2048, 128), U32),
            pltpu.VMEM((NT, S, 128), BF16),
            *[pltpu.VMEM((16, 256, 128), F32)] * 4,
            *[pltpu.VMEM((1024, 128), F32)] * 4,
            *[pltpu.VMEM((2048, 128), F32)] * 2,
            *[pltpu.VMEM((16, 128, 128), F32)] * 4,
            pltpu.VMEM((16, 256, 128), F32),
            pltpu.VMEM((S, 128), F32),
            pltpu.VMEM((NP, 40, 128), F32),
            pltpu.SemaphoreType.DMA((3 * NP + NT + 1,)),
            pltpu.SemaphoreType.DMA((2 * NT,)),
        ],
        compiler_params=pltpu.CompilerParams(vmem_limit_bytes=110 * 1024 * 1024),
    )(jnp.asarray(offs), A_q, A_k, A_v, B_k, B_v, A_ssm_k, B_ssm_k, A_shift_k.T, B_shift_k.T, A_ssm_D, B_ssm_D, gate_w,
      jnp.asarray(G0), jnp.asarray(E1), jnp.asarray(Ginv), jnp.asarray(Pm))


@jax.jit
def pallas_gated_mix__ssm_conv_h3__ssm_conv_h3__prompt_kernel(
    A_q, A_k, A_v, A_shift_k, A_ssm_k, A_ssm_D, B_q, B_k, B_v, B_shift_k, B_ssm_k, B_ssm_D, gate_w,
):
    return run(A_q, A_k, A_v, A_shift_k, A_ssm_k, A_ssm_D, B_q, B_k, B_v, B_shift_k, B_ssm_k, B_ssm_D, gate_w)
```
